```python
import os as _os
_os.environ.setdefault("JAX_PLATFORMS", "cpu")
import jax
import jax.numpy as jnp

def _softmax(x, axis=-1):
    return jax.nn.softmax(x, axis=axis)
def _gelu(x):
    return jax.nn.gelu(x, approximate=True)
def _silu(x):
    return jax.nn.silu(x)
def _sigmoid(x):
    return jax.nn.sigmoid(x)
def _layernorm(x, axis=-1, eps=1e-5):
    m = jnp.mean(x, axis=axis, keepdims=True)
    v = jnp.var(x, axis=axis, keepdims=True)
    return (x - m) / jnp.sqrt(v + eps)
def _scatter_add(tgt, idx, src, axis=0):
    return tgt.at[idx].add(src)
def _segment_sum(src, seg, n):
    return jax.ops.segment_sum(src, seg, n)
class _Rng:
    def __init__(self, key):
        self._k = key
    def _next(self):
        self._k, sub = jax.random.split(self._k)
        return sub
    def normal(self, shape):
        return jax.random.normal(self._next(), shape, dtype=jnp.bfloat16)
    def randint(self, lo, hi, shape):
        return jax.random.randint(self._next(), shape, lo, hi, dtype=jnp.int32)
    def uniform(self, shape, lo=0.0, hi=1.0):
        return jax.random.uniform(self._next(), shape, jnp.bfloat16, lo, hi)
    def permutation(self, n):
        return jax.random.permutation(self._next(), n)


kernel_name = 'interleave_layers__spectral_gfnet__mixer_token_mlp__prompt'

def setup_inputs():
    _rng = _Rng(jax.random.key(int.from_bytes(__import__("os").urandom(4), "little")))
    _w = (lambda a: (lambda t: t.astype(jnp.bfloat16) if jnp.issubdtype(t.dtype, jnp.floating) else t)(jnp.asarray(a)))
    def _A_setup():
        B, S, D = 1, 2048, 640
        Df = D // 2 + 1
        return {
            "x": _w((lambda *s: _rng.normal(s) * 0.05)(B, S, D)),
            "w_r": _w((lambda *s: _rng.normal(s) * 0.2)(S, Df) * 0.02),
            "w_i": _w((lambda *s: _rng.normal(s) * 0.2)(S, Df) * 0.02),
        }
    _A_in = _A_setup()

    def _B_setup():
        B, S, D, F = 1, 2048, 640, 1728
        return {
            "x": _w((lambda *s: _rng.normal(s) * 0.05)(B, S, D)),
            "w1": _w((lambda *s: _rng.normal(s) * 0.1)(S, F) * (S ** -0.5)),
            "b1": _w((lambda *s: _rng.normal(s) * 0.1)(F) * 0.02),
            "w2": _w((lambda *s: _rng.normal(s) * 0.1)(F, S) * (F ** -0.5)),
            "b2": _w((lambda *s: _rng.normal(s) * 0.1)(S) * 0.02),
        }
    _B_in = _B_setup()

    return {
        "A_x": _A_in["x"],
        "A_w_r": _A_in["w_r"],
        "A_w_i": _A_in["w_i"],
        "B_x": _B_in["x"],
        "B_w1": _B_in["w1"],
        "B_b1": _B_in["b1"],
        "B_w2": _B_in["w2"],
        "B_b2": _B_in["b2"],
    }

def reference(A_x, A_w_r, A_w_i, B_x, B_w1, B_b1, B_w2, B_b2):
    def _A_ref(x, w_r, w_i):
        B, S, D = x.shape
        X = (lambda x, axes=(-2,-1): jnp.fft.rfft2(x.astype(jnp.float32), axes=axes))(x, axes=(-2, -1))
        W = w_r + 1j * w_i
        X = X * W
        y = (lambda x, s, axes=(-2,-1): jnp.fft.irfft2(x, s=s, axes=axes).astype(jnp.bfloat16))(X, (S, D), axes=(-2, -1))
        return y

    def _B_ref(x, w1, b1, w2, b2):
        B, S, D = x.shape
        h = _layernorm(x, axis=-1)
        u = jnp.einsum("bsd,sf->bdf", h, w1) + b1
        u = _gelu(u)
        y = jnp.einsum("bdf,fs->bds", u, w2) + b2
        return (lambda x, *d: x.transpose(*d))(y, 0, 2, 1)

    x = A_x
    x = x + _A_ref(_layernorm(x, axis=-1), A_w_r, A_w_i)
    x = x + _B_ref(_layernorm(x, axis=-1), B_w1, B_b1, B_w2, B_b2)
    x = x + _A_ref(_layernorm(x, axis=-1), A_w_r, A_w_i)
    x = x + _B_ref(_layernorm(x, axis=-1), B_w1, B_b1, B_w2, B_b2)
    return x
```

```python
import functools
import numpy as np
import jax
import jax.numpy as jnp
from jax import lax
import jax.experimental.pallas as pl
import jax.experimental.pallas.tpu as pltpu

S, D, F = 2048, 640, 1728
NG = 41
PR = NG * 16
EPS = 1e-5
f32, bf16 = jnp.float32, jnp.bfloat16
NT = (((1,), (1,)), ((), ()))

C1, C2 = float(np.cos(2 * np.pi / 5)), float(np.cos(4 * np.pi / 5))
S1, S2 = float(np.sin(2 * np.pi / 5)), float(np.sin(4 * np.pi / 5))


def _consts():
    G = np.zeros((5, 144, 128))
    GI = np.zeros((5, 128, 128))
    for a in range(5):
        d = a + 5 * np.arange(128)
        for g in range(8):
            for i in range(8):
                l = 8 * g + i
                G[a, 16 * g + i] = np.cos(2 * np.pi * d * l / 640)
                G[a, 16 * g + 8 + i] = -np.sin(2 * np.pi * d * l / 640)
                GI[a, :, 16 * g + i] = (1 if l == 0 else 2) * np.cos(2 * np.pi * d * l / 640)
                GI[a, :, 16 * g + 8 + i] = -2 * np.sin(2 * np.pi * d * l / 640)
        for i, f in enumerate((64, 192, 320)):
            G[a, 128 + i] = np.cos(2 * np.pi * d * f / 640)
            G[a, 136 + i] = -np.sin(2 * np.pi * d * f / 640)
        GI[a, :, 8] = (-1.0) ** np.arange(128)
    GI = GI / (640 * 2048)
    s2 = np.arange(128)
    ang = [2 * np.pi * ((np.outer(s2, k1 + 16 * np.arange(128))) % 2048) / 2048 for k1 in range(16)]
    MS = np.stack([np.concatenate([np.cos(a), -np.sin(a)], 1) for a in ang])
    MI = np.stack([np.concatenate([np.cos(a).T, np.sin(a).T], 1) for a in ang])
    P128 = np.zeros((128, 128))
    for k1 in range(16):
        for j in range(8):
            P128[8 * k1 + j, k1 + 16 * j] = 1.0
    PA = np.zeros((144, 128)); PB = np.zeros((144, 128)); PC = np.zeros((80, 128))
    for l in range(64):
        PA[l, l] = 1.0; PB[l, l] = 1.0; PC[l, l] = 1.0
        if l > 0:
            PA[64 + l, 128 - l] = 1.0
            PB[64 + l, 128 - l] = 1.0
    PA[128, 64] = 1.0
    PB[128, 0] = 1.0
    PB[136 + 1, 64] = 1.0
    PC[64, 0] = 1.0
    PC[72 + 2, 64] = 1.0
    PM = np.concatenate([P128, PA, PB, PC], 0)
    return G, GI, MS, MI, PM


def _cmul_const(x, e, inv):
    r, m = x
    if inv:
        e = (16 - e) % 16
    e = e % 16
    h = float(np.sqrt(0.5))
    if e == 0:
        return x
    if e == 4:
        return (m, -r)
    if e == 12:
        return (-m, r)
    if e == 2:
        return ((r + m) * h, (m - r) * h)
    if e == 6:
        return ((m - r) * h, (r + m) * (-h))
    if e == 14:
        return ((r - m) * h, (r + m) * h)
    if e == 10:
        return ((r + m) * (-h), (r - m) * h)
    c = float(np.cos(2 * np.pi * e / 16))
    s = float(-np.sin(2 * np.pi * e / 16))
    return (r * c - m * s, r * s + m * c)


def _fft4(x, inv, pre=None):
    (ar, ai), (br, bi), (cr, ci), (dr, di) = x
    if pre is None:
        t0 = (ar + cr, ai + ci); t1 = (ar - cr, ai - ci)
    elif not inv:
        t0 = (ar + ci, ai - cr); t1 = (ar - ci, ai + cr)
    else:
        t0 = (ar - ci, ai + cr); t1 = (ar + ci, ai - cr)
    t2 = (br + dr, bi + di); t3 = (br - dr, bi - di)
    y0 = (t0[0] + t2[0], t0[1] + t2[1]); y2 = (t0[0] - t2[0], t0[1] - t2[1])
    ya = (t1[0] + t3[1], t1[1] - t3[0]); yb = (t1[0] - t3[1], t1[1] + t3[0])
    return [y0, yb, y2, ya] if inv else [y0, ya, y2, yb]


def _fft16(x, inv):
    if not inv:
        U = [_fft4([x[a + 4 * b] for b in range(4)], False) for a in range(4)]
        out = [None] * 16
        for kb in range(4):
            v = [U[a][kb] if (a * kb) % 16 == 4 else _cmul_const(U[a][kb], a * kb, False) for a in range(4)]
            y = _fft4(v, False, pre=(True if kb == 2 else None))
            for ka in range(4):
                out[4 * ka + kb] = y[ka]
        return out
    U = [_fft4([x[4 * ka + kb] for ka in range(4)], True) for kb in range(4)]
    out = [None] * 16
    for a in range(4):
        v = [U[kb][a] if (a * kb) % 16 == 4 else _cmul_const(U[kb][a], a * kb, True) for kb in range(4)]
        y = _fft4(v, True, pre=(True if a == 2 else None))
        for b in range(4):
            out[a + 4 * b] = y[b]
    return out


def _r5half(a0, p1, p2, m1, m2):
    q = p1 + p2
    r = (p1 - p2) * ((C1 - C2) / 2)
    b = a0 - q * 0.25
    return a0 + q, b + r, b - r, m1 * S1 + m2 * S2, m1 * S2 - m2 * S1


def _ln_stats(x):
    m = jnp.sum(x, axis=0, keepdims=True) * (1.0 / D)
    xc = x - m
    v = jnp.sum(xc * xc, axis=0, keepdims=True) * (1.0 / D)
    return xc, v


def _split(v):
    v = v.reshape(v.shape[0] // 16, 2, 8, v.shape[1])
    return v[:, 0], v[:, 1]


def _merge(r, i):
    return jnp.stack([r, i], axis=1).reshape(r.shape[0] * 16, r.shape[2])


def kernel(x_hbm, wr_hbm, wi_hbm, w1t_hbm, b1_hbm, w2_hbm, b2_hbm, g_hbm, gi_hbm, ms_hbm, mi_hbm, pm_hbm,
           o_hbm,
           xin, wr, wi, w1t, b1, w2, b2, g, gi, ms, mi, pm, wn, wp, xt, stage, p, q, hb, u, sems):
    copies = [(x_hbm, xin), (g_hbm, g), (ms_hbm, ms), (pm_hbm, pm), (mi_hbm, mi), (gi_hbm, gi),
              (b1_hbm, b1), (b2_hbm, b2), (w1t_hbm, w1t), (w2_hbm, w2), (wr_hbm, wr), (wi_hbm, wi)]
    cps = [pltpu.make_async_copy(a, b, sems.at[i]) for i, (a, b) in enumerate(copies)]
    for i in (3, 10, 11, 0, 1, 2, 4, 5, 6, 7, 8, 9):
        cps[i].start()
    cps[3].wait()
    for part, wsrc in enumerate((wr, wi)):
        cps[10 + part].wait()
        for t2 in range(8):
            o = [lax.dot_general(pm[0:128, :], wsrc[:, 128 * t:128 * (t + 1)], NT, preferred_element_type=f32)
                 for t in (2 * t2, 2 * t2 + 1)]
            for k in range(16):
                wn[k, 16 * t2:16 * (t2 + 1), :] = jnp.concatenate(
                    [o[0][8 * k:8 * (k + 1)], o[1][8 * k:8 * (k + 1)]], axis=0).astype(bf16)
        for k in range(16):
            cs = slice(128 * k, 128 * (k + 1))
            oa = lax.dot_general(pm[128:272, :], wn[k, :, 0:128], NT, preferred_element_type=f32)
            ob = lax.dot_general(pm[272:416, :], wn[k, :, 128:256], NT, preferred_element_type=f32)
            oc_ = lax.dot_general(pm[416:496, 0:65], wn[k, :, 256:321], NT, preferred_element_type=f32)
            blocks = [oa[0:64], ob[0:64], oc_[0:64],
                      jnp.concatenate([ob[64:72] + oc_[64:72], ob[72:128]], axis=0),
                      jnp.concatenate([oa[64:72] + ob[128:136], oa[72:128]], axis=0),
                      oa[128:136] + ob[136:144] + oc_[72:80]]
            allr = jnp.concatenate(blocks, axis=0)
            for gi_ in range(NG):
                wp[16 * gi_ + 8 * part:16 * gi_ + 8 * part + 8, cs] = allr[8 * gi_:8 * (gi_ + 1)]
    cps[0].wait()
    for t in range(16):
        stage[t % 2] = xin[128 * t:128 * (t + 1), :].T.astype(f32)
        for a in range(5):
            xt[128 * a:128 * (a + 1), 128 * t:128 * (t + 1)] = stage[t % 2, pl.ds(a, 128, stride=5), :]
    cps[1].wait()

    for layer in range(2):
        for t in range(16):
            cs = slice(128 * t, 128 * (t + 1))
            xc, v = _ln_stats(xt[:, cs])
            h = (xc * lax.rsqrt(v + EPS)).astype(bf16)
            V = [jnp.dot(g[a], h[128 * a:128 * (a + 1)], preferred_element_type=f32) for a in range(5)]
            sp = [_split(vv[:128]) for vv in V]
            ar = [s[0] for s in sp]; ai = [s[1] for s in sp]
            X0r, A1r, A2r, B1r, B2r = _r5half(ar[0], ar[1] + ar[4], ar[2] + ar[3], ar[1] - ar[4], ar[2] - ar[3])
            X0i, A1i, A2i, B1i, B2i = _r5half(ai[0], ai[1] + ai[4], ai[2] + ai[3], ai[1] - ai[4], ai[2] - ai[3])
            blocks = [(X0r, X0i), (A1r + B1i, A1i - B1r), (A2r + B2i, A2i - B2r), (B2i - A2r, A2i + B2r), (B1i - A1r, A1i + B1r)]
            for j in range(5):
                p[128 * j:128 * (j + 1), cs] = _merge(*blocks[j])
            p[640:656, cs] = ((V[0][128:] + V[1][128:]) + (V[2][128:] + V[3][128:])) + V[4][128:]
        for gidx in range(NG):
            r0 = 16 * gidx
            xs = [(p[r0:r0 + 8, 128 * s:128 * (s + 1)], p[r0 + 8:r0 + 16, 128 * s:128 * (s + 1)]) for s in range(16)]
            ys = _fft16(xs, False)
            for k in range(16):
                q[r0:r0 + 16, 128 * k:128 * (k + 1)] = jnp.concatenate(ys[k], axis=0).astype(bf16)
        if layer == 0:
            cps[2].wait(); cps[4].wait(); cps[5].wait()
        for k in range(16):
            cs = slice(128 * k, 128 * (k + 1))
            R = jnp.dot(q[:, cs], ms[k], preferred_element_type=f32)
            Rr, Ri = _split(R)
            Yr = Rr[:, :, :128] - Ri[:, :, 128:]
            Yi = Rr[:, :, 128:] + Ri[:, :, :128]
            Wr, Wi = _split(wp[:, cs])
            Z = _merge(Yr * Wr - Yi * Wi, Yr * Wi + Yi * Wr).astype(bf16)
            R = jnp.dot(Z, mi[k], preferred_element_type=f32)
            Rr, Ri = _split(R)
            p[:, cs] = _merge(Rr[:, :, :128] - Ri[:, :, 128:], Rr[:, :, 128:] + Ri[:, :, :128])
        for gidx in range(NG):
            r0 = 16 * gidx
            xs = [(p[r0:r0 + 8, 128 * s:128 * (s + 1)], p[r0 + 8:r0 + 16, 128 * s:128 * (s + 1)]) for s in range(16)]
            ys = _fft16(xs, True)
            for k in range(16):
                p[r0:r0 + 16, 128 * k:128 * (k + 1)] = jnp.concatenate(ys[k], axis=0)
        row = lax.broadcasted_iota(jnp.int32, (8, 128), 0)
        for t in range(16):
            cs = slice(128 * t, 128 * (t + 1))
            sp = [_split(p[128 * j:128 * (j + 1), cs]) for j in range(5)]
            Yr = [s[0] for s in sp]; Yi = [s[1] for s in sp]
            V0r, A1r, A2r, B1r, B2r = _r5half(Yr[0], Yr[1] - Yr[4], Yr[2] - Yr[3], Yr[1] + Yr[4], Yr[2] + Yr[3])
            V0i, A1i, A2i, B1i, B2i = _r5half(Yi[0], Yi[1] + Yi[4], Yi[2] + Yi[3], Yi[1] - Yi[4], Yi[2] - Yi[3])
            Vp = [(V0r, V0i), (A1r - B1i, A1i + B1r), (A2r - B2i, A2i + B2r), (A2r + B2i, A2i - B2r), (A1r + B1i, A1i - B1r)]
            e64r, e192r, e320r = p[640:641, cs], p[641:642, cs], p[642:643, cs]
            e64i, e192i = p[648:649, cs], p[649:650, cs]
            ys = []
            for a in range(5):
                th1, th3 = 2 * np.pi * a / 10, 2 * np.pi * 3 * a / 10
                Td = (e64r * float(2 * np.cos(th1)) - e64i * float(2 * np.sin(th1))
                      + e192r * float(2 * np.cos(th3)) - e192i * float(2 * np.sin(th3))
                      + e320r * float((-1) ** a))
                vr, vi = Vp[a]
                vi0 = jnp.where(row == 0, jnp.broadcast_to(Td, (8, 128)), vi[0])
                vi = jnp.concatenate([vi0[None], vi[1:]], axis=0)
                vv = _merge(vr, vi).astype(bf16)
                ys.append(jnp.dot(gi[a], vv, preferred_element_type=f32))
            xn = xt[:, cs] + jnp.concatenate(ys, axis=0)
            xt[:, cs] = xn
            xc, v = _ln_stats(xn)
            r = lax.rsqrt(v + EPS)
            r2 = lax.rsqrt(v * r * r + EPS)
            hb[:, cs] = (xc * (r * r2)).astype(bf16)
        if layer == 0:
            cps[6].wait(); cps[7].wait(); cps[8].wait()
        for c0 in range(0, F, 256):
            c1 = min(F, c0 + 256)
            uu = lax.dot_general(hb[...], w1t[c0:c1, :], NT, preferred_element_type=f32)
            uu = jax.nn.gelu(uu + b1[:, c0:c1].astype(f32), approximate=True)
            u[:, c0:c1] = uu.astype(bf16)
        if layer == 0:
            cps[9].wait()
        for c0 in range(0, S, 256):
            y = jnp.dot(u[...], w2[:, c0:c0 + 256], preferred_element_type=f32)
            xt[:, c0:c0 + 256] = xt[:, c0:c0 + 256] + y + b2[:, c0:c0 + 256].astype(f32)

    for t in range(16):
        for a in range(5):
            stage[t % 2, pl.ds(a, 128, stride=5), :] = xt[128 * a:128 * (a + 1), 128 * t:128 * (t + 1)]
        xin[128 * t:128 * (t + 1), :] = stage[t % 2].astype(bf16).T
    oc = pltpu.make_async_copy(xin, o_hbm, sems.at[12])
    oc.start()
    oc.wait()


@jax.jit
def pallas_interleave_layers__spectral_gfnet__mixer_token_mlp__prompt_kernel(A_x, A_w_r, A_w_i, B_x, B_w1, B_b1, B_w2, B_b2):
    G, GI, MS, MI, PM = _consts()
    args = (A_x.reshape(S, D), A_w_r.T, A_w_i.T, B_w1.T, B_b1.reshape(1, F), B_w2, B_b2.reshape(1, S),
            jnp.asarray(G, bf16), jnp.asarray(GI, bf16), jnp.asarray(MS, bf16), jnp.asarray(MI, bf16), jnp.asarray(PM, bf16))
    out = pl.pallas_call(
        kernel,
        out_shape=jax.ShapeDtypeStruct((S, D), bf16),
        in_specs=[pl.BlockSpec(memory_space=pltpu.HBM)] * len(args),
        out_specs=pl.BlockSpec(memory_space=pltpu.HBM),
        scratch_shapes=[
            pltpu.VMEM((S, D), bf16), pltpu.VMEM((321, S), bf16), pltpu.VMEM((321, S), bf16), pltpu.VMEM((F, S), bf16), pltpu.VMEM((1, F), bf16),
            pltpu.VMEM((F, S), bf16), pltpu.VMEM((1, S), bf16),
            pltpu.VMEM((5, 144, 128), bf16), pltpu.VMEM((5, 128, 128), bf16),
            pltpu.VMEM((16, 128, 256), bf16), pltpu.VMEM((16, 128, 256), bf16), pltpu.VMEM((496, 128), bf16),
            pltpu.VMEM((16, 128, 321), bf16), pltpu.VMEM((PR, S), f32),
            pltpu.VMEM((D, S), f32), pltpu.VMEM((2, D, 128), f32), pltpu.VMEM((PR, S), f32),
            pltpu.VMEM((PR, S), bf16), pltpu.VMEM((D, S), bf16), pltpu.VMEM((D, F), bf16),
            pltpu.SemaphoreType.DMA((13,)),
        ],
        compiler_params=pltpu.CompilerParams(vmem_limit_bytes=100 * 1024 * 1024),
    )(*args)
    return out.reshape(1, S, D)
```

```python
import os, contextlib
import numpy as np
import jax
import jax.numpy as jnp
from jax import lax
import jax.experimental.pallas as pl
import jax.experimental.pallas.tpu as pltpu

S, D, F = 2048, 640, 1728
R = 328
EPS = 1e-5
f32, bf16, u32 = jnp.float32, jnp.bfloat16, jnp.uint32
NT = (((1,), (1,)), ((), ()))

C1, C2 = float(np.cos(2 * np.pi / 5)), float(np.cos(4 * np.pi / 5))
S1, S2 = float(np.sin(2 * np.pi / 5)), float(np.sin(4 * np.pi / 5))
SCOPES = os.environ.get("KSCOPES") == "1"
OPT = dict(kv.split('=') for kv in os.environ.get("KOPT", "").split(',') if kv)


def opt(k, d):
    return type(d)(OPT.get(k, d))


def scope(n):
    return jax.named_scope(n) if SCOPES else contextlib.nullcontext()


def _consts():
    G = np.zeros((5, 144, 128))
    GI = np.zeros((5, 128, 128))
    for a in range(5):
        d = a + 5 * np.arange(128)
        for l in range(64):
            G[a, l] = np.cos(2 * np.pi * d * l / 640)
            G[a, 64 + l] = -np.sin(2 * np.pi * d * l / 640)
            GI[a, :, 16 * (l // 8) + l % 8] = (1 if l == 0 else 2) * np.cos(2 * np.pi * d * l / 640)
            GI[a, :, 16 * (l // 8) + 8 + l % 8] = -2 * np.sin(2 * np.pi * d * l / 640)
        for i, f in enumerate((64, 192, 320)):
            G[a, 128 + i] = np.cos(2 * np.pi * d * f / 640)
            G[a, 136 + i] = -np.sin(2 * np.pi * d * f / 640)
        GI[a, :, 8] = (-1.0) ** np.arange(128)
    GI = GI / (640 * 2048)
    s2 = np.arange(128)
    ang = [2 * np.pi * ((np.outer(s2, k1 + 16 * np.arange(128))) % 2048) / 2048 for k1 in range(16)]
    MS = np.stack([np.stack([np.cos(a), -np.sin(a) - np.cos(a), np.cos(a) - np.sin(a)]) for a in ang])
    MS = MS.reshape(4, 4, 3, 128, 128).transpose(1, 0, 2, 3, 4).reshape(16, 3, 128, 128)
    P128 = np.zeros((128, 128))
    for k1 in range(16):
        for j in range(8):
            P128[8 * k1 + j, k1 + 16 * j] = 1.0
    PA = np.zeros((144, 128)); PB = np.zeros((144, 128)); PC = np.zeros((80, 128))
    for l in range(64):
        PA[l, l] = 1.0; PB[l, l] = 1.0; PC[l, l] = 1.0
        if l > 0:
            PA[64 + l, 128 - l] = 1.0
            PB[64 + l, 128 - l] = 1.0
    PA[128, 64] = 1.0
    PB[128, 0] = 1.0
    PB[136 + 1, 64] = 1.0
    PC[64, 0] = 1.0
    PC[72 + 2, 64] = 1.0
    PM = np.concatenate([P128, PA, PB, PC], 0)
    return G, GI, MS, PM


def _tw16(x, e):
    r, m = x
    e = e % 16
    h = float(np.sqrt(0.5))
    if e == 0:
        return x
    if e == 4:
        return (m, -r)
    if e == 12:
        return (-m, r)
    if e == 2:
        return ((r + m) * h, (m - r) * h)
    if e == 6:
        return ((m - r) * h, (r + m) * (-h))
    if e == 14:
        return ((r - m) * h, (r + m) * h)
    if e == 10:
        return ((r + m) * (-h), (r - m) * h)
    c = float(np.cos(2 * np.pi * e / 16))
    s = float(-np.sin(2 * np.pi * e / 16))
    return (r * c - m * s, r * s + m * c)


def _half4(x, odd, inv):
    (ar, ai), (br, bi), (cr, ci), (dr, di) = x
    if not odd:
        t0 = (ar + cr, ai + ci); t2 = (br + dr, bi + di)
        return [(t0[0] + t2[0], t0[1] + t2[1]), (t0[0] - t2[0], t0[1] - t2[1])]
    t1 = (ar - cr, ai - ci); t3 = (br - dr, bi - di)
    ya = (t1[0] + t3[1], t1[1] - t3[0]); yb = (t1[0] - t3[1], t1[1] + t3[0])
    return [yb, ya] if inv else [ya, yb]


def _fft4(x, inv):
    e = _half4(x, 0, inv); o = _half4(x, 1, inv)
    return [e[0], o[0], e[1], o[1]]


def _r5half(a0, p1, p2, m1, m2):
    q = p1 + p2
    r = (p1 - p2) * ((C1 - C2) / 2)
    b = a0 - q * 0.25
    return a0 + q, b + r, b - r, m1 * S1 + m2 * S2, m1 * S2 - m2 * S1


def tl(t):
    return slice(128 * t, 128 * (t + 1))


def _fold8(x):
    parts = [x[8 * i:8 * (i + 1)] for i in range(x.shape[0] // 8)]
    while len(parts) > 1:
        parts = [parts[i] + parts[i + 1] if i + 1 < len(parts) else parts[i] for i in range(0, len(parts), 2)]
    return parts[0]


def _pk(x):
    return pltpu.bitcast(x.astype(bf16), u32)


def _upk(x):
    return pltpu.bitcast(x, bf16)


NAMES = {}


def put(ref, idx, val):
    if NAMES.get(id(ref), '?') in opt('anc', 'none').split('.'):
        mask = lax.broadcasted_iota(jnp.int32, val.shape, 1) < 4096
        pltpu.store(ref.at[idx], val, mask=mask)
    else:
        ref[idx] = val


def chain(*gens):
    for g in gens:
        yield from g


def mix(a, b):
    live = True
    while live:
        live = False
        for g, n in ((a, 5), (b, 2)):
            for _ in range(n):
                if next(g, 'done') != 'done':
                    live = True
                    yield


def run_all(gen):
    for _ in gen:
        pass


def weave(main, side, ratio):
    credit = 0.0
    for _ in main:
        credit += ratio
        while credit >= 1.0:
            next(side, None)
            credit -= 1.0


def kernel(x_hbm, wr_hbm, wi_hbm, w1t_hbm, b1_hbm, w2_hbm, b2_hbm, g_hbm, gi_hbm, ms_hbm, pm_hbm,
           o_hbm,
           xin, wr, wi, w1t, b1v, w2, b2v, g, gi, ms, pm, wn, wpr, wpi, xt, stage, pr, pi, hb, u, acc, vv, vf,
           cs, b1, b2, sems, rsem):
    groups = {}

    def dma(name, pairs):
        i = len(groups)
        groups[name] = [pltpu.make_async_copy(a_, b_, sems.at[i]) for a_, b_ in pairs]

    def xg(a):
        return [(x_hbm.at[tl(a + 4 * b)], xin.at[tl(a + 4 * b)]) for b in range(4)]
    dma('wr', [(pm_hbm, pm), (wr_hbm, wr)])
    dma('x0', [(g_hbm, g)] + xg(0))
    dma('x1', xg(1))
    dma('wi', [(wi_hbm, wi)])
    dma('x2', xg(2))
    dma('x3', xg(3))
    dma('ms', [(ms_hbm, ms)])
    dma('w1a', [(gi_hbm, gi), (b1_hbm, b1v), (b2_hbm, b2v)]
        + [(w1t_hbm.at[:, tl(4 * b)], w1t.at[:, tl(4 * b)]) for b in range(4)])
    dma('w1b', [(w1t_hbm.at[:, 512 * b + 128:512 * (b + 1)], w1t.at[:, 512 * b + 128:512 * (b + 1)]) for b in range(4)])
    dma('w2', [(w2_hbm, w2)])
    for cl in groups.values():
        for c in cl:
            c.start()
    cps = [c for cl in groups.values() for c in cl]

    def wait(name):
        for c in groups[name]:
            c.wait()
    nat = set(range(16))

    def xread(c, t):
        return stage[t, pl.ds(c, 128, stride=5), :] if t in nat else xt[tl(c), tl(t)]
    NAMES.update({id(v): k for k, v in dict(xt=xt, pr=pr, pi=pi, hb=hb, u=u, acc=acc, vv=vv, vf=vf, cs=cs, wpr=wpr, wpi=wpi).items()})
    csum = {}

    def wprep(wsrc, wdst):
        for t2 in range(8):
            o = [lax.dot_general(pm[0:128, :], wsrc[:, tl(t)], NT, preferred_element_type=f32)
                 for t in (2 * t2, 2 * t2 + 1)]
            for k in range(16):
                wn[k, 8 * t2:8 * (t2 + 1), :] = _pk(jnp.concatenate(
                    [o[0][8 * k:8 * (k + 1)], o[1][8 * k:8 * (k + 1)]], axis=0))
            yield
        for k in range(16):
            oa = lax.dot_general(pm[128:272, :], _upk(wn[k, :, 0:128]), NT, preferred_element_type=f32)
            ob = lax.dot_general(pm[272:416, :], _upk(wn[k, :, 128:256]), NT, preferred_element_type=f32)
            oc_ = lax.dot_general(pm[416:496, 0:65], _upk(wn[k, :, 256:321]), NT, preferred_element_type=f32)
            blocks = [oa[0:64], ob[0:64], oc_[0:64], ob[64:72] + oc_[64:72], ob[72:128],
                      oa[64:72] + ob[128:136], oa[72:128], oa[128:136] + ob[136:144] + oc_[72:80]]
            put(wdst, (slice(None), tl(k)), jnp.concatenate(blocks, axis=0))
            yield

    def addsum(t, x):
        n = csum.get(t) or 0
        put(cs, (slice(16 * n, 16 * n + 16), tl(t)), jnp.concatenate([_fold8(x), _fold8(x * x)], axis=0))
        csum[t] = n + 1

    def xload(t):
        x = xin[tl(t), :].T.astype(f32)
        stage[t] = x
        csum[t] = None
        addsum(t, x)

    def lng(t, dst, col, double):
        n = csum.pop(t)
        sq = cs[0:16, tl(t)]
        for i in range(1, n):
            sq = sq + cs[16 * i:16 * i + 16, tl(t)]
        s, q = sq[0:8], sq[8:16]
        m = jnp.sum(s, axis=0, keepdims=True) * (1.0 / D)
        v = jnp.maximum(jnp.sum(q, axis=0, keepdims=True) * (1.0 / D) - m * m, 0.0)
        r = lax.rsqrt(v + EPS)
        if double:
            r = r * lax.rsqrt(v * r * r + EPS)
        mr = m * r
        for c in range(5):
            put(dst, (slice(64 * c, 64 * (c + 1)), col), _pk(xread(c, t) * r - mr))
            yield

    def p1ln(a):
        for b in range(4):
            yield from lng(a + 4 * b, vv, tl(4 * a + b), False)

    def p1dot(a):
        for c in range(5):
            put(vf, (slice(144 * c, 144 * (c + 1)), slice(512 * a, 512 * (a + 1))), jnp.dot(
                g[c], _upk(vv[64 * c:64 * (c + 1), 512 * a:512 * (a + 1)]), preferred_element_type=f32))
            yield

    def p1post(a):
        def ld(c, r0, b):
            return vf[144 * c + r0:144 * c + r0 + 8, tl(4 * a + b)]
        for gq in range(9):
            for odd in range(2):
                if gq < 8:
                    Y = [_half4([(ld(c, 8 * gq, b), ld(c, 64 + 8 * gq, b)) for b in range(4)], odd, False)
                         for c in range(5)]
                else:
                    E = [tuple(((ld(0, r0, b) + ld(1, r0, b)) + (ld(2, r0, b) + ld(3, r0, b))) + ld(4, r0, b)
                               for r0 in (128, 136)) for b in range(4)]
                    Y = [_half4(E, odd, False)]
                for hi in range(2):
                    kb = odd + 2 * hi
                    if gq < 8:
                        ar = [Y[c][hi][0] for c in range(5)]; ai = [Y[c][hi][1] for c in range(5)]
                        X0r, A1r, A2r, B1r, B2r = _r5half(ar[0], ar[1] + ar[4], ar[2] + ar[3], ar[1] - ar[4], ar[2] - ar[3])
                        X0i, A1i, A2i, B1i, B2i = _r5half(ai[0], ai[1] + ai[4], ai[2] + ai[3], ai[1] - ai[4], ai[2] - ai[3])
                        X = [(X0r, X0i), (A1r + B1i, A1i - B1r), (A2r + B2i, A2i - B2r), (B2i - A2r, A2i + B2r), (B1i - A1r, A1i + B1r)]
                    else:
                        X = [Y[0][hi]]
                    for j in range(len(X)):
                        r0 = 64 * j + 8 * gq if gq < 8 else 320
                        kq = kb if j < 3 else (4 - kb) % 4
                        yr, yi = _tw16(X[j], a * kq)
                        put(pr, (slice(r0, r0 + 8), tl(4 * kq + a)), yr)
                        put(pi, (slice(r0, r0 + 8), tl(4 * kq + a)), yi)
                yield

    def phase1g(a):
        return chain(p1ln(a), p1dot(a), p1post(a))

    NRB = opt('nrb', 3)
    edges = [16 * round(21 * i / NRB) for i in range(NRB)] + [R]
    RBS = list(zip(edges[:-1], edges[1:]))
    units = [(kb, rb) for kb in range(4) for rb in range(NRB)]

    def pack3(xr, xi):
        return (xr + xi).astype(bf16), xr.astype(bf16), xi.astype(bf16)

    def chunks(rb):
        return [(r0, min(RBS[rb][1], r0 + 16)) for r0 in range(RBS[rb][0], RBS[rb][1], 16)]

    def s1(un, st):
        kb, rb = un
        L = [[] for _ in range(4)]
        st['L'] = L
        for r0, r1 in chunks(rb):
            T = _fft4([(pr[r0:r1, tl(4 * kb + a)], pi[r0:r1, tl(4 * kb + a)]) for a in range(4)], False)
            for ka in range(4):
                L[ka].append(pack3(*T[ka]))
            yield

    def dots3(L, m3):
        return [jnp.dot(jnp.concatenate([c[i] for c in L], axis=0), m3[i], preferred_element_type=f32) for i in range(3)]

    def s23(un, st):
        kb, rb = un
        base = RBS[rb][0]
        Z = []
        st['Z'] = Z
        K = {}

        def filt(ka):
            k = 4 * ka + kb
            k1, k2, k3 = K[ka]
            zl = []
            for r0, r1 in chunks(rb):
                q = slice(r0 - base, r1 - base)
                yr, yi = k1[q] - k3[q], k1[q] + k2[q]
                wr_, wi_ = wpr[r0:r1, tl(k)], wpi[r0:r1, tl(k)]
                zl.append(pack3(yr * wr_ - yi * wi_, yr * wi_ + yi * wr_))
            Z.append(zl)
        for ka in range(4):
            K[ka] = dots3(st['L'][ka], ms.at[4 * kb + ka])
            if ka > 0:
                filt(ka - 1)
            yield
        filt(3)

    def s4(un, st):
        kb, rb = un
        K = []
        st['K'] = K
        for ka in range(4):
            m3 = ms.at[4 * kb + ka]
            k1, k2, k3 = [lax.dot_general(jnp.concatenate([c[i] for c in st['Z'][ka]], axis=0), m3[(0, 2, 1)[i]], NT,
                                          preferred_element_type=f32) for i in range(3)]
            K.append((k1 + k3, k1 - k2))
            yield

    def s5(un, st):
        kb, rb = un
        base = RBS[rb][0]
        for r0, r1 in chunks(rb):
            q = slice(r0 - base, r1 - base)
            us = _fft4([(kr[q], ki[q]) for kr, ki in st['K']], True)
            for a in range(4):
                yr, yi = _tw16(us[a], -a * kb)
                put(pr, (slice(r0, r1), tl(4 * kb + a)), yr)
                put(pi, (slice(r0, r1), tl(4 * kb + a)), yi)
            yield

    def p2():
        n = len(units)
        st = [dict() for _ in range(n)]
        run_all(s1(units[0], st[0]))
        for i in range(n + 1):
            if i < n:
                side = s1(units[i + 1], st[i + 1]) if i + 1 < n else iter(())
                weave(s23(units[i], st[i]), side, 2)
                run_all(side)
            if i >= 1:
                side = s5(units[i - 2], st[i - 2]) if i >= 2 else iter(())
                weave(s4(units[i - 1], st[i - 1]), side, 2)
                run_all(side)
        run_all(s5(units[n - 1], st[n - 1]))

    def p3pre(a):
        row = lax.broadcasted_iota(jnp.int32, (8, 128), 0)
        E = _fft4([(pr[320:328, tl(4 * kb + a)], pi[320:328, tl(4 * kb + a)]) for kb in range(4)], True)
        for gq in range(8):
            for odd in range(2):
                Y = []
                for j in range(5):
                    rs = slice(64 * j + 8 * gq, 64 * j + 8 * gq + 8)
                    Y.append(_half4([(pr[rs, tl(4 * kb + a)], pi[rs, tl(4 * kb + a)]) for kb in range(4)], odd, True))
                for hi in range(2):
                    b = odd + 2 * hi
                    Yr = [Y[j][hi][0] for j in range(5)]; Yi = [Y[j][hi][1] for j in range(5)]
                    V0r, A1r, A2r, B1r, B2r = _r5half(Yr[0], Yr[1] - Yr[4], Yr[2] - Yr[3], Yr[1] + Yr[4], Yr[2] + Yr[3])
                    V0i, A1i, A2i, B1i, B2i = _r5half(Yi[0], Yi[1] + Yi[4], Yi[2] + Yi[3], Yi[1] - Yi[4], Yi[2] - Yi[3])
                    Vp = [(V0r, V0i), (A1r - B1i, A1i + B1r), (A2r - B2i, A2i + B2r), (A2r + B2i, A2i - B2r), (A1r + B1i, A1i - B1r)]
                    for c in range(5):
                        vr, vi = Vp[c]
                        if gq == 0:
                            er, ei = E[b]
                            th1, th3 = 2 * np.pi * c / 10, 2 * np.pi * 3 * c / 10
                            Td = (er[0:1] * float(2 * np.cos(th1)) - ei[0:1] * float(2 * np.sin(th1))
                                  + er[1:2] * float(2 * np.cos(th3)) - ei[1:2] * float(2 * np.sin(th3))
                                  + er[2:3] * float((-1) ** c))
                            vi = jnp.where(row == 0, jnp.broadcast_to(Td, (8, 128)), vi)
                        put(vv, (slice(64 * c + 8 * gq, 64 * c + 8 * gq + 8), tl(4 * a + b)), _pk(jnp.concatenate([vr, vi], axis=0)))
                yield

    def p3dot(a):
        for b in range(4):
            csum[a + 4 * b] = None
        for c in range(5):
            y = jnp.dot(gi[c], _upk(vv[64 * c:64 * (c + 1), 512 * a:512 * (a + 1)]), preferred_element_type=f32)
            for b in range(4):
                xn = xread(c, a + 4 * b) + y[:, tl(b)]
                put(xt, (tl(c), tl(a + 4 * b)), xn)
                addsum(a + 4 * b, xn)
            if c == 4:
                nat.difference_update(a + 4 * b for b in range(4))
            yield

    def p3post(a):
        for b in range(4):
            yield from lng(a + 4 * b, hb, tl(4 * a + b), True)

    def phase3g(a):
        return chain(p3pre(a), p3dot(a), p3post(a))

    def cat(ref, rows, tiles):
        return jnp.concatenate([ref[rows, tl(t)] for t in tiles], axis=1)

    def piped(pieces):
        ops = pieces[0][0]()
        prev = None
        for i, (_, compute, finish) in enumerate(pieces):
            y = compute(ops)
            if prev is not None:
                prev[0](prev[1])
            prev = (finish, y)
            if i + 1 < len(pieces):
                ops = pieces[i + 1][0]()
            yield
        prev[0](prev[1])

    def mm1a_fine():
        pieces = []
        for c0 in range(0, F, 128):
            c1 = min(F, c0 + 128)
            for r0 in range(0, D, 128):
                pieces.append((
                    lambda c0=c0, c1=c1, r0=r0: (hb[r0 // 2:r0 // 2 + 64, 0:512], cat(w1t, slice(c0, c1), [0, 4, 8, 12])),
                    lambda o: lax.dot_general(_upk(o[0]), o[1], NT, preferred_element_type=f32),
                    lambda y, c0=c0, c1=c1, r0=r0: put(acc, (slice(r0, r0 + 128), slice(c0, c1)), y)))
        return piped(pieces)

    def mm1b(c0, c1):
        tiles = [a + 4 * b for a in range(1, 4) for b in range(4)]
        uu = lax.dot_general(_upk(hb[:, 512:]), cat(w1t, slice(c0, c1), tiles), NT,
                             preferred_element_type=f32) + acc[:, c0:c1]
        uu = jax.nn.gelu(uu + b1[0:1, c0:c1], approximate=True)
        put(u, (slice(None), slice(c0, c1)), _pk(uu))

    def mm2_epi(r0, r1, t, y):
        xn = xt[r0:r1, tl(t)] + y + b2[0:1, tl(t)]
        put(xt, (slice(r0, r1), tl(t)), xn)
        addsum(t, xn)

    def mm2(tiles):
        y = jnp.dot(_upk(u[...]), cat(w2, slice(None), tiles), preferred_element_type=f32)
        for i, t in enumerate(tiles):
            csum[t] = None
            mm2_epi(0, D, t, y[:, tl(i)])

    def mm2_fine(*pairs):
        pieces = []
        carry = {}

        def start(tiles):
            for t in tiles:
                csum[t] = None
        for tiles in pairs:
            for r0 in range(0, D, 128):
                rs = slice(r0 // 2, r0 // 2 + 64)

                def crem(o, tiles=tiles, r0=r0):
                    if r0 == 0:
                        start(tiles)
                    carry['rem'] = jnp.dot(_upk(o[0]), o[1], preferred_element_type=f32)
                pieces.append((lambda rs=rs, tiles=tiles: (u[rs, 1536:F], cat(w2, slice(1536, F), tiles)), crem, lambda y: None))
                for i, t in enumerate(tiles):
                    for k0 in range(0, 1536, 512):
                        def comp(o, i=i, k0=k0):
                            base = carry['rem'][:, tl(i)] if k0 == 0 else carry['y']
                            carry['y'] = base + jnp.dot(_upk(o[0]), o[1], preferred_element_type=f32)
                            return carry['y']
                        fin = (lambda y, r0=r0, t=t: mm2_epi(r0, r0 + 128, t, y)) if k0 == 1024 else (lambda y: None)
                        pieces.append((lambda rs=rs, k0=k0, t=t: (u[rs, k0:k0 + 512], w2[k0:k0 + 512, tl(t)]), comp, fin))
        return piped(pieces)

    def mm2_out(tiles):
        y = jnp.dot(_upk(u[...]), cat(w2, slice(None), tiles), preferred_element_type=f32)
        for i, t in enumerate(tiles):
            xn = xt[:, tl(t)] + y[:, tl(i)] + b2[0:1, tl(t)]
            for c in range(5):
                stage[t, pl.ds(c, 128, stride=5), :] = xn[tl(c)]

    def xstore(t):
        xin[tl(t), :] = stage[t].astype(bf16).T

    def bar():
        pl.semaphore_signal(rsem, 1)
        pl.semaphore_wait(rsem, 1)

    def take(gen, n):
        for _ in range(n):
            next(gen)
            yield

    def region(main, side, ratio, end=None):
        weave(main, side, ratio)
        run_all(side)
        if end is None:
            bar()
        else:
            wait(end)

    def p3mm1(first=False):
        mm = mm1a_fine()
        n1 = opt('n1', 28)
        region(p3pre(0), iter(()), 0, 'w1a' if first else None)
        if first:
            b1[...] = jnp.broadcast_to(b1v[...].astype(f32).reshape(1, F), (8, F))
            b2[...] = jnp.broadcast_to(b2v[...].astype(f32).reshape(1, S), (8, S))
        run_all(p3dot(0))
        if opt('b0', 0):
            bar()
        run_all(p3post(0))
        region(take(mm, n1), chain(p3pre(1), p3pre(2), p3pre(3)), 48 / (n1 - 2))
        region(chain(p3dot(1), p3dot(2), p3dot(3), take(mm, opt('n2', 2))), iter(()), 0)
        region(mm, chain(p3post(1), p3post(2), p3post(3)), opt('r3', 2.0), 'w1b' if first else None)
        for c0 in range(0, F, 256):
            mm1b(c0, min(F, c0 + 256))

    def mm2p1():
        mm = mm2_fine([10, 14], [3, 7], [11, 15])
        lnq = []
        for i, pair in enumerate(([0, 4], [8, 12], [1, 5], [9, 13], [2, 6])):
            mm2(pair)
            for t in lnq:
                run_all(lng(t, vv, tl(4 * (t % 4) + t // 4), False))
            lnq = pair
        side = chain(*[lng(t, vv, tl(4 * (t % 4) + t // 4), False) for t in lnq])
        weave(take(mm, 36), side, 0.5)
        run_all(side)
        nx = opt('nx', 6)
        region(take(mm, nx), chain(lng(10, vv, tl(10), False), lng(14, vv, tl(11), False)), 10 / nx)
        region(chain(p1dot(0), p1dot(1), p1dot(2)), iter(()), 0)
        side = chain(p1post(0), p1post(1), lng(3, vv, tl(12), False), lng(7, vv, tl(13), False), p1post(2))
        weave(mm, side, opt('r1', 1.05))
        run_all(side)
        if opt('b1', 1):
            bar()
        run_all(chain(lng(11, vv, tl(14), False), lng(15, vv, tl(15), False), p1dot(3)))
        bar()
        region(p1post(3), iter(()), 0)

    ocs = [pltpu.make_async_copy(xin.at[256 * i:256 * (i + 1)], o_hbm.at[256 * i:256 * (i + 1)], sems.at[12 + i]) for i in range(8)]

    def xa(a):
        for b in range(4):
            xload(a + 4 * b)
            yield
        yield from p1ln(a)
        yield from p1dot(a)
    none = iter(())
    with scope("wait0"):
        wait('wr')
    wp = wprep(wr, wpr)
    with scope("s1"):
        region(take(wp, opt('w1', 10)), none, 0, 'x0')
    with scope("s2"):
        region(wp, xa(0), 2.1, 'x1')
    with scope("s3"):
        region(xa(1), p1post(0), 0.62, 'wi')
    wp = wprep(wi, wpi)
    with scope("s4"):
        region(take(wp, opt('w2', 10)), p1post(1), 1.8, 'x2')
    with scope("s5"):
        region(wp, xa(2), 2.1, 'x3')
    with scope("s6"):
        region(xa(3), p1post(2), 0.62)
    with scope("s7"):
        region(p1post(3), none, 0, 'ms')
    for layer in range(2):
        with scope("p2"):
            p2()
        with scope("p3_mm1"):
            p3mm1(layer == 0)
        if layer == 0:
            with scope("waitw2"):
                wait('w2')
        with scope("mm2"):
            if layer == 0:
                mm2p1()
            else:
                flush = [int(v) for v in opt('fl', '3.6.7').split('.')]
                done = 0
                for c in range(8):
                    mm2_out([2 * c, 2 * c + 1])
                    if c in flush:
                        for i in range(done, c):
                            xstore(2 * i); xstore(2 * i + 1)
                            ocs[i].start()
                        done = c
                        if c < 7:
                            bar()
                for i in range(done, 8):
                    xstore(2 * i); xstore(2 * i + 1)
                    ocs[i].start()
    with scope("outdma"):
        for c in ocs:
            c.wait()


@jax.jit
def pallas_interleave_layers__spectral_gfnet__mixer_token_mlp__prompt_kernel(A_x, A_w_r, A_w_i, B_x, B_w1, B_b1, B_w2, B_b2):
    G, GI, MS, PM = _consts()
    args = (A_x.reshape(S, D), A_w_r.T, A_w_i.T, B_w1.T, B_b1, B_w2, B_b2,
            jnp.asarray(G, bf16), jnp.asarray(GI, bf16), jnp.asarray(MS, bf16), jnp.asarray(PM, bf16))
    out = pl.pallas_call(
        kernel,
        out_shape=jax.ShapeDtypeStruct((S, D), bf16),
        in_specs=[pl.BlockSpec(memory_space=pltpu.HBM)] * len(args),
        out_specs=pl.BlockSpec(memory_space=pltpu.HBM),
        scratch_shapes=[
            pltpu.VMEM((S, D), bf16), pltpu.VMEM((321, S), bf16), pltpu.VMEM((321, S), bf16),
            pltpu.VMEM((F, S), bf16), pltpu.VMEM((F,), bf16),
            pltpu.VMEM((F, S), bf16), pltpu.VMEM((S,), bf16),
            pltpu.VMEM((5, 144, 128), bf16), pltpu.VMEM((5, 128, 128), bf16),
            pltpu.VMEM((16, 3, 128, 128), bf16), pltpu.VMEM((496, 128), bf16),
            pltpu.VMEM((16, 64, 321), u32), pltpu.VMEM((R, S), f32), pltpu.VMEM((R, S), f32),
            pltpu.VMEM((D, S), f32), pltpu.VMEM((16, D, 128), f32), pltpu.VMEM((R, S), f32), pltpu.VMEM((R, S), f32),
            pltpu.VMEM((D // 2, S), u32), pltpu.VMEM((D // 2, F), u32), pltpu.VMEM((D, F), f32),
            pltpu.VMEM((D // 2, S), u32), pltpu.VMEM((720, S), f32),
            pltpu.VMEM((80, S), f32), pltpu.VMEM((8, F), f32), pltpu.VMEM((8, S), f32), pltpu.SemaphoreType.DMA((40,)), pltpu.SemaphoreType.REGULAR,
        ],
        compiler_params=pltpu.CompilerParams(vmem_limit_bytes=100 * 1024 * 1024),
    )(*args)
    return out.reshape(1, S, D)
```

```python
import os, contextlib
import numpy as np
import jax
import jax.numpy as jnp
from jax import lax
import jax.experimental.pallas as pl
import jax.experimental.pallas.tpu as pltpu

S, D, F = 2048, 640, 1728
FM = 1664
R = 328
EPS = 1e-5
f32, bf16, u32 = jnp.float32, jnp.bfloat16, jnp.uint32
NT = (((1,), (1,)), ((), ()))

C1, C2 = float(np.cos(2 * np.pi / 5)), float(np.cos(4 * np.pi / 5))
S1, S2 = float(np.sin(2 * np.pi / 5)), float(np.sin(4 * np.pi / 5))
SCOPES = os.environ.get("KSCOPES") == "1"
OPT = dict(kv.split('=') for kv in os.environ.get("KOPT", "").split(',') if kv)


def opt(k, d):
    return type(d)(OPT.get(k, d))


def scope(n):
    return jax.named_scope(n) if SCOPES else contextlib.nullcontext()


def _shuffle(rows):
    rows = np.asarray(rows).reshape(-1, 2, 8)
    return rows.transpose(0, 2, 1).reshape(-1)


EXTRA = {0: 64, 4: 192, 1: 320}


def _consts():
    G = np.zeros((5, 144, 128))
    GI = np.zeros((5, 128, 128))
    lpos = _shuffle(_shuffle(np.arange(64)))
    for a in range(5):
        d = a + 5 * np.arange(128)
        for l in range(64):
            G[a, l] = np.cos(2 * np.pi * d * l / 640)
            G[a, 64 + l] = -np.sin(2 * np.pi * d * l / 640)
        for p in range(64):
            l = lpos[p]
            GI[a, :, 2 * p] = (1 if l == 0 else 2) * np.cos(2 * np.pi * d * l / 640)
            GI[a, :, 2 * p + 1] = -2 * np.sin(2 * np.pi * d * l / 640)
        for i, f in EXTRA.items():
            G[a, 128 + i] = np.cos(2 * np.pi * d * f / 640)
            G[a, 136 + i] = -np.sin(2 * np.pi * d * f / 640)
        GI[a, :, 1] = (-1.0) ** np.arange(128)
    GI = GI / (640 * 2048)
    s2 = np.arange(128)
    k2 = _shuffle(np.arange(128))
    ang = [2 * np.pi * ((np.outer(s2, k1 + 16 * k2)) % 2048) / 2048 for k1 in range(16)]
    MS = np.stack([np.stack([np.cos(a), -np.sin(a) - np.cos(a), np.cos(a) - np.sin(a)]) for a in ang])
    MS = MS.reshape(4, 4, 3, 128, 128).transpose(1, 0, 2, 3, 4).reshape(16, 3, 128, 128)
    P128 = np.zeros((128, 128))
    for k1 in range(16):
        for j in range(8):
            P128[8 * k1 + j, k1 + 16 * j] = 1.0
    l1 = _shuffle(np.arange(64))
    PA = np.zeros((144, 128)); PB = np.zeros((160, 128)); PC = np.zeros((96, 128))
    for p in range(64):
        l = l1[p]
        PA[p, l] = 1.0; PB[p, l] = 1.0; PC[p, l] = 1.0
        if l > 0:
            PA[64 + p, 128 - l] = 1.0
            PB[64 + p, 128 - l] = 1.0
    e1 = list(_shuffle(np.arange(16)))
    PA[128 + e1.index(0), 64] = 1.0
    PB[128, 0] = 1.0
    PB[144 + e1.index(4), 64] = 1.0
    PC[64, 0] = 1.0
    PC[80 + e1.index(1), 64] = 1.0
    PM = np.concatenate([P128, PA, PB, PC], 0)
    return G, GI, MS, PM


def _pack_rows(a):
    b = np.asarray(a, dtype=np.float32).astype(bf16).view(np.uint16).astype(np.uint32)
    return b[..., 0::2, :] | (b[..., 1::2, :] << 16)


def _tw16(x, e):
    r, m = x
    e = e % 16
    h = float(np.sqrt(0.5))
    if e == 0:
        return x
    if e == 4:
        return (m, -r)
    if e == 12:
        return (-m, r)
    if e == 2:
        return ((r + m) * h, (m - r) * h)
    if e == 6:
        return ((m - r) * h, (r + m) * (-h))
    if e == 14:
        return ((r - m) * h, (r + m) * h)
    if e == 10:
        return ((r + m) * (-h), (r - m) * h)
    c = float(np.cos(2 * np.pi * e / 16))
    s = float(-np.sin(2 * np.pi * e / 16))
    return (r * c - m * s, r * s + m * c)


def _half4(x, odd, inv):
    (ar, ai), (br, bi), (cr, ci), (dr, di) = x
    if not odd:
        t0 = (ar + cr, ai + ci); t2 = (br + dr, bi + di)
        return [(t0[0] + t2[0], t0[1] + t2[1]), (t0[0] - t2[0], t0[1] - t2[1])]
    t1 = (ar - cr, ai - ci); t3 = (br - dr, bi - di)
    ya = (t1[0] + t3[1], t1[1] - t3[0]); yb = (t1[0] - t3[1], t1[1] + t3[0])
    return [yb, ya] if inv else [ya, yb]


def _fft4(x, inv):
    e = _half4(x, 0, inv); o = _half4(x, 1, inv)
    return [e[0], o[0], e[1], o[1]]


def _r5half(a0, p1, p2, m1, m2):
    q = p1 + p2
    r = (p1 - p2) * ((C1 - C2) / 2)
    b = a0 - q * 0.25
    return a0 + q, b + r, b - r, m1 * S1 + m2 * S2, m1 * S2 - m2 * S1


def tl(t):
    return slice(128 * t, 128 * (t + 1))


def _fold8(x):
    parts = [x[8 * i:8 * (i + 1)] for i in range(x.shape[0] // 8)]
    while len(parts) > 1:
        parts = [parts[i] + parts[i + 1] if i + 1 < len(parts) else parts[i] for i in range(0, len(parts), 2)]
    return parts[0]


def _pk(x):
    return pltpu.bitcast(x.astype(bf16), u32)


def _ipk(a, b):
    return pltpu.pack_elementwise([a, b], packed_dtype=bf16).astype(u32)


def _upk(x):
    return pltpu.bitcast(x, bf16)


NAMES = {}


def put(ref, idx, val, force=False):
    if force or NAMES.get(id(ref), '?') in opt('anc', 'none').split('.'):
        mask = lax.broadcasted_iota(jnp.int32, val.shape, 1) < 4096
        pltpu.store(ref.at[idx], val, mask=mask)
    else:
        ref[idx] = val


def chain(*gens):
    for g in gens:
        yield from g


def mix(a, b):
    live = True
    while live:
        live = False
        for g, n in ((a, 5), (b, 2)):
            for _ in range(n):
                if next(g, 'done') != 'done':
                    live = True
                    yield


def run_all(gen):
    for _ in gen:
        pass


def woven(main, side, ratio):
    credit = 0.0
    for _ in main:
        credit += ratio
        while credit >= 1.0:
            next(side, None)
            credit -= 1.0
        yield
    yield from side


def woven_nodrain(main, side, ratio, credit=[0.0]):
    for _ in main:
        credit[0] += ratio
        while credit[0] >= 1.0:
            next(side, None)
            credit[0] -= 1.0
        yield


def weave(main, side, ratio):
    credit = 0.0
    for _ in main:
        credit += ratio
        while credit >= 1.0:
            next(side, None)
            credit -= 1.0


def kernel(x_hbm, wr_hbm, wi_hbm, w1t_hbm, b1_hbm, w2_hbm, b2_hbm, g_hbm, gi_hbm, ms_hbm, pm_hbm,
           o_hbm,
           xin, wr, wi, w1t, b1v, w2, b2v, g, gi, ms, pm, wn0, wn1, wpr, wpi, xt, stage, pr, pi, hb, u, acc, vv, vf,
           cs, b1, b2, b1c, zb, sems, rsem):
    groups = {}

    def dma(name, pairs):
        i = len(groups)
        groups[name] = [pltpu.make_async_copy(a_, b_, sems.at[i]) for a_, b_ in pairs]

    def xg(a):
        a = (a + 1) % 4
        return [(x_hbm.at[tl(a + 4 * b)], xin.at[tl(a + 4 * b)]) for b in range(4)]
    dma('wr', [(pm_hbm, pm), (wr_hbm.at[0:128], wr.at[0:128])])
    dma('wrb', [(wr_hbm.at[128:321], wr.at[128:321])])
    dma('x0', [(g_hbm, g)] + xg(0))
    dma('wi', [(wi_hbm.at[0:128], wi.at[0:128])])
    dma('x1', xg(1))
    dma('x2', xg(2))
    dma('wib', [(wi_hbm.at[128:321], wi.at[128:321])])
    dma('x3', xg(3))
    dma('ms0', [(ms_hbm.at[0:8], ms.at[0:8])])
    dma('ms1', [(ms_hbm.at[8:16], ms.at[8:16])])
    dma('w1a', [(gi_hbm, gi), (b1_hbm, b1v), (b2_hbm, b2v)]
        + [(w1t_hbm.at[:, tl(4 * b)], w1t.at[:, tl(4 * b)]) for b in range(4)])
    dma('w1b', [(w1t_hbm.at[:, 512 * b + 128:512 * (b + 1)], w1t.at[:, 512 * b + 128:512 * (b + 1)]) for b in range(4)])
    dma('w2', [(w2_hbm, w2)])
    for cl in groups.values():
        for c in cl:
            c.start()
    cps = [c for cl in groups.values() for c in cl]

    def wait(name):
        for c in groups[name]:
            c.wait()
    nat = set(range(16))

    def xread(c, t):
        return stage[t, pl.ds(c, 128, stride=5), :] if t in nat else xt[tl(c), tl(t)]
    NAMES.update({id(v): k for k, v in dict(xt=xt, pr=pr, pi=pi, hb=hb, u=u, acc=acc, vv=vv, vf=vf, cs=cs, wpr=wpr, wpi=wpi).items()})
    put(zb, (slice(None), slice(None)), jnp.zeros((8, 128), jnp.int32), True)
    tok = []

    def mark(y):
        tok.append(y[0:8, 0:128])

    def pinner(age):
        if len(tok) < age:
            return lambda v: v
        z = pltpu.bitcast(tok[-age], jnp.int32) & zb[...]
        return lambda v: pltpu.bitcast(pltpu.bitcast(v, jnp.int32) | z, f32)
    csum = {}

    def wstep1(wsrc, wn, f0, f1):
        for t2 in range(8):
            o = [lax.dot_general(_upk(pm[0:64, :]), wsrc[f0:f1, tl(t)], NT, preferred_element_type=f32)
                 for t in (2 * t2, 2 * t2 + 1)]
            pk = _ipk(o[0], o[1])
            for k in range(16):
                wn[k, 8 * t2:8 * (t2 + 1), f0:f1] = pk[8 * k:8 * (k + 1)]
            yield

    def wstep2a(wn, wdst):
        for k in range(16):
            oa = lax.dot_general(_upk(pm[64:136, :]), _upk(wn[k, :, 0:128]), NT, preferred_element_type=f32)
            wdst[0:64, tl(k)] = oa[0:64]
            wdst[256:336, tl(k)] = oa[64:144]
            yield

    def wstep2b(wn, wdst):
        for k in range(16):
            ob = lax.dot_general(_upk(pm[136:216, :]), _upk(wn[k, :, 128:256]), NT, preferred_element_type=f32)
            oc_ = lax.dot_general(_upk(pm[216:264, 0:65]), _upk(wn[k, :, 256:321]), NT, preferred_element_type=f32)
            wdst[64:264, tl(k)] = jnp.concatenate(
                [ob[0:64], oc_[0:64], ob[64:72] + oc_[64:72], ob[72:128], wdst[256:264, tl(k)] + ob[128:136]], axis=0)
            wdst[320:336, tl(k)] = wdst[320:336, tl(k)] + ob[144:160] + oc_[80:96]
            yield

    shift = {}

    def addsum(t, x):
        n = csum.get(t) or 0
        cs[16 * n:16 * n + 16, tl(t)] = jnp.concatenate([_fold8(x), _fold8(x * x)], axis=0)
        csum[t] = n + 1

    def shifted(t, x):
        if not csum.get(t):
            shift[t] = x[0:1]
        return x - shift[t]

    def xload(t):
        x = xin[tl(t), :].T.astype(f32)
        stage[t] = x
        csum[t] = None
        addsum(t, x)

    def stats(t, double):
        n = csum.pop(t)
        sq = cs[0:16, tl(t)]
        for i in range(1, n):
            sq = sq + cs[16 * i:16 * i + 16, tl(t)]
        s, q = sq[0:8], sq[8:16]
        m = jnp.sum(s, axis=0, keepdims=True) * (1.0 / D)
        v = jnp.maximum(jnp.sum(q, axis=0, keepdims=True) * (1.0 / D) - m * m, 0.0)
        if double:
            return m, lax.rsqrt(v + EPS * (v + EPS))
        return m, lax.rsqrt(v + EPS)

    def lng(t, dst, col):
        m, r = stats(t, True)
        m8 = jnp.broadcast_to(m + shift.pop(t), (8, 128))
        for c in range(5):
            mp = pinner(opt('age', 2))(m8)
            dst[64 * c:64 * (c + 1), col] = _pk((xread(c, t).reshape(16, 8, 128) - mp[None]).reshape(128, 128) * r)
            yield

    def vcol(t):
        return tl(4 * (t % 4) + t // 4)

    lnst = {}

    def p1cast(a):
        for b in range(4):
            m, r = stats(a + 4 * b, False)
            lnst[a + 4 * b] = (None, r)
            for c in range(5):
                vv[64 * c:64 * (c + 1), tl(4 * a + b)] = _pk(xread(c, a + 4 * b) - m)
            yield

    def p1dot(a):
        st_ = [lnst.pop(a + 4 * b) if a + 4 * b in lnst else stats(a + 4 * b, False) for b in range(4)]
        r = jnp.concatenate([s[1] for s in st_], axis=1)
        dc = None
        if st_[0][0] is not None:
            row = lax.broadcasted_iota(jnp.int32, (8, 512), 0)
            dc = jnp.where(row == 0, jnp.concatenate([s[0] for s in st_], axis=1) * 128.0, 0.0)
        for c in range(5):
            y = jnp.dot(_upk(g[c]), _upk(vv[64 * c:64 * (c + 1), 512 * a:512 * (a + 1)]), preferred_element_type=f32)
            if dc is not None:
                y = jnp.concatenate([y[0:8] - dc, y[8:]], axis=0)
            vf[144 * c:144 * (c + 1), 512 * a:512 * (a + 1)] = y * r
            yield

    def p1post(a):
        def ld(c, r0, b):
            return vf[144 * c + r0:144 * c + r0 + 8, tl(4 * a + b)]
        for gq in (0, 1, 8, 2, 3, 4, 5, 6, 7):
            for odd in range(2):
                if gq < 8:
                    pf = pinner(opt('age3', 3))
                    Y = [_half4([(pf(ld(c, 8 * gq, b)), pf(ld(c, 64 + 8 * gq, b))) if b < 2 else
                                 (ld(c, 8 * gq, b), ld(c, 64 + 8 * gq, b)) for b in range(4)], odd, False)
                         for c in range(5)]
                else:
                    E = [tuple(((ld(0, r0, b) + ld(1, r0, b)) + (ld(2, r0, b) + ld(3, r0, b))) + ld(4, r0, b)
                               for r0 in (128, 136)) for b in range(4)]
                    Y = [_half4(E, odd, False)]
                for hi in range(2):
                    kb = odd + 2 * hi
                    if gq < 8:
                        ar = [Y[c][hi][0] for c in range(5)]; ai = [Y[c][hi][1] for c in range(5)]
                        X0r, A1r, A2r, B1r, B2r = _r5half(ar[0], ar[1] + ar[4], ar[2] + ar[3], ar[1] - ar[4], ar[2] - ar[3])
                        X0i, A1i, A2i, B1i, B2i = _r5half(ai[0], ai[1] + ai[4], ai[2] + ai[3], ai[1] - ai[4], ai[2] - ai[3])
                        X = [(X0r, X0i), (A1r + B1i, A1i - B1r), (A2r + B2i, A2i - B2r), (B2i - A2r, A2i + B2r), (B1i - A1r, A1i + B1r)]
                    else:
                        X = [Y[0][hi]]
                    for j in range(len(X)):
                        r0 = 64 * j + 8 * gq if gq < 8 else 320
                        kq = kb if j < 3 else (4 - kb) % 4
                        yr, yi = _tw16(X[j], a * kq)
                        put(pr, (slice(r0, r0 + 8), tl(4 * kq + a)), yr)
                        put(pi, (slice(r0, r0 + 8), tl(4 * kq + a)), yi)
                yield

    def phase1g(a):
        return chain(p1cast(a), p1dot(a), p1post(a))

    NRB = opt('nrb', 5)
    ALLCH = [(r0, min(R, r0 + 16)) for r0 in range(0, R, 16)]
    edges = [round(21 * i / NRB) for i in range(NRB + 1)]
    CONT = [ALLCH[e0:e1] for e0, e1 in zip(edges[:-1], edges[1:])]
    BYQ = [[ALLCH[4 * j + q] for j in range(5)] + ([ALLCH[20]] if q == 0 else []) for q in range(4)]

    def pack3(xr, xi):
        vals = (xr + xi, xr, xi)
        return tuple(_ipk(v[0:8], v[8:16] if v.shape[0] == 16 else jnp.zeros_like(v)) for v in vals)

    def s1(un, st):
        kb, chs = un
        L = [[] for _ in range(4)]
        st['L'] = L
        for r0, r1 in chs:
            T = _fft4([(pr[r0:r1, tl(4 * kb + a)], pi[r0:r1, tl(4 * kb + a)]) for a in range(4)], False)
            for ka in range(4):
                L[ka].append(pack3(*T[ka]))
            yield

    def dots3(L, m3):
        return [jnp.dot(_upk(jnp.concatenate([c[i] for c in L], axis=0)), _upk(m3[i]), preferred_element_type=f32) for i in range(3)]

    def s23(un, st):
        kb, chs = un
        Z = []
        st['Z'] = Z
        K = {}

        def filt(ka):
            k = 4 * ka + kb
            k1, k2, k3 = K[ka]
            zl = []
            for i, (r0, _) in enumerate(chs):
                q = slice(16 * i, 16 * i + 16)
                yr, yi = k1[q] - k3[q], k1[q] + k2[q]
                wr_, wi_ = wpr[r0:r0 + 16, tl(k)], wpi[r0:r0 + 16, tl(k)]
                zl.append(pack3(yr * wr_ - yi * wi_, yr * wi_ + yi * wr_))
            Z.append(zl)
        for ka in range(4):
            K[ka] = dots3(st['L'][ka], ms.at[4 * kb + ka])
            mark(K[ka][0])
            if ka > 0:
                filt(ka - 1)
            yield
        filt(3)

    def s4(un, st):
        kb, chs = un
        K = []
        st['K'] = K
        for ka in range(4):
            m3 = ms.at[4 * kb + ka]
            k1, k2, k3 = [lax.dot_general(_upk(jnp.concatenate([c[i] for c in st['Z'][ka]], axis=0)), _upk(m3[(0, 2, 1)[i]]), NT,
                                          preferred_element_type=f32) for i in range(3)]
            K.append((k1 + k3, k1 - k2))
            mark(k1)
            yield

    def s5(un, st):
        kb, chs = un
        for i, (r0, r1) in enumerate(chs):
            q = slice(16 * i, 16 * i + r1 - r0)
            us = _fft4([(kr[q], ki[q]) for kr, ki in st['K']], True)
            for a in range(4):
                yr, yi = _tw16(us[a], -a * kb) if opt('tw', 1) == 0 else us[a]
                put(pr, (slice(r0, r1), tl(4 * kb + a)), yr)
                put(pi, (slice(r0, r1), tl(4 * kb + a)), yi)
            yield

    def p2(first=False, head=None, tail=None):
        units = []
        for kb in range(4):
            byq = (kb == 0 and head is not None) or (kb == 3 and tail is not None)
            units += [(kb, chs) for chs in (BYQ if byq else CONT)]
        n = len(units)
        st = [dict() for _ in range(n)]

        def pre(i):
            g_ = s1(units[i], st[i])
            if head is not None and i < 4:
                g_ = chain(take(head, 6 if i == 0 else 4), g_)
            return g_

        def post(i):
            g_ = s5(units[i], st[i])
            if tail is not None and i >= n - 4:
                g_ = chain(g_, take(tail, 4))
            return g_
        run_all(pre(0))
        for i in range(n + 1):
            if first and i < n and units[i][0] == 2 and units[i - 1][0] == 1:
                wait('ms1')
            if i < n:
                side = pre(i + 1) if i + 1 < n else iter(())
                weave(s23(units[i], st[i]), side, 2.5)
                run_all(side)
            if i >= 1:
                side = post(i - 2) if i >= 2 else iter(())
                weave(s4(units[i - 1], st[i - 1]), side, 2.5)
                run_all(side)
        run_all(post(n - 1))
        tok.clear()

    def p2q(first=False):
        units = [(kb, BYQ[q]) for q in range(4) for kb in range(4)]
        n = len(units)
        st = [dict() for _ in range(n)]
        extra = iter(())
        if first:
            wait('ms1')
        run_all(s1(units[0], st[0]))
        rx = opt('rx', 0.5)
        for i in range(n + 1):
            if i < n:
                side = s1(units[i + 1], st[i + 1]) if i + 1 < n else iter(())
                weave(woven_nodrain(s23(units[i], st[i]), extra, rx), side, 1.5)
                run_all(side)
            if i >= 1:
                side = s5(units[i - 2], st[i - 2]) if i >= 2 else iter(())
                weave(woven_nodrain(s4(units[i - 1], st[i - 1]), extra, rx), side, 1.5)
                run_all(side)
                j = i - 2 - opt('dq', 1)
                if j >= 0 and j % 4 == 3:
                    q = j // 4
                    extra = chain(extra, *[p3pre(a, (2 * q, 2 * q + 1)) for a in range(4)])
        run_all(s5(units[n - 1], st[n - 1]))
        run_all(extra)
        tok.clear()
        for a in range(4):
            run_all(p3pre(a, (6, 7)))

    def p3pre(a, gqs=range(8)):
        row = lax.broadcasted_iota(jnp.int32, (8, 128), 0)
        def ldp(rs, kb):
            v = (pr[rs, tl(4 * kb + a)], pi[rs, tl(4 * kb + a)])
            return v if opt('tw', 1) == 0 else _tw16(v, -a * kb)
        if 0 in gqs:
            E = _fft4([ldp(slice(320, 328), kb) for kb in range(4)], True)
        for gq in gqs:
            for odd in range(2):
                Y = []
                pf = pinner(opt('age2', 3))
                for j in range(5):
                    rs = slice(64 * j + 8 * gq, 64 * j + 8 * gq + 8)
                    xs = [ldp(rs, kb) for kb in range(4)]
                    xs = [(pf(xs[0][0]), pf(xs[0][1])), (pf(xs[1][0]), pf(xs[1][1])), xs[2], xs[3]]
                    Y.append(_half4(xs, odd, True))
                for hi in range(2):
                    b = odd + 2 * hi
                    Yr = [Y[j][hi][0] for j in range(5)]; Yi = [Y[j][hi][1] for j in range(5)]
                    V0r, A1r, A2r, B1r, B2r = _r5half(Yr[0], Yr[1] - Yr[4], Yr[2] - Yr[3], Yr[1] + Yr[4], Yr[2] + Yr[3])
                    V0i, A1i, A2i, B1i, B2i = _r5half(Yi[0], Yi[1] + Yi[4], Yi[2] + Yi[3], Yi[1] - Yi[4], Yi[2] - Yi[3])
                    Vp = [(V0r, V0i), (A1r - B1i, A1i + B1r), (A2r - B2i, A2i + B2r), (A2r + B2i, A2i - B2r), (A1r + B1i, A1i - B1r)]
                    for c in range(5):
                        vr, vi = Vp[c]
                        if gq == 0:
                            er, ei = E[b]
                            th1, th3 = 2 * np.pi * c / 10, 2 * np.pi * 3 * c / 10
                            Td = (er[0:1] * float(2 * np.cos(th1)) - ei[0:1] * float(2 * np.sin(th1))
                                  + er[1:2] * float(2 * np.cos(th3)) - ei[1:2] * float(2 * np.sin(th3))
                                  + er[4:5] * float((-1) ** c))
                            vi = jnp.where(row == 0, jnp.broadcast_to(Td, (8, 128)), vi)
                        vv[64 * c + 8 * gq:64 * c + 8 * gq + 8, tl(4 * a + b)] = _ipk(vr, vi)
                yield

    def p3dot(a, mk=False):
        for b in range(4):
            csum[a + 4 * b] = None
        for c in range(5):
            y = jnp.dot(_upk(gi[c]), _upk(vv[64 * c:64 * (c + 1), 512 * a:512 * (a + 1)]), preferred_element_type=f32)
            if mk:
                mark(y)
            for b in range(4):
                xn = xread(c, a + 4 * b) + y[:, tl(b)]
                put(xt, (tl(c), tl(a + 4 * b)), xn, a == 0 and opt('f0', 0) in (1, 2))
                addsum(a + 4 * b, shifted(a + 4 * b, xn))
            if c == 4:
                nat.difference_update(a + 4 * b for b in range(4))
            yield

    def p3post(a):
        for b in range(4):
            yield from lng(a + 4 * b, hb, tl(4 * a + b))

    def phase3g(a):
        return chain(p3pre(a), p3dot(a), p3post(a))

    def cat(ref, rows, tiles):
        return jnp.concatenate([ref[rows, tl(t)] for t in tiles], axis=1)

    def piped(pieces):
        ops = pieces[0][0]()
        prev = None
        for i, (_, compute, finish) in enumerate(pieces):
            y = compute(ops)
            if prev is not None:
                prev[0](prev[1])
            prev = (finish, y)
            if i + 1 < len(pieces):
                ops = pieces[i + 1][0]()
            yield
        prev[0](prev[1])

    def mm1a_fine(marks):
        for c0 in range(0, FM, 128):
            w = cat(w1t, slice(c0, c0 + 128), [0, 4, 8, 12])
            for r0 in range(0, D, 128):
                y = lax.dot_general(_upk(hb[r0 // 2:r0 // 2 + 64, 0:512]), w, NT, preferred_element_type=f32)
                acc[r0:r0 + 128, c0:c0 + 128] = y
                if marks:
                    mark(y)
                yield

    def mm1b(c0, c1):
        tiles = [a + 4 * b for a in range(1, 4) for b in range(4)]
        uu = lax.dot_general(_upk(hb[:, 512:]), cat(w1t, slice(c0, c1), tiles), NT,
                             preferred_element_type=f32) + acc[:, c0:c1]
        uu = jax.nn.gelu(uu + b1[0:1, c0:c1], approximate=True)
        put(u, (slice(None), slice(c0, c1)), _pk(uu))

    def mm1_tail():
        tiles = [a + 4 * b for a in range(4) for b in range(4)]
        ut = lax.dot_general(cat(w1t, slice(FM, F), tiles), _upk(hb[...]), NT, preferred_element_type=f32)
        ut = jax.nn.gelu(ut + jnp.concatenate([b1c[...]] * 5, axis=1), approximate=True)
        u[:, FM:F] = _pk(ut.T)

    def mm2_epi(r0, r1, t, y):
        xn = xt[r0:r1, tl(t)] + y + b2[0:1, tl(t)]
        put(xt, (slice(r0, r1), tl(t)), xn)
        xs = shifted(t, xn)
        vv[r0 // 2:r1 // 2, vcol(t)] = _pk(xs)
        addsum(t, xs)

    def mm2(tiles):
        y = jnp.dot(_upk(u[...]), cat(w2, slice(None), tiles), preferred_element_type=f32)
        for i, t in enumerate(tiles):
            csum[t] = None
            mm2_epi(0, D, t, y[:, tl(i)])

    mk2 = []

    def mm2_fine(*pairs):
        for tiles in pairs:
            for t in tiles:
                csum[t] = None
            w = cat(w2, slice(1536, F), tiles)
            rem = []
            for c in range(5):
                rem.append(jnp.dot(_upk(u[64 * c:64 * (c + 1), 1536:F]), w, preferred_element_type=f32))
                yield
            for i, t in enumerate(tiles):
                y = [r_[:, tl(i)] for r_ in rem]
                for k0 in range(0, 1536, 512):
                    w = w2[k0:k0 + 512, tl(t)]
                    for c in range(5):
                        y[c] = y[c] + jnp.dot(_upk(u[64 * c:64 * (c + 1), k0:k0 + 512]), w, preferred_element_type=f32)
                        if k0 == 1024:
                            mm2_epi(128 * c, 128 * (c + 1), t, y[c])
                        yield

    def mm2_out(tiles):
        y = jnp.dot(_upk(u[...]), cat(w2, slice(None), tiles), preferred_element_type=f32)
        for i, t in enumerate(tiles):
            xn = xt[:, tl(t)] + y[:, tl(i)] + b2[0:1, tl(t)]
            for c in range(5):
                stage[t, pl.ds(c, 128, stride=5), :] = xn[tl(c)]

    def xstore(t):
        xin[tl(t), :] = stage[t].astype(bf16).T

    def bar():
        pl.semaphore_signal(rsem, 1)
        pl.semaphore_wait(rsem, 1)

    def take(gen, n):
        for _ in range(n):
            next(gen)
            yield

    def region(main, side, ratio, end=None):
        weave(main, side, ratio)
        run_all(side)
        if end is None:
            bar()
        else:
            with scope('W' + end):
                wait(end)

    def none_():
        return iter(())

    def p3mm1(first=False):
        marks = []
        mm = mm1a_fine(marks)
        pq = opt('pq', 0)
        region(none_() if pq else p3pre(0), none_(), 0, 'w1a' if first else None)
        if first:
            b1[...] = jnp.broadcast_to(b1v[...].astype(f32).reshape(1, F), (8, F))
            b1c[...] = jnp.broadcast_to(b1v[...].astype(f32).reshape(1, F)[:, F - 128:F], (128, 128)).T[64:128]
            b2[...] = jnp.broadcast_to(b2v[...].astype(f32).reshape(1, S), (8, S))
        if pq:
            run_all(p3dot(0))
            run_all(p3dot(1, True))
            side = p3post(0)
            weave(chain(p3dot(2, True), p3dot(3, True)), side, opt('r0', 2.5))
            run_all(side)
            tok.clear()
        else:
            n1 = opt('n1', 40)
            run_all(p3dot(0))
            bar()
            run_all(p3post(0))
            if opt('pb', 0):
                marks.append(1)
                run_all(take(mm, 3))
                side = chain(p3pre(1), p3pre(2), p3pre(3))
                weave(take(mm, n1 - 3), side, 48 / (n1 - 7))
                run_all(side)
                marks.clear()
                tok.clear()
            else:
                region(take(mm, n1), chain(p3pre(1), p3pre(2), p3pre(3)), 48 / (n1 - 2))
            run_all(chain(p3dot(1), p3dot(2), p3dot(3)))
        if opt('pin', 1):
            marks.append(1)
            run_all(take(mm, opt('n2', 3)))
        else:
            region(take(mm, opt('n2', 3)), none_(), 0)
        side = chain(p3post(1), p3post(2), p3post(3))
        weave(mm, side, opt('r3q', 1.2) if pq else opt('r3', 2.8))
        run_all(side)
        if first:
            wait('w1b')
        elif opt('lb', 0):
            bar()
        tok.clear()
        for i, c0 in enumerate(range(0, FM, 256)):
            mm1b(c0, min(FM, c0 + 256))
            if i == opt('tp', 2):
                mm1_tail()

    def mm2p1():
        if opt('mv', 0) == 0:
            for i, pair in enumerate(([1, 5], [9, 13], [2, 6], [10, 14], [3, 7], [11, 15])):
                mm2(pair)
                if i in (2, 4):
                    run_all(p1dot(i // 2))
            mm = mm2_fine([0, 4], [8, 12])
            if opt('pm', 0):
                run_all(chain(take(mm, opt('nx', 4)), p1dot(3)))
                mk2.append(1)
                run_all(take(mm, 4))
            else:
                region(chain(take(mm, opt('nx', 4)), p1dot(3), take(mm, 2)), iter(()), 0)
            side = chain(p1post(1), p1post(2), p1post(3))
            weave(mm, side, opt('r1', 0.9))
            run_all(side)
            mk2.clear()
            tok.clear()
            run_all(p1dot(0))
            bar()
            if not opt('hd', 0):
                region(p1post(0), iter(()), 0)
            return
        for pair in ([0, 4], [8, 12], [1, 5], [9, 13], [2, 6], [10, 14], [3, 7], [11, 15]):
            mm2(pair)
        run_all(p1dot(0))
        for a in range(1, 4):
            side = p1post(a - 1)
            weave(p1dot(a), side, 3.6)
            run_all(side)
        region(p1post(3), iter(()), 0)

    ocs = []

    def flush(t0, t1):
        for t in range(t0, t1):
            xstore(t)
        c = pltpu.make_async_copy(xin.at[128 * t0:128 * t1], o_hbm.at[128 * t0:128 * t1], sems.at[20 + len(ocs)])
        c.start()
        ocs.append(c)

    def out_fine(tiles):
        rem = [jnp.dot(_upk(u[64 * c:64 * (c + 1), 1536:F]), cat(w2, slice(1536, F), tiles), preferred_element_type=f32)
               for c in range(5)]
        yield
        for i, t in enumerate(tiles):
            y = [r_[:, tl(i)] for r_ in rem]
            for k0 in range(0, 1536, 512):
                w = w2[k0:k0 + 512, tl(t)]
                for c in range(5):
                    y[c] = y[c] + jnp.dot(_upk(u[64 * c:64 * (c + 1), k0:k0 + 512]), w, preferred_element_type=f32)
                    if k0 == 1024:
                        stage[t, pl.ds(c, 128, stride=5), :] = xt[tl(c), tl(t)] + y[c] + b2[0:1, tl(t)]
                yield

    def mm2_last():
        ev = opt('ev', 1)
        f1 = opt('f1', 5)
        for c in range(7):
            mm2_out([2 * c, 2 * c + 1])
            if c == f1:
                flush(0, 2 * f1)
                bar()
        if ev == 0:
            mm2_out([14, 15])
            flush(2 * f1, 14)
            flush(14, 16)
            return
        mm = out_fine([14, 15])
        run_all(take(mm, opt('e1', 5)))
        flush(2 * f1, 15 if opt('e1', 5) >= 4 else 14)
        bar()
        run_all(mm)
        flush(15 if opt('e1', 5) >= 4 else 14, 16)

    def xl(a):
        for b in range(4):
            xload(a + 4 * b)
            yield

    def lnd(a):
        return chain(p1cast(a), p1dot(a))
    none = iter(())
    with scope("wait0"):
        wait('wr')
    with scope("s1"):
        region(chain(wstep1(wr, wn0, 0, 128), wstep2a(wn0, wpr)), none, 0, 'wrb')
    wp = chain(wstep1(wr, wn0, 128, 321), wstep2b(wn0, wpr))
    with scope("s2"):
        region(take(wp, opt('w1', 20)), none, 0, 'x0')
    with scope("s3"):
        region(wp, xl(1), 0.5, 'wi')
    with scope("s4"):
        region(lnd(1), wstep1(wi, wn1, 0, 128), 1.0, 'x1')
    with scope("s5"):
        region(xl(2), woven(p1post(1), wstep2a(wn1, wpi), 0.9), 4.5, 'x2')
    with scope("s6"):
        region(xl(3), lnd(2), 2.3)
    with scope("s7"):
        region(lnd(3), p1post(2), 2.0, 'wib')
    with scope("s8"):
        region(wstep1(wi, wn1, 128, 321), p1post(3), 2.3, 'x3')
    with scope("s9"):
        region(chain(xl(0), lnd(0)), wstep2b(wn1, wpi), 1.3)
    with scope("s10"):
        region(p1post(0), none, 0, 'ms0')
    for layer in range(2):
        with scope("p2"):
            if opt('pq', 0):
                p2q(layer == 0)
            else:
                p2(layer == 0, p1post(0) if opt('hd', 0) else None, p3pre(0) if opt('tl', 0) else None)
        with scope("p3_mm1"):
            p3mm1(layer == 0)
        if layer == 0:
            with scope("waitw2"):
                wait('w2')
        with scope("mm2"):
            if layer == 0:
                mm2p1()
            else:
                mm2_last()
    with scope("outdma"):
        for c in ocs:
            c.wait()


@jax.jit
def pallas_interleave_layers__spectral_gfnet__mixer_token_mlp__prompt_kernel(A_x, A_w_r, A_w_i, B_x, B_w1, B_b1, B_w2, B_b2):
    G, GI, MS, PM = _consts()
    args = (A_x.reshape(S, D), A_w_r.T, A_w_i.T, B_w1.T, B_b1, B_w2, B_b2,
            _pack_rows(G), _pack_rows(GI), _pack_rows(MS), _pack_rows(PM))
    out = pl.pallas_call(
        kernel,
        out_shape=jax.ShapeDtypeStruct((S, D), bf16),
        in_specs=[pl.BlockSpec(memory_space=pltpu.HBM)] * len(args),
        out_specs=pl.BlockSpec(memory_space=pltpu.HBM),
        scratch_shapes=[
            pltpu.VMEM((S, D), bf16), pltpu.VMEM((321, S), bf16), pltpu.VMEM((321, S), bf16),
            pltpu.VMEM((F, S), bf16), pltpu.VMEM((F,), bf16),
            pltpu.VMEM((F, S), bf16), pltpu.VMEM((S,), bf16),
            pltpu.VMEM((5, 72, 128), u32), pltpu.VMEM((5, 64, 128), u32),
            pltpu.VMEM((16, 3, 64, 128), u32), pltpu.VMEM((264, 128), u32),
            pltpu.VMEM((16, 64, 321), u32), pltpu.VMEM((16, 64, 321), u32), pltpu.VMEM((R + 8, S), f32), pltpu.VMEM((R + 8, S), f32),
            pltpu.VMEM((D, S), f32), pltpu.VMEM((16, D, 128), f32), pltpu.VMEM((R, S), f32), pltpu.VMEM((R, S), f32),
            pltpu.VMEM((D // 2, S), u32), pltpu.VMEM((D // 2, F), u32), pltpu.VMEM((D, F), f32),
            pltpu.VMEM((D // 2, S), u32), pltpu.VMEM((720, S), f32),
            pltpu.VMEM((80, S), f32), pltpu.VMEM((8, F), f32), pltpu.VMEM((8, S), f32), pltpu.VMEM((64, 128), f32), pltpu.VMEM((8, 128), jnp.int32), pltpu.SemaphoreType.DMA((40,)), pltpu.SemaphoreType.REGULAR,
        ],
        compiler_params=pltpu.CompilerParams(vmem_limit_bytes=100 * 1024 * 1024),
    )(*args)
    return out.reshape(1, S, D)
```

```python
import math

import numpy as np
import jax
import jax.numpy as jnp
from jax import lax
import jax.experimental.pallas as pl
import jax.experimental.pallas.tpu as pltpu

S, D, F = 2048, 640, 1728
FM = 1664
R = 328
EPS = 1e-5
f32, bf16, u32, i32 = jnp.float32, jnp.bfloat16, jnp.uint32, jnp.int32
NT = (((1,), (1,)), ((), ()))

C1, C2 = float(np.cos(2 * np.pi / 5)), float(np.cos(4 * np.pi / 5))
S1, S2 = float(np.sin(2 * np.pi / 5)), float(np.sin(4 * np.pi / 5))
EXTRA = {0: 64, 4: 192, 1: 320}


def _shuffle(rows):
    return np.asarray(rows).reshape(-1, 2, 8).transpose(0, 2, 1).reshape(-1)


def _pack_rows(a):
    b = np.asarray(a, dtype=np.float32).astype(bf16).view(np.uint16).astype(np.uint32)
    return b[..., 0::2, :] | (b[..., 1::2, :] << 16)


def _tables():
    gi = np.zeros((5, 128, 128))
    lpos = _shuffle(_shuffle(np.arange(64)))
    for c in range(5):
        d = c + 5 * np.arange(128)
        for p in range(64):
            gi[c, :, 2 * p] = (1 if lpos[p] == 0 else 2) * np.cos(2 * np.pi * d * lpos[p] / 640)
            gi[c, :, 2 * p + 1] = -2 * np.sin(2 * np.pi * d * lpos[p] / 640)
        gi[c, :, 1] = (-1.0) ** np.arange(128)
    gi = gi / (D * S)
    k2 = _shuffle(np.arange(128))
    j = np.arange(64)
    ms = np.zeros((16, 5, 128, 128))
    for k1 in range(16):
        m = ms[4 * (k1 % 4) + k1 // 4]
        a = 2 * np.pi * (np.outer(np.arange(128), k1 + 16 * k2) % S) / S
        m[0], m[1], m[2] = np.cos(a), -np.sin(a) - np.cos(a), np.cos(a) - np.sin(a)
        te, to = a[0::2, :64], a[1::2, :64]
        m[3, 2 * j] = np.concatenate([np.cos(te), -np.sin(te)], 1)
        m[3, 2 * j + 1] = np.concatenate([np.sin(te), np.cos(te)], 1)
        m[4, 2 * j + 1] = np.concatenate([np.cos(to), np.sin(to)], 1)
        m[4, (2 * j + 2) % 128] = np.concatenate([np.sin(to), -np.cos(to)], 1)
    return _pack_rows(gi), _pack_rows(ms)


def _tw16(x, e):
    r, m = x
    e = e % 16
    h = float(np.sqrt(0.5))
    if e == 0:
        return x
    if e == 4:
        return (m, -r)
    if e == 12:
        return (-m, r)
    if e == 2:
        return ((r + m) * h, (m - r) * h)
    if e == 6:
        return ((m - r) * h, (r + m) * (-h))
    if e == 14:
        return ((r - m) * h, (r + m) * h)
    if e == 10:
        return ((r + m) * (-h), (r - m) * h)
    c = float(np.cos(2 * np.pi * e / 16))
    s = float(-np.sin(2 * np.pi * e / 16))
    return (r * c - m * s, r * s + m * c)


def _half4(x, odd, inv):
    (ar, ai), (br, bi), (cr, ci), (dr, di) = x
    if not odd:
        t0 = (ar + cr, ai + ci)
        t2 = (br + dr, bi + di)
        return [(t0[0] + t2[0], t0[1] + t2[1]), (t0[0] - t2[0], t0[1] - t2[1])]
    t1 = (ar - cr, ai - ci)
    t3 = (br - dr, bi - di)
    ya = (t1[0] + t3[1], t1[1] - t3[0])
    yb = (t1[0] - t3[1], t1[1] + t3[0])
    return [yb, ya] if inv else [ya, yb]


def _fft4(x, inv):
    e, o = _half4(x, 0, inv), _half4(x, 1, inv)
    return [e[0], o[0], e[1], o[1]]


def _r5half(a0, p1, p2, m1, m2):
    q = p1 + p2
    r = (p1 - p2) * ((C1 - C2) / 2)
    b = a0 - q * 0.25
    return a0 + q, b + r, b - r, m1 * S1 + m2 * S2, m1 * S2 - m2 * S1


def _fold8(x):
    parts = [x[8 * i:8 * (i + 1)] for i in range(x.shape[0] // 8)]
    while len(parts) > 1:
        parts = [parts[i] + parts[i + 1] if i + 1 < len(parts) else parts[i] for i in range(0, len(parts), 2)]
    return parts[0]


def _pk(x):
    return pltpu.bitcast(x.astype(bf16), u32)


def _ipk(a, b):
    return pltpu.pack_elementwise([a, b], packed_dtype=bf16).astype(u32)


def _upk(x):
    return pltpu.bitcast(x, bf16)


def _mm(a, b):
    return jnp.dot(a, b, preferred_element_type=f32)


def _mm_nt(a, b):
    return lax.dot_general(a, b, NT, preferred_element_type=f32)


def _iota(shape, axis):
    return lax.broadcasted_iota(i32, shape, axis)


def tl(t):
    return slice(128 * t, 128 * (t + 1))


def chain(*gens):
    for gen in gens:
        yield from gen


def take(gen, n):
    for _ in range(n):
        next(gen)
        yield


def woven(main, side, ratio):
    credit = 0.0
    for _ in main:
        credit += ratio
        while credit >= 1.0:
            next(side, None)
            credit -= 1.0
        yield
    yield from side


def emit(*gens):
    for _ in chain(*gens):
        pass


def _kernel(x_hbm, wr_hbm, wi_hbm, w1t_hbm, b1_hbm, w2_hbm, b2_hbm, gi_hbm, ms_hbm,
            o_hbm,
            xin, wr, wi, w1t, b1v, w2, b2v, g, gi, ms, pm, wn0, wn1, wpr, wpi, xt, stage, pr, pi, hb, u, acc,
            vv, vf, cs, b1, b2, b1c, zb, sems, rsem):
    groups = {}

    def dma(name, pairs):
        sem = sems.at[len(groups)]
        groups[name] = [pltpu.make_async_copy(src, dst, sem) for src, dst in pairs]

    def xtiles(a):
        return [(x_hbm.at[tl(a + 4 * b)], xin.at[tl(a + 4 * b)]) for b in range(4)]

    def w1cols(r0, r1):
        return [(w1t_hbm.at[r0:r1, 512 * b + 128:512 * (b + 1)], w1t.at[r0:r1, 512 * b + 128:512 * (b + 1)])
                for b in range(4)]

    dma('wr0', [(wr_hbm.at[0:128], wr.at[0:128])])
    dma('wr1', [(wr_hbm.at[128:321], wr.at[128:321])])
    dma('x1', xtiles(1))
    dma('wi0', [(wi_hbm.at[0:128], wi.at[0:128])])
    dma('x2', xtiles(2))
    dma('x3', xtiles(3))
    dma('wi1', [(wi_hbm.at[128:321], wi.at[128:321])])
    dma('x0', xtiles(0))
    dma('ms0', [(ms_hbm.at[0:8], ms.at[0:8])])
    dma('ms1', [(ms_hbm.at[8:16], ms.at[8:16])])
    dma('w1a', [(gi_hbm, gi), (b1_hbm, b1v), (b2_hbm, b2v)]
        + [(w1t_hbm.at[:, tl(4 * b)], w1t.at[:, tl(4 * b)]) for b in range(4)])
    dma('w1b', w1cols(0, 1024))
    dma('w2', w1cols(1024, F) + [(w2_hbm, w2)])
    for copies in groups.values():
        for cp in copies:
            cp.start()

    def sync(name=None):
        if name is None:
            pl.semaphore_signal(rsem, 1)
            pl.semaphore_wait(rsem, 1)
        else:
            for cp in groups[name]:
                cp.wait()

    pltpu.store(zb, jnp.zeros((8, 128), i32), mask=_iota((8, 128), 1) < 4096)
    tok = []

    def pin(v):
        if len(tok) < 2:
            return v
        return pltpu.bitcast(pltpu.bitcast(v, i32) | (pltpu.bitcast(tok[-2], i32) & zb[...]), f32)

    nat = set(range(16))

    def xread(c, t):
        return stage[t, pl.ds(c, 128, stride=5), :] if t in nat else xt[tl(c), tl(t)]

    def pick(nrows, colfn):
        halves = []
        for h in range(2):
            row = 2 * _iota((nrows // 2, 128), 0) + h
            halves.append(jnp.where(_iota((nrows // 2, 128), 1) == colfn(row), 1.0, 0.0))
        return halves

    def build_tables():
        def lsh(p):
            return (p & ~15) + 8 * (p & 1) + ((p & 15) >> 1)

        def rev(r):
            return jnp.where(r == 64, -1, 128 - lsh(r - 64))
        e1 = list(_shuffle(np.arange(16)))
        p128 = pick(128, lambda r: (r >> 3) + 16 * (r & 7))
        pm[0:64, :] = _ipk(*p128)
        pm[264:328, :] = _ipk(-p128[0], -p128[1])
        pm[64:136, :] = _ipk(*pick(144, lambda r: jnp.where(r < 64, lsh(r), jnp.where(
            r < 128, rev(r), jnp.where(r == 128 + e1.index(0), 64, -1)))))
        pm[136:216, :] = _ipk(*pick(160, lambda r: jnp.where(r < 64, lsh(r), jnp.where(
            r < 128, rev(r), jnp.where(r == 128, 0, jnp.where(r == 144 + e1.index(4), 64, -1))))))
        pm[216:264, :] = _ipk(*pick(96, lambda r: jnp.where(r < 64, lsh(r), jnp.where(
            r == 64, 0, jnp.where(r == 80 + e1.index(1), 64, -1)))))
        for c in range(5):
            halves = []
            for h in range(2):
                row = 2 * _iota((64, 128), 0) + h
                d = c + 5 * _iota((64, 128), 1)
                idx = jnp.where(row < 64, d * row, jnp.where(row == 64, (d - c) * 64, d * (row - 64) + 160))
                idx = idx - 640 * (((idx >> 7) * 52429) >> 18)
                idx = jnp.where(idx > 320, 640 - idx, idx)
                neg = idx > 160
                x2 = jnp.where(neg, 320 - idx, idx).astype(f32) * float(2 * np.pi / 640)
                x2 = x2 * x2
                cosv = jnp.full((64, 128), 1.0 / math.factorial(14), f32)
                for n in range(12, -1, -2):
                    cosv = 1.0 / math.factorial(n) - x2 * cosv
                halves.append(jnp.where(neg, -cosv, cosv))
            g[c] = _ipk(*halves)

    def wstep1(wsrc, wn, f0, f1):
        for t2 in range(8):
            p0 = 264 if (wsrc is wi and t2 < 4) else 0
            o = [_mm_nt(_upk(pm[p0:p0 + 64, :]), wsrc[f0:f1, tl(t)]) for t in (2 * t2, 2 * t2 + 1)]
            pk = _ipk(o[0], o[1])
            for k in range(16):
                wn[k, 8 * t2:8 * (t2 + 1), f0:f1] = pk[8 * k:8 * (k + 1)]
            yield

    def wstep2a(wn, wdst):
        for k in range(16):
            oa = _mm_nt(_upk(pm[64:136, :]), _upk(wn[k, :, 0:128]))
            wdst[0:64, tl(k)] = oa[0:64]
            wdst[256:336, tl(k)] = oa[64:144]
            yield

    def wstep2b(wn, wdst):
        for k in range(16):
            ob = _mm_nt(_upk(pm[136:216, :]), _upk(wn[k, :, 128:256]))
            oc = _mm_nt(_upk(pm[216:264, 0:65]), _upk(wn[k, :, 256:321]))
            wdst[64:264, tl(k)] = jnp.concatenate(
                [ob[0:64], oc[0:64], ob[64:72] + oc[64:72], ob[72:128], wdst[256:264, tl(k)] + ob[128:136]], axis=0)
            wdst[320:336, tl(k)] = wdst[320:336, tl(k)] + ob[144:160] + oc[80:96]
            yield

    nsum, shift, ready = {}, {}, {}

    def addsum(t, x):
        n = nsum.get(t, 0)
        cs[16 * n:16 * n + 16, tl(t)] = jnp.concatenate([_fold8(x), _fold8(x * x)], axis=0)
        nsum[t] = n + 1

    def shifted(t, x):
        if t not in nsum:
            shift[t] = x[0:1]
        return x - shift[t]

    def stats(t, double):
        n = nsum.pop(t)
        sq = cs[0:16, tl(t)]
        for i in range(1, n):
            sq = sq + cs[16 * i:16 * i + 16, tl(t)]
        m = jnp.sum(sq[0:8], axis=0, keepdims=True) * (1.0 / D)
        v = jnp.maximum(jnp.sum(sq[8:16], axis=0, keepdims=True) * (1.0 / D) - m * m, 0.0)
        if double:
            return m, lax.rsqrt(v + EPS * (v + EPS))
        return m, lax.rsqrt(v + EPS)

    def xload(a):
        for b in range(4):
            t = a + 4 * b
            x = xin[tl(t), :].T.astype(f32)
            stage[t] = x
            addsum(t, x)
            yield

    def p1cast(a):
        for b in range(4):
            m, r = stats(a + 4 * b, False)
            ready[a + 4 * b] = (None, r)
            for c in range(5):
                vv[64 * c:64 * (c + 1), tl(4 * a + b)] = _pk(xread(c, a + 4 * b) - m)
            yield

    def p1dot(a):
        st = [ready.pop(a + 4 * b) if a + 4 * b in ready else stats(a + 4 * b, False) for b in range(4)]
        r = jnp.concatenate([s[1] for s in st], axis=1)
        row = _iota((8, 512), 0)
        dc = er = ei = None
        if st[0][0] is not None:
            dc = jnp.where(row == 0, jnp.concatenate([s[0] for s in st], axis=1) * 128.0, 0.0)
        for c in range(5):
            y = _mm(_upk(g[c]), _upk(vv[64 * c:64 * (c + 1), 512 * a:512 * (a + 1)]))
            if dc is not None:
                y = jnp.concatenate([y[0:8] - dc, y[8:]], axis=0)
            y = y * r
            u64 = jnp.broadcast_to(y[64:65], (8, 512))
            cr = ci = jnp.zeros((8, 512), f32)
            for i, f in EXTRA.items():
                cr = jnp.where(row == i, float(np.cos(2 * np.pi * c * f / 640)), cr)
                ci = jnp.where(row == i, float(-np.sin(2 * np.pi * c * f / 640)), ci)
            er = u64 * cr if er is None else er + u64 * cr
            if c > 0:
                ei = u64 * ci if ei is None else ei + u64 * ci
            vf[128 * c:128 * (c + 1), 512 * a:512 * (a + 1)] = jnp.concatenate(
                [y[0:64], jnp.where(row == 0, 0.0, y[64:72]), y[72:]], axis=0)
            if c == 4:
                vf[640:656, 512 * a:512 * (a + 1)] = jnp.concatenate([er, ei], axis=0)
            yield

    def p1post(a):
        def ld(c, r0, b):
            return vf[128 * c + r0:128 * c + r0 + 8, tl(4 * a + b)]
        for gq in (0, 1, 8, 2, 3, 4, 5, 6, 7):
            for odd in range(2):
                if gq < 8:
                    y = [_half4([(ld(c, 8 * gq, b), ld(c, 64 + 8 * gq, b)) for b in range(4)], odd, False)
                         for c in range(5)]
                else:
                    y = [_half4([(ld(5, 0, b), ld(5, 8, b)) for b in range(4)], odd, False)]
                for hi in range(2):
                    kb = odd + 2 * hi
                    if gq < 8:
                        ar = [y[c][hi][0] for c in range(5)]
                        ai = [y[c][hi][1] for c in range(5)]
                        x0r, a1r, a2r, b1r, b2r = _r5half(ar[0], ar[1] + ar[4], ar[2] + ar[3], ar[1] - ar[4],
                                                          ar[2] - ar[3])
                        x0i, a1i, a2i, b1i, b2i = _r5half(ai[0], ai[1] + ai[4], ai[2] + ai[3], ai[1] - ai[4],
                                                          ai[2] - ai[3])
                        xs = [(x0r, x0i), (a1r + b1i, a1i - b1r), (a2r + b2i, a2i - b2r),
                              (b2i - a2r, a2i + b2r), (b1i - a1r, a1i + b1r)]
                    else:
                        xs = [y[0][hi]]
                    for j in range(len(xs)):
                        r0 = 64 * j + 8 * gq if gq < 8 else 320
                        kq = kb if j < 3 else (4 - kb) % 4
                        yr, yi = _tw16(xs[j], a * kq)
                        pr[r0:r0 + 8, tl(4 * kq + a)] = yr
                        pi[r0:r0 + 8, tl(4 * kq + a)] = yi
                yield

    chunks = [(r0, min(R, r0 + 16)) for r0 in range(0, R, 16)]
    edges = [0, 4, 8, 13, 17, 21]
    units = [(kb, chunks[e0:e1]) for kb in range(4) for e0, e1 in zip(edges[:-1], edges[1:])]
    lane = _iota((8, 128), 1)

    def pk16(v):
        return _ipk(v[0:8], v[8:16] if v.shape[0] == 16 else jnp.zeros_like(v))

    def rows(parts, h):
        return _upk(jnp.concatenate([p[h] for p in parts], axis=0))

    def phase2(first):
        even, low = (lane & 1) == 0, lane < 64
        lhs, eo, z, out = {}, {}, {}, {}

        def pre(i):
            kb, chs = units[i]
            for r0, r1 in chs:
                t4 = _fft4([(pr[r0:r1, tl(4 * kb + a)], pi[r0:r1, tl(4 * kb + a)]) for a in range(4)], False)
                for ka in range(4):
                    re, im = pk16(t4[ka][0]), pltpu.roll(pk16(t4[ka][1]), 1, 1)
                    lhs.setdefault((i, ka), []).append((jnp.where(even, re, im), jnp.where(even, im, re)))
                yield

        def fwd(i, ka):
            m = ms.at[4 * units[i][0] + ka]
            parts = lhs.pop((i, ka))
            eo[i, ka] = [_mm(rows(parts, h), _upk(m[3 + h])) for h in range(2)]

        def filt(i, ka):
            kb, chs = units[i]
            e, o = eo.pop((i, ka))
            z[i, ka] = []
            for j, (r0, _) in enumerate(chs):
                q = slice(16 * j, 16 * j + 16)
                p_, q_ = e[q] + o[q], pltpu.roll(e[q] - o[q], 64, 1)
                w_r, w_i = wpr[r0:r0 + 16, tl(4 * ka + kb)], wpi[r0:r0 + 16, tl(4 * ka + kb)]
                p_, q_ = p_ * w_r + q_ * w_i, q_ * w_r - p_ * w_i
                pp, qp = pk16(p_), pk16(q_)
                z[i, ka].append((pk16(p_ + q_), jnp.where(low, pp, qp), jnp.where(low, qp, pp)))

        def inv(i, ka):
            m = ms.at[4 * units[i][0] + ka]
            parts = z.pop((i, ka))
            k1, k2, k3 = [_mm_nt(rows(parts, h), _upk(m[(0, 2, 1)[h]])) for h in range(3)]
            out.setdefault(i, []).append((k1 + k3, k1 - k2))

        def post(i):
            kb, chs = units[i]
            for j, (r0, r1) in enumerate(chs):
                q = slice(16 * j, 16 * j + r1 - r0)
                t4 = _fft4([(kr[q], ki[q]) for kr, ki in out[i]], True)
                for a in range(4):
                    pr[r0:r1, tl(4 * kb + a)] = t4[a][0]
                    pi[r0:r1, tl(4 * kb + a)] = t4[a][1]
                yield

        steps = [(i, ka) for i in range(len(units)) for ka in range(4)]
        lag = 3
        emit(pre(0))
        gpre, gpost = iter(()), iter(())
        for s in range(len(steps) + lag):
            if s < len(steps):
                i, ka = steps[s]
                if ka == 0:
                    emit(gpre)
                    if first and i == len(units) // 2:
                        sync('ms1')
                    gpre = pre(i + 1) if i + 1 < len(units) else iter(())
                fwd(i, ka)
            next(gpost, None)
            if 1 <= s <= len(steps):
                filt(*steps[s - 1])
            next(gpre, None)
            if s >= lag:
                i, ka = steps[s - lag]
                inv(i, ka)
                if ka == 3:
                    emit(gpost)
                    gpost = post(i)
            if s % 4 == 2:
                next(gpre, None)
                next(gpost, None)
        emit(gpost)

    def p3pre(a):
        row = _iota((8, 128), 0)

        def ld(rs, kb):
            return _tw16((pr[rs, tl(4 * kb + a)], pi[rs, tl(4 * kb + a)]), -a * kb)
        ex = _fft4([ld(slice(320, 328), kb) for kb in range(4)], True)
        for gq in range(8):
            for odd in range(2):
                y = [_half4([ld(slice(64 * j + 8 * gq, 64 * j + 8 * gq + 8), kb) for kb in range(4)], odd, True)
                     for j in range(5)]
                for hi in range(2):
                    b = odd + 2 * hi
                    yr = [y[j][hi][0] for j in range(5)]
                    yi = [y[j][hi][1] for j in range(5)]
                    v0r, a1r, a2r, b1r, b2r = _r5half(yr[0], yr[1] - yr[4], yr[2] - yr[3], yr[1] + yr[4],
                                                      yr[2] + yr[3])
                    v0i, a1i, a2i, b1i, b2i = _r5half(yi[0], yi[1] + yi[4], yi[2] + yi[3], yi[1] - yi[4],
                                                      yi[2] - yi[3])
                    vs = [(v0r, v0i), (a1r - b1i, a1i + b1r), (a2r - b2i, a2i + b2r), (a2r + b2i, a2i - b2r),
                          (a1r + b1i, a1i - b1r)]
                    for c in range(5):
                        vr, vi = vs[c]
                        if gq == 0:
                            er, ei = ex[b]
                            th1, th3 = 2 * np.pi * c / 10, 2 * np.pi * 3 * c / 10
                            t64 = (er[0:1] * float(2 * np.cos(th1)) - ei[0:1] * float(2 * np.sin(th1))
                                   + er[1:2] * float(2 * np.cos(th3)) - ei[1:2] * float(2 * np.sin(th3))
                                   + er[4:5] * float((-1) ** c))
                            vi = jnp.where(row == 0, jnp.broadcast_to(t64, (8, 128)), vi)
                        vv[64 * c + 8 * gq:64 * c + 8 * gq + 8, tl(4 * a + b)] = _ipk(vr, vi)
                yield

    def p3dot(a):
        for c in range(5):
            y = _mm(_upk(gi[c]), _upk(vv[64 * c:64 * (c + 1), 512 * a:512 * (a + 1)]))
            for b in range(4):
                xn = xread(c, a + 4 * b) + y[:, tl(b)]
                xt[tl(c), tl(a + 4 * b)] = xn
                addsum(a + 4 * b, shifted(a + 4 * b, xn))
            if c == 4:
                nat.difference_update(a + 4 * b for b in range(4))
            yield

    def p3post(a):
        for b in range(4):
            t = a + 4 * b
            m, r = stats(t, True)
            m8 = jnp.broadcast_to(m + shift.pop(t), (8, 128))
            for c in range(5):
                xc = (xt[tl(c), tl(t)].reshape(16, 8, 128) - pin(m8)[None]).reshape(128, 128)
                hb[64 * c:64 * (c + 1), tl(4 * a + b)] = _pk(xc * r)
                yield

    def cat(ref, rs, tiles):
        return jnp.concatenate([ref[rs, tl(t)] for t in tiles], axis=1)

    def mm1_first(marking):
        for c0 in range(0, FM, 128):
            w = cat(w1t, slice(c0, c0 + 128), [0, 4, 8, 12])
            for c in range(5):
                y = _mm_nt(_upk(hb[64 * c:64 * (c + 1), 0:512]), w)
                acc[tl(c), c0:c0 + 128] = y
                if marking:
                    tok.append(y[0:8])
                yield

    def mm1_rest(c0, c1):
        tiles = [a + 4 * b for a in range(1, 4) for b in range(4)]
        h = _mm_nt(_upk(hb[:, 512:]), cat(w1t, slice(c0, c1), tiles)) + acc[:, c0:c1]
        u[:, c0:c1] = _pk(jax.nn.gelu(h + b1[0:1, c0:c1], approximate=True))

    def mm1_tail():
        tiles = [a + 4 * b for a in range(4) for b in range(4)]
        h = _mm_nt(cat(w1t, slice(FM, F), tiles), _upk(hb[...])) + jnp.concatenate([b1c[...]] * 5, axis=1)
        u[:, FM:F] = _pk(jax.nn.gelu(h, approximate=True).T)

    def to_state(c0, c1, t, y):
        xn = xt[128 * c0:128 * c1, tl(t)] + y + b2[0:1, tl(t)]
        xt[128 * c0:128 * c1, tl(t)] = xn
        xs = shifted(t, xn)
        vv[64 * c0:64 * c1, tl(4 * (t % 4) + t // 4)] = _pk(xs)
        addsum(t, xs)

    def to_output(c0, c1, t, y):
        xn = xt[128 * c0:128 * c1, tl(t)] + y + b2[0:1, tl(t)]
        for c in range(c0, c1):
            stage[t, pl.ds(c, 128, stride=5), :] = xn[tl(c - c0)]

    def mm2(tiles, sink):
        y = _mm(_upk(u[...]), cat(w2, slice(None), tiles))
        for i, t in enumerate(tiles):
            sink(0, 5, t, y[:, tl(i)])

    def mm2_fine(tiles, sink):
        w = cat(w2, slice(1536, F), tiles)
        rem = []
        for c in range(5):
            rem.append(_mm(_upk(u[64 * c:64 * (c + 1), 1536:F]), w))
            yield
        for i, t in enumerate(tiles):
            y = [r[:, tl(i)] for r in rem]
            for k0 in range(0, 1536, 512):
                w = w2[k0:k0 + 512, tl(t)]
                for c in range(5):
                    y[c] = y[c] + _mm(_upk(u[64 * c:64 * (c + 1), k0:k0 + 512]), w)
                    if k0 == 1024:
                        sink(c, c + 1, t, y[c])
                    yield

    def phase3_mm1(first):
        marking = []
        mm = mm1_first(marking)
        emit(p3pre(0))
        sync('w1a' if first else None)
        if first:
            b1f = b1v[...].astype(f32).reshape(1, F)
            b1[...] = jnp.broadcast_to(b1f, (8, F))
            b1c[...] = jnp.broadcast_to(b1f[:, F - 128:F], (128, 128)).T[64:128]
            b2[...] = jnp.broadcast_to(b2v[...].astype(f32).reshape(1, S), (8, S))
        emit(p3dot(0))
        sync()
        emit(p3post(0), woven(take(mm, 44), chain(p3pre(1), p3pre(2), p3pre(3)), 48 / 42))
        sync('w1b' if first else None)
        emit(p3dot(1), p3dot(2), p3dot(3))
        marking.append(True)
        emit(take(mm, 3), woven(mm, chain(p3post(1), p3post(2), p3post(3)), 3.4))
        tok.clear()
        for i, c0 in enumerate(range(0, FM, 256)):
            mm1_rest(c0, min(FM, c0 + 256))
            if i == 5:
                mm1_tail()
            if first and i == 3:
                sync('w2')

    def mm2_phase1():
        for i, pair in enumerate(([1, 5], [9, 13], [2, 6], [10, 14], [3, 7], [11, 15])):
            mm2(pair, to_state)
            if i in (2, 4):
                emit(p1dot(i // 2))
        mm = chain(mm2_fine([0, 4], to_state), mm2_fine([8, 12], to_state))
        emit(take(mm, 4), p1dot(3), take(mm, 2))
        sync()
        emit(woven(mm, chain(p1post(1), p1post(2), p1post(3)), 0.9), p1dot(0), p1post(0))
        sync()

    outs = []

    def flush(t0, t1):
        for t in range(t0, t1):
            xin[tl(t), :] = stage[t].astype(bf16).T
        cp = pltpu.make_async_copy(xin.at[128 * t0:128 * t1], o_hbm.at[128 * t0:128 * t1],
                                   sems.at[len(groups) + len(outs)])
        cp.start()
        outs.append(cp)

    def mm2_output():
        for c in range(7):
            mm2([2 * c, 2 * c + 1], to_output)
            if c == 5:
                flush(0, 10)
                sync()
        mm = mm2_fine([14, 15], to_output)
        emit(take(mm, 25))
        flush(10, 15)
        sync()
        emit(mm)
        flush(15, 16)

    build_tables()
    sync('wr0')
    emit(wstep1(wr, wn0, 0, 128), wstep2a(wn0, wpr))
    sync('wr1')
    wp = chain(wstep1(wr, wn0, 128, 321), wstep2b(wn0, wpr))
    emit(take(wp, 20))
    sync('x1')
    emit(woven(wp, xload(1), 0.5))
    sync('wi0')
    emit(woven(chain(p1cast(1), p1dot(1)), wstep1(wi, wn1, 0, 128), 1.0))
    sync('x2')
    emit(woven(xload(2), woven(p1post(1), wstep2a(wn1, wpi), 0.9), 4.5))
    sync('x3')
    emit(woven(xload(3), chain(p1cast(2), p1dot(2)), 2.3))
    sync()
    emit(woven(chain(p1cast(3), p1dot(3)), p1post(2), 2.0))
    sync('wi1')
    emit(woven(wstep1(wi, wn1, 128, 321), p1post(3), 2.3))
    sync('x0')
    emit(woven(chain(xload(0), p1cast(0), p1dot(0)), wstep2b(wn1, wpi), 1.3), p1post(0))
    sync('ms0')
    for layer in range(2):
        phase2(layer == 0)
        phase3_mm1(layer == 0)
        if layer == 0:
            mm2_phase1()
        else:
            mm2_output()
    for cp in outs:
        cp.wait()


@jax.jit
def pallas_interleave_layers__spectral_gfnet__mixer_token_mlp__prompt_kernel(A_x, A_w_r, A_w_i, B_x, B_w1, B_b1, B_w2, B_b2):
    gi, ms = _tables()
    args = (A_x.reshape(S, D), A_w_r.T, A_w_i.T, B_w1.T, B_b1, B_w2, B_b2, gi, ms)
    vmem = pltpu.VMEM
    out = pl.pallas_call(
        _kernel,
        out_shape=jax.ShapeDtypeStruct((S, D), bf16),
        in_specs=[pl.BlockSpec(memory_space=pltpu.HBM)] * len(args),
        out_specs=pl.BlockSpec(memory_space=pltpu.HBM),
        scratch_shapes=[
            vmem((S, D), bf16), vmem((321, S), bf16), vmem((321, S), bf16),
            vmem((F, S), bf16), vmem((F,), bf16), vmem((F, S), bf16), vmem((S,), bf16),
            vmem((5, 64, 128), u32), vmem((5, 64, 128), u32),
            vmem((16, 5, 64, 128), u32), vmem((328, 128), u32),
            vmem((16, 64, 321), u32), vmem((16, 64, 321), u32),
            vmem((R + 8, S), f32), vmem((R + 8, S), f32),
            vmem((D, S), f32), vmem((16, D, 128), f32),
            vmem((R, S), f32), vmem((R, S), f32),
            vmem((D // 2, S), u32), vmem((D // 2, F), u32), vmem((D, FM), f32),
            vmem((D // 2, S), u32), vmem((656, S), f32), vmem((80, S), f32),
            vmem((8, F), f32), vmem((8, S), f32), vmem((64, 128), f32),
            vmem((8, 128), i32),
            pltpu.SemaphoreType.DMA((16,)), pltpu.SemaphoreType.REGULAR,
        ],
        compiler_params=pltpu.CompilerParams(vmem_limit_bytes=100 * 1024 * 1024),
    )(*args)
    return out.reshape(1, S, D)
```

```python
import math

import numpy as np
import jax
import jax.numpy as jnp
from jax import lax
import jax.experimental.pallas as pl
import jax.experimental.pallas.tpu as pltpu

S, D, F = 2048, 640, 1728
FM = 1664
R = 328
EPS = 1e-5
f32, bf16, u32, i32 = jnp.float32, jnp.bfloat16, jnp.uint32, jnp.int32
NT = (((1,), (1,)), ((), ()))

C1, C2 = float(np.cos(2 * np.pi / 5)), float(np.cos(4 * np.pi / 5))
S1, S2 = float(np.sin(2 * np.pi / 5)), float(np.sin(4 * np.pi / 5))
EXTRA = {0: 64, 4: 192, 1: 320}


def _shuffle(rows):
    return np.asarray(rows).reshape(-1, 2, 8).transpose(0, 2, 1).reshape(-1)


def _pack_rows(a):
    b = np.asarray(a, dtype=np.float32).astype(bf16).view(np.uint16).astype(np.uint32)
    return b[..., 0::2, :] | (b[..., 1::2, :] << 16)


def _tables():
    gi = np.zeros((5, 128, 128))
    lpos = _shuffle(_shuffle(np.arange(64)))
    for c in range(5):
        d = c + 5 * np.arange(128)
        for p in range(64):
            gi[c, :, 2 * p] = (1 if lpos[p] == 0 else 2) * np.cos(2 * np.pi * d * lpos[p] / 640)
            gi[c, :, 2 * p + 1] = -2 * np.sin(2 * np.pi * d * lpos[p] / 640)
        gi[c, :, 1] = (-1.0) ** np.arange(128)
    gi = gi / (D * S)
    k2 = _shuffle(np.arange(128))
    j = np.arange(64)
    ms = np.zeros((16, 5, 128, 128))
    for k1 in range(16):
        m = ms[4 * (k1 % 4) + k1 // 4]
        a = 2 * np.pi * (np.outer(np.arange(128), k1 + 16 * k2) % S) / S
        m[0], m[1], m[2] = np.cos(a), -np.sin(a) - np.cos(a), np.cos(a) - np.sin(a)
        te, to = a[0::2, :64], a[1::2, :64]
        m[3, 2 * j] = np.concatenate([np.cos(te), -np.sin(te)], 1)
        m[3, 2 * j + 1] = np.concatenate([np.sin(te), np.cos(te)], 1)
        m[4, 2 * j + 1] = np.concatenate([np.cos(to), np.sin(to)], 1)
        m[4, (2 * j + 2) % 128] = np.concatenate([np.sin(to), -np.cos(to)], 1)
    return _pack_rows(gi), _pack_rows(ms)


def _tw16(x, e):
    r, m = x
    e = e % 16
    h = float(np.sqrt(0.5))
    if e == 0:
        return x
    if e == 4:
        return (m, -r)
    if e == 12:
        return (-m, r)
    if e == 2:
        return ((r + m) * h, (m - r) * h)
    if e == 6:
        return ((m - r) * h, (r + m) * (-h))
    if e == 14:
        return ((r - m) * h, (r + m) * h)
    if e == 10:
        return ((r + m) * (-h), (r - m) * h)
    c = float(np.cos(2 * np.pi * e / 16))
    s = float(-np.sin(2 * np.pi * e / 16))
    return (r * c - m * s, r * s + m * c)


def _half4(x, odd, inv):
    (ar, ai), (br, bi), (cr, ci), (dr, di) = x
    if not odd:
        t0 = (ar + cr, ai + ci)
        t2 = (br + dr, bi + di)
        return [(t0[0] + t2[0], t0[1] + t2[1]), (t0[0] - t2[0], t0[1] - t2[1])]
    t1 = (ar - cr, ai - ci)
    t3 = (br - dr, bi - di)
    ya = (t1[0] + t3[1], t1[1] - t3[0])
    yb = (t1[0] - t3[1], t1[1] + t3[0])
    return [yb, ya] if inv else [ya, yb]


def _fft4(x, inv):
    e, o = _half4(x, 0, inv), _half4(x, 1, inv)
    return [e[0], o[0], e[1], o[1]]


def _r5half(a0, p1, p2, m1, m2):
    q = p1 + p2
    r = (p1 - p2) * ((C1 - C2) / 2)
    b = a0 - q * 0.25
    return a0 + q, b + r, b - r, m1 * S1 + m2 * S2, m1 * S2 - m2 * S1


def _fold8(x):
    parts = [x[8 * i:8 * (i + 1)] for i in range(x.shape[0] // 8)]
    while len(parts) > 1:
        parts = [parts[i] + parts[i + 1] if i + 1 < len(parts) else parts[i] for i in range(0, len(parts), 2)]
    return parts[0]


def _pk(x):
    return pltpu.bitcast(x.astype(bf16), u32)


def _ipk(a, b):
    return pltpu.pack_elementwise([a, b], packed_dtype=bf16).astype(u32)


def _upk(x):
    return pltpu.bitcast(x, bf16)


def _mm(a, b):
    return jnp.dot(a, b, preferred_element_type=f32)


def _mm_nt(a, b):
    return lax.dot_general(a, b, NT, preferred_element_type=f32)


def _iota(shape, axis):
    return lax.broadcasted_iota(i32, shape, axis)


def tl(t):
    return slice(128 * t, 128 * (t + 1))


def chain(*gens):
    for gen in gens:
        yield from gen


def take(gen, n):
    for _ in range(n):
        next(gen)
        yield


def woven(main, side, ratio):
    credit = 0.0
    for _ in main:
        credit += ratio
        while credit >= 1.0:
            next(side, None)
            credit -= 1.0
        yield
    yield from side


def emit(*gens):
    for _ in chain(*gens):
        pass


def _kernel(x_hbm, wr_hbm, wi_hbm, w1t_hbm, b1_hbm, w2_hbm, b2_hbm, gi_hbm, ms_hbm,
            o_hbm,
            xin, wr, wi, w1t, b1v, w2, b2v, g, gi, ms, pm, wn0, wn1, wpr, wpi, xt, stage, pr, pi, hb, u, acc,
            vv, vf, cs, b1, b2, b1c, zb, sems, rsem):
    groups = {}

    def dma(name, pairs):
        sem = sems.at[len(groups)]
        groups[name] = [pltpu.make_async_copy(src, dst, sem) for src, dst in pairs]

    def xtiles(a):
        return [(x_hbm.at[tl(a + 4 * b)], xin.at[tl(a + 4 * b)]) for b in range(4)]

    def w1cols(r0, r1):
        return [(w1t_hbm.at[r0:r1, 512 * b + 128:512 * (b + 1)], w1t.at[r0:r1, 512 * b + 128:512 * (b + 1)])
                for b in range(4)]

    dma('wr0', [(wr_hbm.at[0:128], wr.at[0:128])])
    dma('wr1', [(wr_hbm.at[128:321], wr.at[128:321])])
    dma('x1', xtiles(1))
    dma('wi0', [(wi_hbm.at[0:128], wi.at[0:128])])
    dma('x2', xtiles(2))
    dma('x3', xtiles(3))
    dma('wi1', [(wi_hbm.at[128:321], wi.at[128:321])])
    dma('x0', xtiles(0))
    dma('ms0', [(ms_hbm.at[0:8], ms.at[0:8])])
    dma('ms1', [(ms_hbm.at[8:16], ms.at[8:16])])
    dma('w1a', [(gi_hbm, gi), (b1_hbm, b1v), (b2_hbm, b2v)]
        + [(w1t_hbm.at[:, tl(4 * b)], w1t.at[:, tl(4 * b)]) for b in range(4)])
    dma('w1b', w1cols(0, 1024))
    dma('w2', w1cols(1024, F) + [(w2_hbm, w2)])
    for copies in groups.values():
        for cp in copies:
            cp.start()

    def sync(name=None):
        if name is None:
            pl.semaphore_signal(rsem, 1)
            pl.semaphore_wait(rsem, 1)
        else:
            for cp in groups[name]:
                cp.wait()

    pltpu.store(zb, jnp.zeros((8, 128), i32), mask=_iota((8, 128), 1) < 4096)
    tok = []

    def pin(v):
        if len(tok) < 2:
            return v
        return pltpu.bitcast(pltpu.bitcast(v, i32) | (pltpu.bitcast(tok[-2], i32) & zb[...]), f32)

    nat = set(range(16))

    def xread(c, t):
        return stage[t, pl.ds(c, 128, stride=5), :] if t in nat else xt[tl(c), tl(t)]

    def pick(nrows, colfn):
        halves = []
        for h in range(2):
            row = 2 * _iota((nrows // 2, 128), 0) + h
            halves.append(jnp.where(_iota((nrows // 2, 128), 1) == colfn(row), 1.0, 0.0))
        return halves

    def build_tables():
        def lsh(p):
            return (p & ~15) + 8 * (p & 1) + ((p & 15) >> 1)

        p128 = pick(128, lambda r: (r >> 3) + 16 * (r & 7))
        pm[0:64, :] = _ipk(*p128)
        pm[64:128, :] = _ipk(-p128[0], -p128[1])
        pm[128:200, :] = _ipk(*pick(144, lambda r: jnp.where(r < 64, lsh(r), jnp.where(
            (r == 64) | (r == 130), 64, jnp.where(r < 128, 128 - lsh(r - 64), -1)))))
        for c in range(5):
            halves = []
            for h in range(2):
                row = 2 * _iota((64, 128), 0) + h
                d = c + 5 * _iota((64, 128), 1)
                idx = jnp.where(row < 64, d * row, jnp.where(row == 64, (d - c) * 64, d * (row - 64) + 160))
                idx = idx - 640 * (((idx >> 7) * 52429) >> 18)
                idx = jnp.where(idx > 320, 640 - idx, idx)
                neg = idx > 160
                x2 = jnp.where(neg, 320 - idx, idx).astype(f32) * float(2 * np.pi / 640)
                x2 = x2 * x2
                cosv = jnp.full((64, 128), 1.0 / math.factorial(14), f32)
                for n in range(12, -1, -2):
                    cosv = 1.0 / math.factorial(n) - x2 * cosv
                halves.append(jnp.where(neg, -cosv, cosv))
            g[c] = _ipk(*halves)

    def wstep1(wsrc, wn, f0, f1):
        for t2 in range(8):
            p0 = 64 if (wsrc is wi and t2 < 4) else 0
            o = [_mm_nt(_upk(pm[p0:p0 + 64, :]), wsrc[f0:f1, tl(t)]) for t in (2 * t2, 2 * t2 + 1)]
            pk = _ipk(o[0], o[1])
            for k in range(16):
                wn[k, 8 * t2:8 * (t2 + 1), f0:f1] = pk[8 * k:8 * (k + 1)]
            yield

    def wstep2a(wn, wdst):
        for k in range(16):
            oa = _mm_nt(_upk(pm[128:192, :]), _upk(wn[k, :, 0:128]))
            wdst[0:64, tl(k)] = oa[0:64]
            wdst[256:320, tl(k)] = oa[64:128]
            yield

    def wstep2b(wn, wdst):
        top = _iota((8, 128), 0) == 0
        for k in range(16):
            ob = _mm_nt(_upk(pm[128:192, :]), _upk(wn[k, :, 128:256]))
            oc = _mm_nt(_upk(jnp.concatenate([pm[128:160, 0:65], pm[192:200, 0:65]], axis=0)), _upk(wn[k, :, 256:321]))
            j4 = wdst[256:264, tl(k)]
            wdst[64:264, tl(k)] = jnp.concatenate(
                [ob[0:64], oc[0:64], jnp.where(top, oc[0:8], ob[64:72]), ob[72:128], jnp.where(top, ob[0:8], j4)],
                axis=0)
            wdst[320:336, tl(k)] = jnp.concatenate(
                [jnp.where(top, j4, oc[64:72]), jnp.where(top, ob[64:72], 0.0)], axis=0)
            yield

    nsum, shift, ready = {}, {}, {}

    def addsum(t, x):
        n = nsum.get(t, 0)
        cs[16 * n:16 * n + 16, tl(t)] = jnp.concatenate([_fold8(x), _fold8(x * x)], axis=0)
        nsum[t] = n + 1

    def shifted(t, x):
        if t not in nsum:
            shift[t] = x[0:1]
        return x - shift[t]

    def stats(t, double):
        n = nsum.pop(t)
        sq = cs[0:16, tl(t)]
        for i in range(1, n):
            sq = sq + cs[16 * i:16 * i + 16, tl(t)]
        m = jnp.sum(sq[0:8], axis=0, keepdims=True) * (1.0 / D)
        v = jnp.maximum(jnp.sum(sq[8:16], axis=0, keepdims=True) * (1.0 / D) - m * m, 0.0)
        if double:
            return m, lax.rsqrt(v + EPS * (v + EPS))
        return m, lax.rsqrt(v + EPS)

    def xload(a):
        for b in range(4):
            t = a + 4 * b
            x = xin[tl(t), :].T.astype(f32)
            stage[t] = x
            addsum(t, x)
            yield

    def p1cast(a):
        for b in range(4):
            m, r = stats(a + 4 * b, False)
            ready[a + 4 * b] = (None, r)
            for c in range(5):
                vv[64 * c:64 * (c + 1), tl(4 * a + b)] = _pk(xread(c, a + 4 * b) - m)
            yield

    def p1dot(a):
        st = [ready.pop(a + 4 * b) if a + 4 * b in ready else stats(a + 4 * b, False) for b in range(4)]
        r = jnp.concatenate([s[1] for s in st], axis=1)
        row = _iota((8, 512), 0)
        dc = er = ei = None
        if st[0][0] is not None:
            dc = jnp.where(row == 0, jnp.concatenate([s[0] for s in st], axis=1) * 128.0, 0.0)
        for c in range(5):
            y = _mm(_upk(g[c]), _upk(vv[64 * c:64 * (c + 1), 512 * a:512 * (a + 1)]))
            if dc is not None:
                y = jnp.concatenate([y[0:8] - dc, y[8:]], axis=0)
            y = y * r
            u64 = jnp.broadcast_to(y[64:65], (8, 512))
            cr = ci = jnp.zeros((8, 512), f32)
            for i, f in EXTRA.items():
                cr = jnp.where(row == i, float(np.cos(2 * np.pi * c * f / 640)), cr)
                ci = jnp.where(row == i, float(-np.sin(2 * np.pi * c * f / 640)), ci)
            er = u64 * cr if er is None else er + u64 * cr
            if c > 0:
                ei = u64 * ci if ei is None else ei + u64 * ci
            vf[128 * c:128 * (c + 1), 512 * a:512 * (a + 1)] = jnp.concatenate(
                [y[0:64], jnp.where(row == 0, 0.0, y[64:72]), y[72:]], axis=0)
            if c == 4:
                vf[640:656, 512 * a:512 * (a + 1)] = jnp.concatenate([er, ei], axis=0)
            yield

    def p1post(a):
        def ld(c, r0, b):
            return vf[128 * c + r0:128 * c + r0 + 8, tl(4 * a + b)]
        for gq in (0, 1, 8, 2, 3, 4, 5, 6, 7):
            for odd in range(2):
                if gq < 8:
                    y = [_half4([(ld(c, 8 * gq, b), ld(c, 64 + 8 * gq, b)) for b in range(4)], odd, False)
                         for c in range(5)]
                else:
                    y = [_half4([(ld(5, 0, b), ld(5, 8, b)) for b in range(4)], odd, False)]
                for hi in range(2):
                    kb = odd + 2 * hi
                    if gq < 8:
                        ar = [y[c][hi][0] for c in range(5)]
                        ai = [y[c][hi][1] for c in range(5)]
                        x0r, a1r, a2r, b1r, b2r = _r5half(ar[0], ar[1] + ar[4], ar[2] + ar[3], ar[1] - ar[4],
                                                          ar[2] - ar[3])
                        x0i, a1i, a2i, b1i, b2i = _r5half(ai[0], ai[1] + ai[4], ai[2] + ai[3], ai[1] - ai[4],
                                                          ai[2] - ai[3])
                        xs = [(x0r, x0i), (a1r + b1i, a1i - b1r), (a2r + b2i, a2i - b2r),
                              (b2i - a2r, a2i + b2r), (b1i - a1r, a1i + b1r)]
                    else:
                        xs = [y[0][hi]]
                    for j in range(len(xs)):
                        r0 = 64 * j + 8 * gq if gq < 8 else 320
                        kq = kb if j < 3 else (4 - kb) % 4
                        yr, yi = _tw16(xs[j], a * kq)
                        pr[r0:r0 + 8, tl(4 * kq + a)] = yr
                        pi[r0:r0 + 8, tl(4 * kq + a)] = yi
                yield

    chunks = [(r0, min(R, r0 + 16)) for r0 in range(0, R, 16)]
    edges = [0, 4, 8, 13, 17, 21]
    units = [(kb, chunks[e0:e1]) for kb in range(4) for e0, e1 in zip(edges[:-1], edges[1:])]
    lane = _iota((8, 128), 1)

    def pk16(v):
        return _ipk(v[0:8], v[8:16] if v.shape[0] == 16 else jnp.zeros_like(v))

    def rows(parts, h):
        return _upk(jnp.concatenate([p[h] for p in parts], axis=0))

    def phase2(first):
        even, low = (lane & 1) == 0, lane < 64
        lhs, eo, z, out = {}, {}, {}, {}

        def pre(i):
            kb, chs = units[i]
            for r0, r1 in chs:
                t4 = _fft4([(pr[r0:r1, tl(4 * kb + a)], pi[r0:r1, tl(4 * kb + a)]) for a in range(4)], False)
                for ka in range(4):
                    re, im = pk16(t4[ka][0]), pltpu.roll(pk16(t4[ka][1]), 1, 1)
                    lhs.setdefault((i, ka), []).append((jnp.where(even, re, im), jnp.where(even, im, re)))
                yield

        def fwd(i, ka):
            m = ms.at[4 * units[i][0] + ka]
            parts = lhs.pop((i, ka))
            eo[i, ka] = [_mm(rows(parts, h), _upk(m[3 + h])) for h in range(2)]

        def filt(i, ka):
            kb, chs = units[i]
            e, o = eo.pop((i, ka))
            z[i, ka] = []
            for j, (r0, _) in enumerate(chs):
                q = slice(16 * j, 16 * j + 16)
                p_, q_ = e[q] + o[q], pltpu.roll(e[q] - o[q], 64, 1)
                w_r, w_i = wpr[r0:r0 + 16, tl(4 * ka + kb)], wpi[r0:r0 + 16, tl(4 * ka + kb)]
                p_, q_ = p_ * w_r + q_ * w_i, q_ * w_r - p_ * w_i
                pp, qp = pk16(p_), pk16(q_)
                z[i, ka].append((pk16(p_ + q_), jnp.where(low, pp, qp), jnp.where(low, qp, pp)))

        def inv(i, ka):
            m = ms.at[4 * units[i][0] + ka]
            parts = z.pop((i, ka))
            k1, k2, k3 = [_mm_nt(rows(parts, h), _upk(m[(0, 2, 1)[h]])) for h in range(3)]
            out.setdefault(i, []).append((k1 + k3, k1 - k2))

        def post(i):
            kb, chs = units[i]
            for j, (r0, r1) in enumerate(chs):
                q = slice(16 * j, 16 * j + r1 - r0)
                t4 = _fft4([(kr[q], ki[q]) for kr, ki in out[i]], True)
                for a in range(4):
                    pr[r0:r1, tl(4 * kb + a)] = t4[a][0]
                    pi[r0:r1, tl(4 * kb + a)] = t4[a][1]
                yield

        steps = [(i, ka) for i in range(len(units)) for ka in range(4)]
        lag = 3
        emit(pre(0))
        gpre, gpost = iter(()), iter(())
        for s in range(len(steps) + lag):
            if s < len(steps):
                i, ka = steps[s]
                if ka == 0:
                    emit(gpre)
                    if first and i == len(units) // 2:
                        sync('ms1')
                    gpre = pre(i + 1) if i + 1 < len(units) else iter(())
                fwd(i, ka)
            next(gpost, None)
            if 1 <= s <= len(steps):
                filt(*steps[s - 1])
            next(gpre, None)
            if s >= lag:
                i, ka = steps[s - lag]
                inv(i, ka)
                if ka == 3:
                    emit(gpost)
                    gpost = post(i)
            if s % 4 == 2:
                next(gpre, None)
                next(gpost, None)
        emit(gpost)

    def p3pre(a):
        row = _iota((8, 128), 0)

        def ld(rs, kb):
            return _tw16((pr[rs, tl(4 * kb + a)], pi[rs, tl(4 * kb + a)]), -a * kb)
        ex = _fft4([ld(slice(320, 328), kb) for kb in range(4)], True)
        for gq in range(8):
            for odd in range(2):
                y = [_half4([ld(slice(64 * j + 8 * gq, 64 * j + 8 * gq + 8), kb) for kb in range(4)], odd, True)
                     for j in range(5)]
                for hi in range(2):
                    b = odd + 2 * hi
                    yr = [y[j][hi][0] for j in range(5)]
                    yi = [y[j][hi][1] for j in range(5)]
                    v0r, a1r, a2r, b1r, b2r = _r5half(yr[0], yr[1] - yr[4], yr[2] - yr[3], yr[1] + yr[4],
                                                      yr[2] + yr[3])
                    v0i, a1i, a2i, b1i, b2i = _r5half(yi[0], yi[1] + yi[4], yi[2] + yi[3], yi[1] - yi[4],
                                                      yi[2] - yi[3])
                    vs = [(v0r, v0i), (a1r - b1i, a1i + b1r), (a2r - b2i, a2i + b2r), (a2r + b2i, a2i - b2r),
                          (a1r + b1i, a1i - b1r)]
                    for c in range(5):
                        vr, vi = vs[c]
                        if gq == 0:
                            er, ei = ex[b]
                            th1, th3 = 2 * np.pi * c / 10, 2 * np.pi * 3 * c / 10
                            t64 = (er[0:1] * float(2 * np.cos(th1)) - ei[0:1] * float(2 * np.sin(th1))
                                   + er[1:2] * float(2 * np.cos(th3)) - ei[1:2] * float(2 * np.sin(th3))
                                   + er[4:5] * float((-1) ** c))
                            vi = jnp.where(row == 0, jnp.broadcast_to(t64, (8, 128)), vi)
                        vv[64 * c + 8 * gq:64 * c + 8 * gq + 8, tl(4 * a + b)] = _ipk(vr, vi)
                yield

    def p3dot(a):
        for c in range(5):
            y = _mm(_upk(gi[c]), _upk(vv[64 * c:64 * (c + 1), 512 * a:512 * (a + 1)]))
            for b in range(4):
                xn = xread(c, a + 4 * b) + y[:, tl(b)]
                xt[tl(c), tl(a + 4 * b)] = xn
                addsum(a + 4 * b, shifted(a + 4 * b, xn))
            if c == 4:
                nat.difference_update(a + 4 * b for b in range(4))
            yield

    def p3post(a):
        for b in range(4):
            t = a + 4 * b
            m, r = stats(t, True)
            m8 = jnp.broadcast_to(m + shift.pop(t), (8, 128))
            for c in range(5):
                xc = (xt[tl(c), tl(t)].reshape(16, 8, 128) - pin(m8)[None]).reshape(128, 128)
                hb[64 * c:64 * (c + 1), tl(4 * a + b)] = _pk(xc * r)
                yield

    def cat(ref, rs, tiles):
        return jnp.concatenate([ref[rs, tl(t)] for t in tiles], axis=1)

    def mm1_first(marking):
        for c0 in range(0, FM, 128):
            w = cat(w1t, slice(c0, c0 + 128), [0, 4, 8, 12])
            for c in range(5):
                y = _mm_nt(_upk(hb[64 * c:64 * (c + 1), 0:512]), w)
                acc[tl(c), c0:c0 + 128] = y
                if marking:
                    tok.append(y[0:8])
                yield

    def mm1_rest(c0, c1):
        tiles = [a + 4 * b for a in range(1, 4) for b in range(4)]
        h = _mm_nt(_upk(hb[:, 512:]), cat(w1t, slice(c0, c1), tiles)) + acc[:, c0:c1]
        u[:, c0:c1] = _pk(jax.nn.gelu(h + b1[0:1, c0:c1], approximate=True))

    def mm1_tail():
        tiles = [a + 4 * b for a in range(4) for b in range(4)]
        h = _mm_nt(cat(w1t, slice(FM, F), tiles), _upk(hb[...])) + jnp.concatenate([b1c[...]] * 5, axis=1)
        u[:, FM:F] = _pk(jax.nn.gelu(h, approximate=True).T)

    def to_state(c0, c1, t, y):
        xn = xt[128 * c0:128 * c1, tl(t)] + y + b2[0:1, tl(t)]
        xt[128 * c0:128 * c1, tl(t)] = xn
        xs = shifted(t, xn)
        vv[64 * c0:64 * c1, tl(4 * (t % 4) + t // 4)] = _pk(xs)
        addsum(t, xs)

    def to_output(c0, c1, t, y):
        xn = xt[128 * c0:128 * c1, tl(t)] + y + b2[0:1, tl(t)]
        for c in range(c0, c1):
            stage[t, pl.ds(c, 128, stride=5), :] = xn[tl(c - c0)]

    def mm2(tiles, sink):
        y = _mm(_upk(u[...]), cat(w2, slice(None), tiles))
        for i, t in enumerate(tiles):
            sink(0, 5, t, y[:, tl(i)])

    def mm2_fine(tiles, sink):
        w = cat(w2, slice(1536, F), tiles)
        rem = []
        for c in range(5):
            rem.append(_mm(_upk(u[64 * c:64 * (c + 1), 1536:F]), w))
            yield
        for i, t in enumerate(tiles):
            y = [r[:, tl(i)] for r in rem]
            for k0 in range(0, 1536, 512):
                w = w2[k0:k0 + 512, tl(t)]
                for c in range(5):
                    y[c] = y[c] + _mm(_upk(u[64 * c:64 * (c + 1), k0:k0 + 512]), w)
                    if k0 == 1024:
                        sink(c, c + 1, t, y[c])
                    yield

    def phase3_mm1(first):
        marking = []
        mm = mm1_first(marking)
        emit(p3pre(0))
        sync('w1a' if first else None)
        if first:
            b1f = b1v[...].astype(f32).reshape(1, F)
            b1[...] = jnp.broadcast_to(b1f, (8, F))
            b1c[...] = jnp.broadcast_to(b1f[:, F - 128:F], (128, 128)).T[64:128]
            b2[...] = jnp.broadcast_to(b2v[...].astype(f32).reshape(1, S), (8, S))
        emit(p3dot(0))
        sync()
        emit(p3post(0), woven(take(mm, 52), chain(p3pre(1), p3pre(2), p3pre(3)), 48 / 50))
        sync('w1b' if first else None)
        emit(p3dot(1), p3dot(2), p3dot(3))
        marking.append(True)
        emit(take(mm, 3), woven(mm, chain(p3post(1), p3post(2), p3post(3)), 6.0))
        tok.clear()
        for i, c0 in enumerate(range(0, FM, 256)):
            mm1_rest(c0, min(FM, c0 + 256))
            if i == 5:
                mm1_tail()
            if first and i == 3:
                sync('w2')

    def mm2_phase1():
        for i, pair in enumerate(([1, 5], [9, 13], [2, 6], [10, 14], [3, 7], [11, 15])):
            mm2(pair, to_state)
            if i in (2, 4):
                emit(p1dot(i // 2))
        mm = chain(mm2_fine([0, 4], to_state), mm2_fine([8, 12], to_state))
        emit(take(mm, 4), p1dot(3), take(mm, 2))
        sync()
        emit(woven(mm, chain(p1post(1), p1post(2), p1post(3)), 0.9), p1dot(0), p1post(0))
        sync()

    outs = []

    def flush(t0, t1):
        for t in range(t0, t1):
            xin[tl(t), :] = stage[t].astype(bf16).T
        cp = pltpu.make_async_copy(xin.at[128 * t0:128 * t1], o_hbm.at[128 * t0:128 * t1],
                                   sems.at[len(groups) + len(outs)])
        cp.start()
        outs.append(cp)

    def mm2_output():
        for c in range(7):
            mm2([2 * c, 2 * c + 1], to_output)
            if c == 5:
                flush(0, 10)
                sync()
        mm = mm2_fine([14, 15], to_output)
        emit(take(mm, 25))
        flush(10, 15)
        sync()
        emit(mm)
        flush(15, 16)

    build_tables()
    sync('wr0')
    emit(wstep1(wr, wn0, 0, 128), wstep2a(wn0, wpr))
    sync('wr1')
    wp = chain(wstep1(wr, wn0, 128, 321), wstep2b(wn0, wpr))
    emit(take(wp, 20))
    sync('x1')
    emit(woven(wp, xload(1), 0.5))
    sync('wi0')
    emit(woven(chain(p1cast(1), p1dot(1)), wstep1(wi, wn1, 0, 128), 1.0))
    sync('x2')
    emit(woven(xload(2), woven(p1post(1), wstep2a(wn1, wpi), 0.9), 4.5))
    sync('x3')
    emit(woven(xload(3), chain(p1cast(2), p1dot(2)), 2.3))
    sync()
    emit(woven(chain(p1cast(3), p1dot(3)), p1post(2), 2.0))
    sync('wi1')
    emit(woven(wstep1(wi, wn1, 128, 321), p1post(3), 2.3))
    sync('x0')
    emit(woven(chain(xload(0), p1cast(0), p1dot(0)), wstep2b(wn1, wpi), 1.3), p1post(0))
    sync('ms0')
    for layer in range(2):
        phase2(layer == 0)
        phase3_mm1(layer == 0)
        if layer == 0:
            mm2_phase1()
        else:
            mm2_output()
    for cp in outs:
        cp.wait()


@jax.jit
def pallas_interleave_layers__spectral_gfnet__mixer_token_mlp__prompt_kernel(A_x, A_w_r, A_w_i, B_x, B_w1, B_b1, B_w2, B_b2):
    gi, ms = _tables()
    args = (A_x.reshape(S, D), A_w_r.T, A_w_i.T, B_w1.T, B_b1, B_w2, B_b2, gi, ms)
    vmem = pltpu.VMEM
    out = pl.pallas_call(
        _kernel,
        out_shape=jax.ShapeDtypeStruct((S, D), bf16),
        in_specs=[pl.BlockSpec(memory_space=pltpu.HBM)] * len(args),
        out_specs=pl.BlockSpec(memory_space=pltpu.HBM),
        scratch_shapes=[
            vmem((S, D), bf16), vmem((321, S), bf16), vmem((321, S), bf16),
            vmem((F, S), bf16), vmem((F,), bf16), vmem((F, S), bf16), vmem((S,), bf16),
            vmem((5, 64, 128), u32), vmem((5, 64, 128), u32),
            vmem((16, 5, 64, 128), u32), vmem((200, 128), u32),
            vmem((16, 64, 321), u32), vmem((16, 64, 321), u32),
            vmem((R + 8, S), f32), vmem((R + 8, S), f32),
            vmem((D, S), f32), vmem((16, D, 128), f32),
            vmem((R, S), f32), vmem((R, S), f32),
            vmem((D // 2, S), u32), vmem((D // 2, F), u32), vmem((D, FM), f32),
            vmem((D // 2, S), u32), vmem((656, S), f32), vmem((80, S), f32),
            vmem((8, F), f32), vmem((8, S), f32), vmem((64, 128), f32),
            vmem((8, 128), i32),
            pltpu.SemaphoreType.DMA((16,)), pltpu.SemaphoreType.REGULAR,
        ],
        compiler_params=pltpu.CompilerParams(vmem_limit_bytes=100 * 1024 * 1024),
    )(*args)
    return out.reshape(1, S, D)
```

```python
import math

import numpy as np
import jax
import jax.numpy as jnp
from jax import lax
import jax.experimental.pallas as pl
import jax.experimental.pallas.tpu as pltpu

S, D, F = 2048, 640, 1728
FM = 1664
R = 328
EPS = 1e-5
f32, bf16, u32, i32 = jnp.float32, jnp.bfloat16, jnp.uint32, jnp.int32
NT = (((1,), (1,)), ((), ()))

C1, C2 = float(np.cos(2 * np.pi / 5)), float(np.cos(4 * np.pi / 5))
S1, S2 = float(np.sin(2 * np.pi / 5)), float(np.sin(4 * np.pi / 5))
EXTRA = {0: 64, 4: 192, 1: 320}


def _shuffle(rows):
    return np.asarray(rows).reshape(-1, 2, 8).transpose(0, 2, 1).reshape(-1)


def _pack_rows(a):
    b = np.asarray(a, dtype=np.float32).astype(bf16).view(np.uint16).astype(np.uint32)
    return b[..., 0::2, :] | (b[..., 1::2, :] << 16)


def _tables():
    gi = np.zeros((5, 128, 128))
    lpos = _shuffle(_shuffle(np.arange(64)))
    for c in range(5):
        d = c + 5 * np.arange(128)
        for p in range(64):
            gi[c, :, 2 * p] = (1 if lpos[p] == 0 else 2) * np.cos(2 * np.pi * d * lpos[p] / 640)
            gi[c, :, 2 * p + 1] = -2 * np.sin(2 * np.pi * d * lpos[p] / 640)
        gi[c, :, 1] = (-1.0) ** np.arange(128)
    gi = gi / (D * S)
    k2 = _shuffle(np.arange(128))
    j = np.arange(64)
    ms = np.zeros((16, 5, 128, 128))
    for k1 in range(16):
        m = ms[4 * (k1 % 4) + k1 // 4]
        a = 2 * np.pi * (np.outer(np.arange(128), k1 + 16 * k2) % S) / S
        m[0], m[1], m[2] = np.cos(a), -np.sin(a) - np.cos(a), np.cos(a) - np.sin(a)
        te, to = a[0::2, :64], a[1::2, :64]
        m[3, 2 * j] = np.concatenate([np.cos(te), -np.sin(te)], 1)
        m[3, 2 * j + 1] = np.concatenate([np.sin(te), np.cos(te)], 1)
        m[4, 2 * j + 1] = np.concatenate([np.cos(to), np.sin(to)], 1)
        m[4, (2 * j + 2) % 128] = np.concatenate([np.sin(to), -np.cos(to)], 1)
    return _pack_rows(gi), _pack_rows(ms)


def _tw16(x, e):
    r, m = x
    e = e % 16
    h = float(np.sqrt(0.5))
    if e == 0:
        return x
    if e == 4:
        return (m, -r)
    if e == 12:
        return (-m, r)
    if e == 2:
        return ((r + m) * h, (m - r) * h)
    if e == 6:
        return ((m - r) * h, (r + m) * (-h))
    if e == 14:
        return ((r - m) * h, (r + m) * h)
    if e == 10:
        return ((r + m) * (-h), (r - m) * h)
    c = float(np.cos(2 * np.pi * e / 16))
    s = float(-np.sin(2 * np.pi * e / 16))
    return (r * c - m * s, r * s + m * c)


def _half4(x, odd, inv):
    (ar, ai), (br, bi), (cr, ci), (dr, di) = x
    if not odd:
        t0 = (ar + cr, ai + ci)
        t2 = (br + dr, bi + di)
        return [(t0[0] + t2[0], t0[1] + t2[1]), (t0[0] - t2[0], t0[1] - t2[1])]
    t1 = (ar - cr, ai - ci)
    t3 = (br - dr, bi - di)
    ya = (t1[0] + t3[1], t1[1] - t3[0])
    yb = (t1[0] - t3[1], t1[1] + t3[0])
    return [yb, ya] if inv else [ya, yb]


def _fft4(x, inv):
    e, o = _half4(x, 0, inv), _half4(x, 1, inv)
    return [e[0], o[0], e[1], o[1]]


def _r5half(a0, p1, p2, m1, m2):
    q = p1 + p2
    r = (p1 - p2) * ((C1 - C2) / 2)
    b = a0 - q * 0.25
    return a0 + q, b + r, b - r, m1 * S1 + m2 * S2, m1 * S2 - m2 * S1


def _fold8(x):
    parts = [x[8 * i:8 * (i + 1)] for i in range(x.shape[0] // 8)]
    while len(parts) > 1:
        parts = [parts[i] + parts[i + 1] if i + 1 < len(parts) else parts[i] for i in range(0, len(parts), 2)]
    return parts[0]


def _pk(x):
    return pltpu.bitcast(x.astype(bf16), u32)


def _ipk(a, b):
    return pltpu.pack_elementwise([a, b], packed_dtype=bf16).astype(u32)


def _upk(x):
    return pltpu.bitcast(x, bf16)


def _mm(a, b):
    return jnp.dot(a, b, preferred_element_type=f32)


def _mm_nt(a, b):
    return lax.dot_general(a, b, NT, preferred_element_type=f32)


def _iota(shape, axis):
    return lax.broadcasted_iota(i32, shape, axis)


def tl(t):
    return slice(128 * t, 128 * (t + 1))


def chain(*gens):
    for gen in gens:
        yield from gen


def take(gen, n):
    for _ in range(n):
        next(gen)
        yield


def woven(main, side, ratio):
    credit = 0.0
    for _ in main:
        credit += ratio
        while credit >= 1.0:
            next(side, None)
            credit -= 1.0
        yield
    yield from side


def emit(*gens):
    for _ in chain(*gens):
        pass


def _kernel(x_hbm, wr_hbm, wi_hbm, w1t_hbm, b1_hbm, w2_hbm, b2_hbm, gi_hbm, ms_hbm,
            o_hbm,
            xin, wr, wi, w1t, b1v, w2, b2v, g, gi, ms, pm, wn0, wn1, wpr, wpi, xt, stage, pr, pi, hb, u, acc,
            vv, vf, cs, b1, b2, b1c, zb, sems, rsem):
    groups = {}

    def dma(name, pairs):
        sem = sems.at[len(groups)]
        groups[name] = [pltpu.make_async_copy(src, dst, sem) for src, dst in pairs]

    def xtiles(a):
        return [(x_hbm.at[tl(a + 4 * b)], xin.at[tl(a + 4 * b)]) for b in range(4)]

    def w1cols(r0, r1):
        return [(w1t_hbm.at[r0:r1, 512 * b + 128:512 * (b + 1)], w1t.at[r0:r1, 512 * b + 128:512 * (b + 1)])
                for b in range(4)]

    dma('wr0', [(wr_hbm.at[0:128], wr.at[0:128])])
    dma('wr1', [(wr_hbm.at[128:321], wr.at[128:321])])
    dma('x1', xtiles(1))
    dma('wi0', [(wi_hbm.at[0:128], wi.at[0:128])])
    dma('x2', xtiles(2))
    dma('x3', xtiles(3))
    dma('wi1', [(wi_hbm.at[128:321], wi.at[128:321])])
    dma('x0', xtiles(0))
    dma('ms0', [(ms_hbm.at[0:8], ms.at[0:8])])
    dma('ms1', [(ms_hbm.at[8:16], ms.at[8:16])])
    dma('w1a', [(gi_hbm, gi), (b1_hbm, b1v), (b2_hbm, b2v)]
        + [(w1t_hbm.at[:, tl(4 * b)], w1t.at[:, tl(4 * b)]) for b in range(4)])
    dma('w1b', w1cols(0, 1024))
    dma('w2', w1cols(1024, F) + [(w2_hbm, w2)])
    for copies in groups.values():
        for cp in copies:
            cp.start()

    def sync(name=None):
        if name is None:
            pl.semaphore_signal(rsem, 1)
            pl.semaphore_wait(rsem, 1)
        else:
            for cp in groups[name]:
                cp.wait()

    pltpu.store(zb, jnp.zeros((8, 128), i32), mask=_iota((8, 128), 1) < 4096)
    tok = []

    def pin(v):
        if len(tok) < 2:
            return v
        return pltpu.bitcast(pltpu.bitcast(v, i32) | (pltpu.bitcast(tok[-2], i32) & zb[...]), f32)

    nat = set(range(16))

    def xread(c, t):
        return stage[t, pl.ds(c, 128, stride=5), :] if t in nat else xt[tl(c), tl(t)]

    def pick(nrows, colfn):
        halves = []
        for h in range(2):
            row = 2 * _iota((nrows // 2, 128), 0) + h
            halves.append(jnp.where(_iota((nrows // 2, 128), 1) == colfn(row), 1.0, 0.0))
        return halves

    def build_tables():
        def lsh(p):
            return (p & ~15) + 8 * (p & 1) + ((p & 15) >> 1)

        p128 = pick(128, lambda r: (r >> 3) + 16 * (r & 7))
        pm[0:64, :] = _ipk(*p128)
        pm[64:128, :] = _ipk(-p128[0], -p128[1])
        pm[128:200, :] = _ipk(*pick(144, lambda r: jnp.where(r < 64, lsh(r), jnp.where(
            (r == 64) | (r == 130), 64, jnp.where(r < 128, 128 - lsh(r - 64), -1)))))
        for c in range(5):
            halves = []
            for h in range(2):
                row = 2 * _iota((64, 128), 0) + h
                d = c + 5 * _iota((64, 128), 1)
                idx = jnp.where(row < 64, d * row, jnp.where(row == 64, (d - c) * 64, d * (row - 64) + 160))
                idx = idx - 640 * (((idx >> 7) * 52429) >> 18)
                idx = jnp.where(idx > 320, 640 - idx, idx)
                neg = idx > 160
                x2 = jnp.where(neg, 320 - idx, idx).astype(f32) * float(2 * np.pi / 640)
                x2 = x2 * x2
                cosv = jnp.full((64, 128), 1.0 / math.factorial(14), f32)
                for n in range(12, -1, -2):
                    cosv = 1.0 / math.factorial(n) - x2 * cosv
                halves.append(jnp.where(neg, -cosv, cosv))
            g[c] = _ipk(*halves)

    def wstep1(wsrc, wn, f0, f1):
        for t2 in range(8):
            p0 = 64 if (wsrc is wi and t2 < 4) else 0
            o = [_mm_nt(_upk(pm[p0:p0 + 64, :]), wsrc[f0:f1, tl(t)]) for t in (2 * t2, 2 * t2 + 1)]
            pk = _ipk(o[0], o[1])
            for k in range(16):
                wn[k, 8 * t2:8 * (t2 + 1), f0:f1] = pk[8 * k:8 * (k + 1)]
            yield

    def wstep2a(wn, wdst):
        for k in range(16):
            oa = _mm_nt(_upk(pm[128:192, :]), _upk(wn[k, :, 0:128]))
            wdst[0:64, tl(k)] = oa[0:64]
            wdst[256:320, tl(k)] = oa[64:128]
            yield

    def wstep2b(wn, wdst):
        top = _iota((8, 128), 0) == 0
        for k in range(16):
            ob = _mm_nt(_upk(pm[128:192, :]), _upk(wn[k, :, 128:256]))
            oc = _mm_nt(_upk(jnp.concatenate([pm[128:160, 0:65], pm[192:200, 0:65]], axis=0)), _upk(wn[k, :, 256:321]))
            j4 = wdst[256:264, tl(k)]
            wdst[64:264, tl(k)] = jnp.concatenate(
                [ob[0:64], oc[0:64], jnp.where(top, oc[0:8], ob[64:72]), ob[72:128], jnp.where(top, ob[0:8], j4)],
                axis=0)
            wdst[320:336, tl(k)] = jnp.concatenate(
                [jnp.where(top, j4, oc[64:72]), jnp.where(top, ob[64:72], 0.0)], axis=0)
            yield

    nsum, shift, ready = {}, {}, {}

    def addsum(t, x):
        n = nsum.get(t, 0)
        cs[16 * n:16 * n + 16, tl(t)] = jnp.concatenate([_fold8(x), _fold8(x * x)], axis=0)
        nsum[t] = n + 1

    def shifted(t, x):
        if t not in nsum:
            shift[t] = x[0:1]
        return x - shift[t]

    def stats(t, double):
        n = nsum.pop(t)
        sq = cs[0:16, tl(t)]
        for i in range(1, n):
            sq = sq + cs[16 * i:16 * i + 16, tl(t)]
        m = jnp.sum(sq[0:8], axis=0, keepdims=True) * (1.0 / D)
        v = jnp.maximum(jnp.sum(sq[8:16], axis=0, keepdims=True) * (1.0 / D) - m * m, 0.0)
        if double:
            return m, lax.rsqrt(v + EPS * (v + EPS))
        return m, lax.rsqrt(v + EPS)

    def xload(a):
        for b in range(4):
            t = a + 4 * b
            x = xin[tl(t), :].T.astype(f32)
            stage[t] = x
            addsum(t, x)
            yield

    def p1cast(a):
        for b in range(4):
            m, r = stats(a + 4 * b, False)
            ready[a + 4 * b] = (None, r)
            for c in range(5):
                vv[64 * c:64 * (c + 1), tl(4 * a + b)] = _pk(xread(c, a + 4 * b) - m)
            yield

    def p1dot(a):
        st = [ready.pop(a + 4 * b) if a + 4 * b in ready else stats(a + 4 * b, False) for b in range(4)]
        r = jnp.concatenate([s[1] for s in st], axis=1)
        row = _iota((8, 512), 0)
        dc = er = ei = None
        if st[0][0] is not None:
            dc = jnp.where(row == 0, jnp.concatenate([s[0] for s in st], axis=1) * 128.0, 0.0)
        for c in range(5):
            y = _mm(_upk(g[c]), _upk(vv[64 * c:64 * (c + 1), 512 * a:512 * (a + 1)]))
            if dc is not None:
                y = jnp.concatenate([y[0:8] - dc, y[8:]], axis=0)
            y = y * r
            u64 = jnp.broadcast_to(y[64:65], (8, 512))
            cr = ci = jnp.zeros((8, 512), f32)
            for i, f in EXTRA.items():
                cr = jnp.where(row == i, float(np.cos(2 * np.pi * c * f / 640)), cr)
                ci = jnp.where(row == i, float(-np.sin(2 * np.pi * c * f / 640)), ci)
            er = u64 * cr if er is None else er + u64 * cr
            if c > 0:
                ei = u64 * ci if ei is None else ei + u64 * ci
            vf[128 * c:128 * (c + 1), 512 * a:512 * (a + 1)] = jnp.concatenate(
                [y[0:64], jnp.where(row == 0, 0.0, y[64:72]), y[72:]], axis=0)
            if c == 4:
                vf[640:656, 512 * a:512 * (a + 1)] = jnp.concatenate([er, ei], axis=0)
            yield

    def p1post(a):
        def ld(c, r0, b):
            return vf[128 * c + r0:128 * c + r0 + 8, tl(4 * a + b)]
        for gq in (0, 1, 8, 2, 3, 4, 5, 6, 7):
            for odd in range(2):
                if gq < 8:
                    y = [_half4([(ld(c, 8 * gq, b), ld(c, 64 + 8 * gq, b)) for b in range(4)], odd, False)
                         for c in range(5)]
                else:
                    y = [_half4([(ld(5, 0, b), ld(5, 8, b)) for b in range(4)], odd, False)]
                for hi in range(2):
                    kb = odd + 2 * hi
                    if gq < 8:
                        ar = [y[c][hi][0] for c in range(5)]
                        ai = [y[c][hi][1] for c in range(5)]
                        x0r, a1r, a2r, b1r, b2r = _r5half(ar[0], ar[1] + ar[4], ar[2] + ar[3], ar[1] - ar[4],
                                                          ar[2] - ar[3])
                        x0i, a1i, a2i, b1i, b2i = _r5half(ai[0], ai[1] + ai[4], ai[2] + ai[3], ai[1] - ai[4],
                                                          ai[2] - ai[3])
                        xs = [(x0r, x0i), (a1r + b1i, a1i - b1r), (a2r + b2i, a2i - b2r),
                              (b2i - a2r, a2i + b2r), (b1i - a1r, a1i + b1r)]
                    else:
                        xs = [y[0][hi]]
                    for j in range(len(xs)):
                        r0 = 64 * j + 8 * gq if gq < 8 else 320
                        kq = kb if j < 3 else (4 - kb) % 4
                        yr, yi = _tw16(xs[j], a * kq)
                        pr[r0:r0 + 8, tl(4 * kq + a)] = yr
                        pi[r0:r0 + 8, tl(4 * kq + a)] = yi
                yield

    chunks = [(r0, min(R, r0 + 16)) for r0 in range(0, R, 16)]
    edges = [0, 4, 8, 13, 17, 21]
    units = [(kb, chunks[e0:e1]) for kb in range(4) for e0, e1 in zip(edges[:-1], edges[1:])]
    lane = _iota((8, 128), 1)

    def pk16(v):
        return _ipk(v[0:8], v[8:16] if v.shape[0] == 16 else jnp.zeros_like(v))

    def rows(parts, h):
        return _upk(jnp.concatenate([p[h] for p in parts], axis=0))

    def phase2(first):
        even, low = (lane & 1) == 0, lane < 64
        lhs, eo, z, out = {}, {}, {}, {}

        def pre(i):
            kb, chs = units[i]
            for r0, r1 in chs:
                t4 = _fft4([(pr[r0:r1, tl(4 * kb + a)], pi[r0:r1, tl(4 * kb + a)]) for a in range(4)], False)
                for ka in range(4):
                    re, im = pk16(t4[ka][0]), pltpu.roll(pk16(t4[ka][1]), 1, 1)
                    lhs.setdefault((i, ka), []).append((jnp.where(even, re, im), jnp.where(even, im, re)))
                yield

        def fwd(i, ka):
            m = ms.at[4 * units[i][0] + ka]
            parts = lhs.pop((i, ka))
            eo[i, ka] = [_mm(rows(parts, h), _upk(m[3 + h])) for h in range(2)]

        def filt(i, ka):
            kb, chs = units[i]
            e, o = eo.pop((i, ka))
            z[i, ka] = []
            for j, (r0, _) in enumerate(chs):
                q = slice(16 * j, 16 * j + 16)
                p_, q_ = e[q] + o[q], pltpu.roll(e[q] - o[q], 64, 1)
                w_r, w_i = wpr[r0:r0 + 16, tl(4 * ka + kb)], wpi[r0:r0 + 16, tl(4 * ka + kb)]
                p_, q_ = p_ * w_r + q_ * w_i, q_ * w_r - p_ * w_i
                pp, qp = pk16(p_), pk16(q_)
                z[i, ka].append((pk16(p_ + q_), jnp.where(low, pp, qp), jnp.where(low, qp, pp)))

        def inv(i, ka):
            m = ms.at[4 * units[i][0] + ka]
            parts = z.pop((i, ka))
            k1, k2, k3 = [_mm_nt(rows(parts, h), _upk(m[(0, 2, 1)[h]])) for h in range(3)]
            out.setdefault(i, []).append((k1 + k3, k1 - k2))

        def post(i, h):
            kb, chs = units[i]
            (ar, ai), (br, bi) = out.pop(i)
            for j, (r0, r1) in enumerate(chs):
                q = slice(16 * j, 16 * j + r1 - r0)
                pr[r0:r1, tl(4 * kb + 2 * h)] = ar[q] + br[q]
                pi[r0:r1, tl(4 * kb + 2 * h)] = ai[q] + bi[q]
                pr[r0:r1, tl(4 * kb + 2 * h + 1)] = ar[q] - br[q]
                pi[r0:r1, tl(4 * kb + 2 * h + 1)] = ai[q] - bi[q]

        steps = [(i, ka) for i in range(len(units)) for ka in (0, 2, 1, 3)]
        lag = 5
        emit(pre(0))
        gpre = iter(())
        for s in range(len(steps) + lag):
            if s < len(steps):
                i, ka = steps[s]
                if ka == 0:
                    emit(gpre)
                    if first and i == len(units) // 2:
                        sync('ms1')
                    gpre = pre(i + 1) if i + 1 < len(units) else iter(())
                fwd(i, ka)
            if 1 <= s <= len(steps):
                filt(*steps[s - 1])
            next(gpre, None)
            if s >= lag:
                i, ka = steps[s - lag]
                inv(i, ka)
                if ka >= 2:
                    post(i, ka - 2)
            if s % 4 == 2:
                next(gpre, None)

    def p3pre(a):
        row = _iota((8, 128), 0)

        def ld(rs, kb):
            c0, c1 = tl(4 * kb + a % 2), tl(4 * kb + 2 + a % 2)
            ar, ai, br, bi = pr[rs, c0], pi[rs, c0], pr[rs, c1], pi[rs, c1]
            v = ((ar + br, ai + bi) if a == 0 else (ar - bi, ai + br) if a == 1 else
                 (ar - br, ai - bi) if a == 2 else (ar + bi, ai - br))
            return _tw16(v, -a * kb)
        ex = _fft4([ld(slice(320, 328), kb) for kb in range(4)], True)
        for gq in range(8):
            for odd in range(2):
                y = [_half4([ld(slice(64 * j + 8 * gq, 64 * j + 8 * gq + 8), kb) for kb in range(4)], odd, True)
                     for j in range(5)]
                for hi in range(2):
                    b = odd + 2 * hi
                    yr = [y[j][hi][0] for j in range(5)]
                    yi = [y[j][hi][1] for j in range(5)]
                    v0r, a1r, a2r, b1r, b2r = _r5half(yr[0], yr[1] - yr[4], yr[2] - yr[3], yr[1] + yr[4],
                                                      yr[2] + yr[3])
                    v0i, a1i, a2i, b1i, b2i = _r5half(yi[0], yi[1] + yi[4], yi[2] + yi[3], yi[1] - yi[4],
                                                      yi[2] - yi[3])
                    vs = [(v0r, v0i), (a1r - b1i, a1i + b1r), (a2r - b2i, a2i + b2r), (a2r + b2i, a2i - b2r),
                          (a1r + b1i, a1i - b1r)]
                    for c in range(5):
                        vr, vi = vs[c]
                        if gq == 0:
                            er, ei = ex[b]
                            th1, th3 = 2 * np.pi * c / 10, 2 * np.pi * 3 * c / 10
                            t64 = (er[0:1] * float(2 * np.cos(th1)) - ei[0:1] * float(2 * np.sin(th1))
                                   + er[1:2] * float(2 * np.cos(th3)) - ei[1:2] * float(2 * np.sin(th3))
                                   + er[4:5] * float((-1) ** c))
                            vi = jnp.where(row == 0, jnp.broadcast_to(t64, (8, 128)), vi)
                        vv[64 * c + 8 * gq:64 * c + 8 * gq + 8, tl(4 * a + b)] = _ipk(vr, vi)
                yield

    def p3dot(a):
        for c in range(5):
            y = _mm(_upk(gi[c]), _upk(vv[64 * c:64 * (c + 1), 512 * a:512 * (a + 1)]))
            for b in range(4):
                xn = xread(c, a + 4 * b) + y[:, tl(b)]
                xt[tl(c), tl(a + 4 * b)] = xn
                addsum(a + 4 * b, shifted(a + 4 * b, xn))
            if c == 4:
                nat.difference_update(a + 4 * b for b in range(4))
            yield

    def p3post(a):
        for b in range(4):
            t = a + 4 * b
            m, r = stats(t, True)
            m8 = jnp.broadcast_to(m + shift.pop(t), (8, 128))
            for c in range(5):
                xc = (xt[tl(c), tl(t)].reshape(16, 8, 128) - pin(m8)[None]).reshape(128, 128)
                hb[64 * c:64 * (c + 1), tl(4 * a + b)] = _pk(xc * r)
                yield

    def cat(ref, rs, tiles):
        return jnp.concatenate([ref[rs, tl(t)] for t in tiles], axis=1)

    def mm1_first(marking):
        for c0 in range(0, FM, 128):
            w = cat(w1t, slice(c0, c0 + 128), [0, 4, 8, 12])
            for c in range(5):
                y = _mm_nt(_upk(hb[64 * c:64 * (c + 1), 0:512]), w)
                acc[tl(c), c0:c0 + 128] = y
                if marking:
                    tok.append(y[0:8])
                yield

    def mm1_rest(c0, c1):
        tiles = [a + 4 * b for a in range(1, 4) for b in range(4)]
        h = _mm_nt(_upk(hb[:, 512:]), cat(w1t, slice(c0, c1), tiles)) + acc[:, c0:c1]
        u[:, c0:c1] = _pk(jax.nn.gelu(h + b1[0:1, c0:c1], approximate=True))

    def mm1_tail():
        tiles = [a + 4 * b for a in range(4) for b in range(4)]
        h = _mm_nt(cat(w1t, slice(FM, F), tiles), _upk(hb[...])) + jnp.concatenate([b1c[...]] * 5, axis=1)
        u[:, FM:F] = _pk(jax.nn.gelu(h, approximate=True).T)

    def to_state(c0, c1, t, y):
        xn = xt[128 * c0:128 * c1, tl(t)] + y + b2[0:1, tl(t)]
        xt[128 * c0:128 * c1, tl(t)] = xn
        xs = shifted(t, xn)
        vv[64 * c0:64 * c1, tl(4 * (t % 4) + t // 4)] = _pk(xs)
        addsum(t, xs)

    def to_output(c0, c1, t, y):
        xn = xt[128 * c0:128 * c1, tl(t)] + y + b2[0:1, tl(t)]
        for c in range(c0, c1):
            stage[t, pl.ds(c, 128, stride=5), :] = xn[tl(c - c0)]

    def mm2(tiles, sink):
        y = _mm(_upk(u[...]), cat(w2, slice(None), tiles))
        for i, t in enumerate(tiles):
            sink(0, 5, t, y[:, tl(i)])

    def mm2_fine(tiles, sink):
        w = cat(w2, slice(1536, F), tiles)
        rem = []
        for c in range(5):
            rem.append(_mm(_upk(u[64 * c:64 * (c + 1), 1536:F]), w))
            yield
        for i, t in enumerate(tiles):
            y = [r[:, tl(i)] for r in rem]
            for k0 in range(0, 1536, 512):
                w = w2[k0:k0 + 512, tl(t)]
                for c in range(5):
                    y[c] = y[c] + _mm(_upk(u[64 * c:64 * (c + 1), k0:k0 + 512]), w)
                    if k0 == 1024:
                        sink(c, c + 1, t, y[c])
                    yield

    def phase3_mm1(first):
        marking = []
        mm = mm1_first(marking)
        emit(p3pre(0))
        sync('w1a' if first else None)
        if first:
            b1f = b1v[...].astype(f32).reshape(1, F)
            b1[...] = jnp.broadcast_to(b1f, (8, F))
            b1c[...] = jnp.broadcast_to(b1f[:, F - 128:F], (128, 128)).T[64:128]
            b2[...] = jnp.broadcast_to(b2v[...].astype(f32).reshape(1, S), (8, S))
        emit(p3dot(0))
        sync()
        emit(p3post(0), woven(take(mm, 52), chain(p3pre(1), p3pre(2), p3pre(3)), 48 / 50))
        sync('w1b' if first else None)
        emit(p3dot(1), p3dot(2), p3dot(3))
        marking.append(True)
        emit(take(mm, 3), woven(mm, chain(p3post(1), p3post(2), p3post(3)), 6.0))
        tok.clear()
        for i, c0 in enumerate(range(0, FM, 256)):
            mm1_rest(c0, min(FM, c0 + 256))
            if i == 5:
                mm1_tail()
            if first and i == 3:
                sync('w2')

    def mm2_phase1():
        for i, pair in enumerate(([1, 5], [9, 13], [2, 6], [10, 14], [3, 7], [11, 15])):
            mm2(pair, to_state)
            if i in (2, 4):
                emit(p1dot(i // 2))
        mm = chain(mm2_fine([0, 4], to_state), mm2_fine([8, 12], to_state))
        emit(take(mm, 4), p1dot(3), take(mm, 2))
        sync()
        emit(woven(mm, chain(p1post(1), p1post(2), p1post(3)), 0.9), p1dot(0), p1post(0))
        sync()

    outs = []

    def flush(t0, t1):
        for t in range(t0, t1):
            xin[tl(t), :] = stage[t].astype(bf16).T
        cp = pltpu.make_async_copy(xin.at[128 * t0:128 * t1], o_hbm.at[128 * t0:128 * t1],
                                   sems.at[len(groups) + len(outs)])
        cp.start()
        outs.append(cp)

    def mm2_output():
        for c in range(7):
            mm2([2 * c, 2 * c + 1], to_output)
            if c == 5:
                flush(0, 10)
                sync()
        mm = mm2_fine([14, 15], to_output)
        emit(take(mm, 25))
        flush(10, 15)
        sync()
        emit(mm)
        flush(15, 16)

    build_tables()
    sync('wr0')
    emit(wstep1(wr, wn0, 0, 128), wstep2a(wn0, wpr))
    sync('wr1')
    wp = chain(wstep1(wr, wn0, 128, 321), wstep2b(wn0, wpr))
    emit(take(wp, 20))
    sync('x1')
    emit(woven(wp, xload(1), 0.5))
    sync('wi0')
    emit(woven(chain(p1cast(1), p1dot(1)), wstep1(wi, wn1, 0, 128), 1.0))
    sync('x2')
    emit(woven(xload(2), woven(p1post(1), wstep2a(wn1, wpi), 0.9), 4.5))
    sync('x3')
    emit(woven(xload(3), chain(p1cast(2), p1dot(2)), 2.3))
    sync()
    emit(woven(chain(p1cast(3), p1dot(3)), p1post(2), 2.0))
    sync('wi1')
    emit(woven(wstep1(wi, wn1, 128, 321), p1post(3), 2.3))
    sync('x0')
    emit(woven(chain(xload(0), p1cast(0), p1dot(0)), wstep2b(wn1, wpi), 1.3), p1post(0))
    sync('ms0')
    for layer in range(2):
        phase2(layer == 0)
        phase3_mm1(layer == 0)
        if layer == 0:
            mm2_phase1()
        else:
            mm2_output()
    for cp in outs:
        cp.wait()


@jax.jit
def pallas_interleave_layers__spectral_gfnet__mixer_token_mlp__prompt_kernel(A_x, A_w_r, A_w_i, B_x, B_w1, B_b1, B_w2, B_b2):
    gi, ms = _tables()
    args = (A_x.reshape(S, D), A_w_r.T, A_w_i.T, B_w1.T, B_b1, B_w2, B_b2, gi, ms)
    vmem = pltpu.VMEM
    out = pl.pallas_call(
        _kernel,
        out_shape=jax.ShapeDtypeStruct((S, D), bf16),
        in_specs=[pl.BlockSpec(memory_space=pltpu.HBM)] * len(args),
        out_specs=pl.BlockSpec(memory_space=pltpu.HBM),
        scratch_shapes=[
            vmem((S, D), bf16), vmem((321, S), bf16), vmem((321, S), bf16),
            vmem((F, S), bf16), vmem((F,), bf16), vmem((F, S), bf16), vmem((S,), bf16),
            vmem((5, 64, 128), u32), vmem((5, 64, 128), u32),
            vmem((16, 5, 64, 128), u32), vmem((200, 128), u32),
            vmem((16, 64, 321), u32), vmem((16, 64, 321), u32),
            vmem((R + 8, S), f32), vmem((R + 8, S), f32),
            vmem((D, S), f32), vmem((16, D, 128), f32),
            vmem((R, S), f32), vmem((R, S), f32),
            vmem((D // 2, S), u32), vmem((D // 2, F), u32), vmem((D, FM), f32),
            vmem((D // 2, S), u32), vmem((656, S), f32), vmem((80, S), f32),
            vmem((8, F), f32), vmem((8, S), f32), vmem((64, 128), f32),
            vmem((8, 128), i32),
            pltpu.SemaphoreType.DMA((16,)), pltpu.SemaphoreType.REGULAR,
        ],
        compiler_params=pltpu.CompilerParams(vmem_limit_bytes=100 * 1024 * 1024),
    )(*args)
    return out.reshape(1, S, D)
```

```python
import math

import numpy as np
import jax
import jax.numpy as jnp
from jax import lax
import jax.experimental.pallas as pl
import jax.experimental.pallas.tpu as pltpu

S, D, F = 2048, 640, 1728
FM = 1664
R = 328
EPS = 1e-5
TMP_ROWS, TMP_TILES = 1024, 16
f32, bf16, u32, i32 = jnp.float32, jnp.bfloat16, jnp.uint32, jnp.int32
NT = (((1,), (1,)), ((), ()))

C1, C2 = float(np.cos(2 * np.pi / 5)), float(np.cos(4 * np.pi / 5))
S1, S2 = float(np.sin(2 * np.pi / 5)), float(np.sin(4 * np.pi / 5))
EXTRA = (64, 192, 320)


def _pack_rows(a):
    b = np.asarray(a, dtype=np.float32).astype(bf16).view(np.uint16).astype(np.uint32)
    return b[..., 0::2, :] | (b[..., 1::2, :] << 16)


def _tables():
    gi = np.zeros((5, 128, 128))
    for c in range(5):
        d = c + 5 * np.arange(128)
        for l in range(64):
            gi[c, :, 16 * (l // 8) + l % 8] = (1 if l == 0 else 2) * np.cos(2 * np.pi * d * l / 640)
            gi[c, :, 16 * (l // 8) + 8 + l % 8] = -2 * np.sin(2 * np.pi * d * l / 640)
        gi[c, :, 8] = (-1.0) ** np.arange(128)
    gi = gi / (D * S)
    k2 = np.arange(128)
    j = np.arange(64)
    ms = np.zeros((16, 5, 128, 128))
    for k1 in range(16):
        m = ms[4 * (k1 % 4) + k1 // 4]
        a = 2 * np.pi * (np.outer(np.arange(128), k1 + 16 * k2) % S) / S
        m[0], m[1], m[2] = np.cos(a), -np.sin(a) - np.cos(a), np.cos(a) - np.sin(a)
        te, to = a[0::2, :64], a[1::2, :64]
        m[3, 2 * j] = np.concatenate([np.cos(te), -np.sin(te)], 1)
        m[3, 2 * j + 1] = np.concatenate([np.sin(te), np.cos(te)], 1)
        m[4, 2 * j + 1] = np.concatenate([np.cos(to), np.sin(to)], 1)
        m[4, (2 * j + 2) % 128] = np.concatenate([np.sin(to), -np.cos(to)], 1)
    return _pack_rows(gi), _pack_rows(ms)


def _tw16(x, e):
    r, m = x
    e = e % 16
    h = float(np.sqrt(0.5))
    if e == 0:
        return x
    if e == 4:
        return (m, -r)
    if e == 12:
        return (-m, r)
    if e == 2:
        return ((r + m) * h, (m - r) * h)
    if e == 6:
        return ((m - r) * h, (r + m) * (-h))
    if e == 14:
        return ((r - m) * h, (r + m) * h)
    if e == 10:
        return ((r + m) * (-h), (r - m) * h)
    c = float(np.cos(2 * np.pi * e / 16))
    s = float(-np.sin(2 * np.pi * e / 16))
    return (r * c - m * s, r * s + m * c)


def _half4(x, odd, inv):
    (ar, ai), (br, bi), (cr, ci), (dr, di) = x
    if not odd:
        t0 = (ar + cr, ai + ci)
        t2 = (br + dr, bi + di)
        return [(t0[0] + t2[0], t0[1] + t2[1]), (t0[0] - t2[0], t0[1] - t2[1])]
    t1 = (ar - cr, ai - ci)
    t3 = (br - dr, bi - di)
    ya = (t1[0] + t3[1], t1[1] - t3[0])
    yb = (t1[0] - t3[1], t1[1] + t3[0])
    return [yb, ya] if inv else [ya, yb]


def _fft4(x, inv):
    e, o = _half4(x, 0, inv), _half4(x, 1, inv)
    return [e[0], o[0], e[1], o[1]]


def _r5half(a0, p1, p2, m1, m2):
    q = p1 + p2
    r = (p1 - p2) * ((C1 - C2) / 2)
    b = a0 - q * 0.25
    return a0 + q, b + r, b - r, m1 * S1 + m2 * S2, m1 * S2 - m2 * S1


def _fold8(x):
    parts = [x[8 * i:8 * (i + 1)] for i in range(x.shape[0] // 8)]
    while len(parts) > 1:
        parts = [parts[i] + parts[i + 1] if i + 1 < len(parts) else parts[i] for i in range(0, len(parts), 2)]
    return parts[0]


def _pk(x):
    return pltpu.bitcast(x.astype(bf16), u32)


def _upk(x):
    return pltpu.bitcast(x, bf16)


def _mm(a, b):
    return jnp.dot(a, b, preferred_element_type=f32)


def _mm_nt(a, b):
    return lax.dot_general(a, b, NT, preferred_element_type=f32)


def _iota(shape, axis):
    return lax.broadcasted_iota(i32, shape, axis)


def tl(t):
    return slice(128 * t, 128 * (t + 1))


def chain(*gens):
    for gen in gens:
        yield from gen


def take(gen, n):
    for _ in range(n):
        next(gen)
        yield


def woven(main, side, ratio):
    credit = 0.0
    for _ in main:
        credit += ratio
        while credit >= 1.0:
            next(side, None)
            credit -= 1.0
        yield
    yield from side


def emit(*gens):
    for _ in chain(*gens):
        pass


def _kernel(x_hbm, wr_hbm, wi_hbm, w1t_hbm, b1_hbm, w2_hbm, b2_hbm, gi_hbm, ms_hbm,
            o_hbm,
            xin, wr, wi, w1t, b1v, w2, b2v, g, gi, ms, pm, wn0, wn1, wpr, wpi, xt, stage, pr, pi, hb, u, acc,
            vv, vf, cs, b1, b2, b1c, zb, tmp, sems, rsem):
    groups = {}

    def dma(name, pairs):
        sem = sems.at[len(groups)]
        groups[name] = [pltpu.make_async_copy(src, dst, sem) for src, dst in pairs]

    def xtiles(a):
        return [(x_hbm.at[tl(a + 4 * b)], xin.at[tl(a + 4 * b)]) for b in range(4)]

    def w1cols(r0, r1):
        return [(w1t_hbm.at[r0:r1, 512 * b + 128:512 * (b + 1)], w1t.at[r0:r1, 512 * b + 128:512 * (b + 1)])
                for b in range(4)]

    dma('wr0', [(wr_hbm.at[0:128], wr.at[0:128])])
    dma('wr1', [(wr_hbm.at[128:321], wr.at[128:321])])
    dma('x1', xtiles(1))
    dma('wi0', [(wi_hbm.at[0:128], wi.at[0:128])])
    dma('x2', xtiles(2))
    dma('x3', xtiles(3))
    dma('wi1', [(wi_hbm.at[128:321], wi.at[128:321])])
    dma('x0', xtiles(0))
    dma('ms0', [(ms_hbm.at[0:8], ms.at[0:8])])
    dma('ms1', [(ms_hbm.at[8:16], ms.at[8:16])])
    dma('w1a', [(gi_hbm, gi), (b1_hbm, b1v), (b2_hbm, b2v)]
        + [(w1t_hbm.at[:, tl(4 * b)], w1t.at[:, tl(4 * b)]) for b in range(4)])
    dma('w1b', w1cols(0, 1024))
    dma('w2', w1cols(1024, F) + [(w2_hbm, w2)])
    for copies in groups.values():
        for cp in copies:
            cp.start()

    def sync(name=None):
        if name is None:
            pl.semaphore_signal(rsem, 1)
            pl.semaphore_wait(rsem, 1)
        else:
            for cp in groups[name]:
                cp.wait()

    pltpu.store(zb, jnp.zeros((8, 128), i32), mask=_iota((8, 128), 1) < 4096)
    tok = []

    def pin(v):
        if len(tok) < 2:
            return v
        return pltpu.bitcast(pltpu.bitcast(v, i32) | (pltpu.bitcast(tok[-2], i32) & zb[...]), f32)

    slot = [0, 0]

    def pk(x):
        n = x.shape[0] // 2
        if slot[0] + n > TMP_ROWS:
            slot[0], slot[1] = 0, (slot[1] + 1) % TMP_TILES
        rs, cols = slice(slot[0], slot[0] + n), tl(slot[1])
        slot[0] += n
        tmp[rs, cols] = _pk(x)
        return tmp[rs, cols]

    nat = set(range(16))

    def xread(c, t):
        return stage[t, pl.ds(c, 128, stride=5), :] if t in nat else xt[tl(c), tl(t)]

    def pick(nrows, colfn):
        return jnp.where(_iota((nrows, 128), 1) == colfn(_iota((nrows, 128), 0)), 1.0, 0.0)

    def build_tables():
        p128 = pick(128, lambda r: (r >> 3) + 16 * (r & 7))
        pm[0:64, :] = pk(p128)
        pm[64:128, :] = pk(-p128)
        pm[128:200, :] = pk(pick(144, lambda r: jnp.where(r < 64, r, jnp.where(
            (r == 64) | (r == 130), 64, jnp.where(r < 128, 192 - r, -1)))))
        for c in range(5):
            row = _iota((128, 128), 0)
            d = c + 5 * _iota((128, 128), 1)
            idx = jnp.where(row < 64, d * row, jnp.where(row == 64, (d - c) * 64, d * (row - 64) + 160))
            idx = idx - 640 * (((idx >> 7) * 52429) >> 18)
            idx = jnp.where(idx > 320, 640 - idx, idx)
            neg = idx > 160
            x2 = jnp.where(neg, 320 - idx, idx).astype(f32) * float(2 * np.pi / 640)
            x2 = x2 * x2
            cosv = jnp.full((128, 128), 1.0 / math.factorial(14), f32)
            for n in range(12, -1, -2):
                cosv = 1.0 / math.factorial(n) - x2 * cosv
            g[c] = pk(jnp.where(neg, -cosv, cosv))

    def wstep1(wsrc, wn, f0, f1):
        for t2 in range(8):
            p0 = 64 if (wsrc is wi and t2 < 4) else 0
            o = [_mm_nt(_upk(pm[p0:p0 + 64, :]), wsrc[f0:f1, tl(t)]) for t in (2 * t2, 2 * t2 + 1)]
            for k in range(16):
                wn[8 * t2:8 * (t2 + 1), 384 * k + f0:384 * k + f1] = _pk(
                    jnp.concatenate([o[0][8 * k:8 * (k + 1)], o[1][8 * k:8 * (k + 1)]], axis=0))
            yield

    def wstep2a(wn, wdst):
        for k in range(16):
            oa = _mm_nt(_upk(pm[128:192, :]), _upk(wn[:, 384 * k:384 * k + 128]))
            wdst[0:64, tl(k)] = oa[0:64]
            wdst[256:320, tl(k)] = oa[64:128]
            yield

    def wstep2b(wn, wdst):
        row = _iota((8, 128), 0)
        top = row == 0
        for k in range(16):
            ob = _mm_nt(_upk(pm[128:192, :]), _upk(wn[:, 384 * k + 128:384 * k + 256]))
            oc = _mm_nt(_upk(jnp.concatenate([pm[128:160, 0:65], pm[192:200, 0:65]], axis=0)), _upk(wn[:, 384 * k + 256:384 * k + 321]))
            j4 = wdst[256:264, tl(k)]
            wdst[64:264, tl(k)] = jnp.concatenate(
                [ob[0:64], oc[0:64], jnp.where(top, oc[0:8], ob[64:72]), ob[72:128], jnp.where(top, ob[0:8], j4)],
                axis=0)
            ex = jnp.where(top, j4, jnp.where(row == 1, pltpu.roll(ob[64:72], 1, 0), oc[64:72]))
            wdst[320:336, tl(k)] = jnp.concatenate([ex, oc[72:80]], axis=0)
            yield

    nsum, shift, ready = {}, {}, {}

    def addsum(t, x):
        n = nsum.get(t, 0)
        cs[16 * n:16 * n + 16, tl(t)] = jnp.concatenate([_fold8(x), _fold8(x * x)], axis=0)
        nsum[t] = n + 1

    def shifted(t, x):
        if t not in nsum:
            shift[t] = x[0:1]
        return x - shift[t]

    def stats(t, double):
        n = nsum.pop(t)
        sq = cs[0:16, tl(t)]
        for i in range(1, n):
            sq = sq + cs[16 * i:16 * i + 16, tl(t)]
        m = jnp.sum(sq[0:8], axis=0, keepdims=True) * (1.0 / D)
        v = jnp.maximum(jnp.sum(sq[8:16], axis=0, keepdims=True) * (1.0 / D) - m * m, 0.0)
        if double:
            return m, lax.rsqrt(v + EPS * (v + EPS))
        return m, lax.rsqrt(v + EPS)

    def xload(a):
        for b in range(4):
            t = a + 4 * b
            x = xin[tl(t), :].T.astype(f32)
            stage[t] = x
            addsum(t, x)
            yield

    def p1cast(a):
        for b in range(4):
            m, r = stats(a + 4 * b, False)
            ready[a + 4 * b] = (None, r)
            for c in range(5):
                vv[64 * c:64 * (c + 1), tl(4 * a + b)] = _pk(xread(c, a + 4 * b) - m)
            yield

    def p1dot(a):
        st = [ready.pop(a + 4 * b) if a + 4 * b in ready else stats(a + 4 * b, False) for b in range(4)]
        r = jnp.concatenate([s[1] for s in st], axis=1)
        row = _iota((8, 512), 0)
        dc = er = ei = None
        if st[0][0] is not None:
            dc = jnp.where(row == 0, jnp.concatenate([s[0] for s in st], axis=1) * 128.0, 0.0)
        for c in range(5):
            y = _mm(_upk(g[c]), _upk(vv[64 * c:64 * (c + 1), 512 * a:512 * (a + 1)]))
            if dc is not None:
                y = jnp.concatenate([y[0:8] - dc, y[8:]], axis=0)
            y = y * r
            u64 = jnp.broadcast_to(y[64:65], (8, 512))
            cr = ci = jnp.zeros((8, 512), f32)
            for i, f in enumerate(EXTRA):
                cr = jnp.where(row == i, float(np.cos(2 * np.pi * c * f / 640)), cr)
                ci = jnp.where(row == i, float(-np.sin(2 * np.pi * c * f / 640)), ci)
            er = u64 * cr if er is None else er + u64 * cr
            if c > 0:
                ei = u64 * ci if ei is None else ei + u64 * ci
            vf[128 * c:128 * (c + 1), 512 * a:512 * (a + 1)] = jnp.concatenate(
                [y[0:64], jnp.where(row == 0, 0.0, y[64:72]), y[72:]], axis=0)
            if c == 4:
                vf[640:656, 512 * a:512 * (a + 1)] = jnp.concatenate([er, ei], axis=0)
            yield

    def p1post(a):
        def ld(c, r0, b):
            return vf[128 * c + r0:128 * c + r0 + 8, tl(4 * a + b)]
        for gq in (0, 1, 8, 2, 3, 4, 5, 6, 7):
            for odd in range(2):
                if gq < 8:
                    y = [_half4([(ld(c, 8 * gq, b), ld(c, 64 + 8 * gq, b)) for b in range(4)], odd, False)
                         for c in range(5)]
                else:
                    y = [_half4([(ld(5, 0, b), ld(5, 8, b)) for b in range(4)], odd, False)]
                for hi in range(2):
                    kb = odd + 2 * hi
                    if gq < 8:
                        ar = [y[c][hi][0] for c in range(5)]
                        ai = [y[c][hi][1] for c in range(5)]
                        x0r, a1r, a2r, b1r, b2r = _r5half(ar[0], ar[1] + ar[4], ar[2] + ar[3], ar[1] - ar[4],
                                                          ar[2] - ar[3])
                        x0i, a1i, a2i, b1i, b2i = _r5half(ai[0], ai[1] + ai[4], ai[2] + ai[3], ai[1] - ai[4],
                                                          ai[2] - ai[3])
                        xs = [(x0r, x0i), (a1r + b1i, a1i - b1r), (a2r + b2i, a2i - b2r),
                              (b2i - a2r, a2i + b2r), (b1i - a1r, a1i + b1r)]
                    else:
                        xs = [y[0][hi]]
                    for j in range(len(xs)):
                        r0 = 64 * j + 8 * gq if gq < 8 else 320
                        kq = kb if j < 3 else (4 - kb) % 4
                        yr, yi = _tw16(xs[j], a * kq)
                        pr[r0:r0 + 8, tl(4 * kq + a)] = yr
                        pi[r0:r0 + 8, tl(4 * kq + a)] = yi
                yield

    chunks = [(r0, min(R, r0 + 16)) for r0 in range(0, R, 16)]
    edges = [0, 4, 8, 13, 17, 21]
    units = [(kb, chunks[e0:e1]) for kb in range(4) for e0, e1 in zip(edges[:-1], edges[1:])]
    lane = _iota((8, 128), 1)

    def pk16(v):
        return pk(v if v.shape[0] == 16 else jnp.concatenate([v, jnp.zeros_like(v)], axis=0))

    def rows(parts, h):
        return _upk(jnp.concatenate([p[h] for p in parts], axis=0))

    def phase2(first):
        even, low = (lane & 1) == 0, lane < 64
        lhs, eo, z, out = {}, {}, {}, {}

        def pre(i):
            kb, chs = units[i]
            for r0, r1 in chs:
                t4 = _fft4([(pr[r0:r1, tl(4 * kb + a)], pi[r0:r1, tl(4 * kb + a)]) for a in range(4)], False)
                for ka in range(4):
                    re, im = pk16(t4[ka][0]), pltpu.roll(pk16(t4[ka][1]), 1, 1)
                    lhs.setdefault((i, ka), []).append((jnp.where(even, re, im), jnp.where(even, im, re)))
                yield

        def fwd(i, ka):
            m = ms.at[4 * units[i][0] + ka]
            parts = lhs.pop((i, ka))
            eo[i, ka] = [_mm(rows(parts, h), _upk(m[3 + h])) for h in range(2)]

        def filt(i, ka):
            kb, chs = units[i]
            e, o = eo.pop((i, ka))
            z[i, ka] = []
            for j, (r0, _) in enumerate(chs):
                q = slice(16 * j, 16 * j + 16)
                p_, q_ = e[q] + o[q], pltpu.roll(e[q] - o[q], 64, 1)
                w_r, w_i = wpr[r0:r0 + 16, tl(4 * ka + kb)], wpi[r0:r0 + 16, tl(4 * ka + kb)]
                p_, q_ = p_ * w_r + q_ * w_i, q_ * w_r - p_ * w_i
                pp, qp = pk16(p_), pk16(q_)
                z[i, ka].append((pk16(p_ + q_), jnp.where(low, pp, qp), jnp.where(low, qp, pp)))

        def inv(i, ka):
            m = ms.at[4 * units[i][0] + ka]
            parts = z.pop((i, ka))
            k1, k2, k3 = [_mm_nt(rows(parts, h), _upk(m[(0, 2, 1)[h]])) for h in range(3)]
            out.setdefault(i, []).append((k1 + k3, k1 - k2))

        def post(i, h):
            kb, chs = units[i]
            (ar, ai), (br, bi) = out.pop(i)
            for j, (r0, r1) in enumerate(chs):
                q = slice(16 * j, 16 * j + r1 - r0)
                pr[r0:r1, tl(4 * kb + 2 * h)] = ar[q] + br[q]
                pi[r0:r1, tl(4 * kb + 2 * h)] = ai[q] + bi[q]
                pr[r0:r1, tl(4 * kb + 2 * h + 1)] = ar[q] - br[q]
                pi[r0:r1, tl(4 * kb + 2 * h + 1)] = ai[q] - bi[q]

        steps = [(i, ka) for i in range(len(units)) for ka in (0, 2, 1, 3)]
        lag = 4
        emit(pre(0))
        gpre = iter(())
        for s in range(len(steps) + lag):
            if s < len(steps):
                i, ka = steps[s]
                if ka == 0:
                    emit(gpre)
                    if first and i == len(units) // 2:
                        sync('ms1')
                    gpre = pre(i + 1) if i + 1 < len(units) else iter(())
                fwd(i, ka)
            if 1 <= s <= len(steps):
                filt(*steps[s - 1])
            next(gpre, None)
            if s >= lag:
                i, ka = steps[s - lag]
                inv(i, ka)
                if ka >= 2:
                    post(i, ka - 2)
            if s % 4 == 2:
                next(gpre, None)

    def p3pre(a):
        row = _iota((8, 128), 0)

        def ld(rs, kb):
            c0, c1 = tl(4 * kb + a % 2), tl(4 * kb + 2 + a % 2)
            ar, ai, br, bi = pr[rs, c0], pi[rs, c0], pr[rs, c1], pi[rs, c1]
            v = ((ar + br, ai + bi) if a == 0 else (ar - bi, ai + br) if a == 1 else
                 (ar - br, ai - bi) if a == 2 else (ar + bi, ai - br))
            return _tw16(v, -a * kb)
        ex = _fft4([ld(slice(320, 328), kb) for kb in range(4)], True)
        for gq in range(8):
            for odd in range(2):
                y = [_half4([ld(slice(64 * j + 8 * gq, 64 * j + 8 * gq + 8), kb) for kb in range(4)], odd, True)
                     for j in range(5)]
                for hi in range(2):
                    b = odd + 2 * hi
                    yr = [y[j][hi][0] for j in range(5)]
                    yi = [y[j][hi][1] for j in range(5)]
                    v0r, a1r, a2r, b1r, b2r = _r5half(yr[0], yr[1] - yr[4], yr[2] - yr[3], yr[1] + yr[4],
                                                      yr[2] + yr[3])
                    v0i, a1i, a2i, b1i, b2i = _r5half(yi[0], yi[1] + yi[4], yi[2] + yi[3], yi[1] - yi[4],
                                                      yi[2] - yi[3])
                    vs = [(v0r, v0i), (a1r - b1i, a1i + b1r), (a2r - b2i, a2i + b2r), (a2r + b2i, a2i - b2r),
                          (a1r + b1i, a1i - b1r)]
                    for c in range(5):
                        vr, vi = vs[c]
                        if gq == 0:
                            er, ei = ex[b]
                            th1, th3 = 2 * np.pi * c / 10, 2 * np.pi * 3 * c / 10
                            t64 = (er[0:1] * float(2 * np.cos(th1)) - ei[0:1] * float(2 * np.sin(th1))
                                   + er[1:2] * float(2 * np.cos(th3)) - ei[1:2] * float(2 * np.sin(th3))
                                   + er[2:3] * float((-1) ** c))
                            vi = jnp.where(row == 0, jnp.broadcast_to(t64, (8, 128)), vi)
                        vv[64 * c + 8 * gq:64 * c + 8 * gq + 8, tl(4 * a + b)] = _pk(jnp.concatenate([vr, vi], axis=0))
                yield

    def p3dot(a):
        for c in range(5):
            y = _mm(_upk(gi[c]), _upk(vv[64 * c:64 * (c + 1), 512 * a:512 * (a + 1)]))
            for b in range(4):
                xn = xread(c, a + 4 * b) + y[:, tl(b)]
                xt[tl(c), tl(a + 4 * b)] = xn
                addsum(a + 4 * b, shifted(a + 4 * b, xn))
            if c == 4:
                nat.difference_update(a + 4 * b for b in range(4))
            yield

    def p3post(a):
        for b in range(4):
            t = a + 4 * b
            m, r = stats(t, True)
            m8 = jnp.broadcast_to(m + shift.pop(t), (8, 128))
            for c in range(5):
                xc = (xt[tl(c), tl(t)].reshape(16, 8, 128) - pin(m8)[None]).reshape(128, 128)
                hb[64 * c:64 * (c + 1), tl(4 * a + b)] = _pk(xc * r)
                yield

    def cat(ref, rs, tiles):
        return jnp.concatenate([ref[rs, tl(t)] for t in tiles], axis=1)

    def mm1_first(marking):
        for c0 in range(0, FM, 128):
            w = cat(w1t, slice(c0, c0 + 128), [0, 4, 8, 12])
            for c in range(5):
                y = _mm_nt(_upk(hb[64 * c:64 * (c + 1), 0:512]), w)
                acc[tl(c), c0:c0 + 128] = y
                if marking:
                    tok.append(y[0:8])
                yield

    def mm1_rest(c0, c1):
        tiles = [a + 4 * b for a in range(1, 4) for b in range(4)]
        h = _mm_nt(_upk(hb[:, 512:]), cat(w1t, slice(c0, c1), tiles)) + acc[:, c0:c1]
        u[:, c0:c1] = _pk(jax.nn.gelu(h + b1[0:1, c0:c1], approximate=True))

    def mm1_tail():
        tiles = [a + 4 * b for a in range(4) for b in range(4)]
        h = _mm_nt(cat(w1t, slice(FM, F), tiles), _upk(hb[...])) + jnp.concatenate([b1c[...]] * 5, axis=1)
        u[:, FM:F] = _pk(jax.nn.gelu(h, approximate=True).T)

    def to_state(c0, c1, t, y):
        xn = xt[128 * c0:128 * c1, tl(t)] + y + b2[0:1, tl(t)]
        xt[128 * c0:128 * c1, tl(t)] = xn
        xs = shifted(t, xn)
        vv[64 * c0:64 * c1, tl(4 * (t % 4) + t // 4)] = _pk(xs)
        addsum(t, xs)

    def to_output(c0, c1, t, y):
        xn = xt[128 * c0:128 * c1, tl(t)] + y + b2[0:1, tl(t)]
        for c in range(c0, c1):
            stage[t, pl.ds(c, 128, stride=5), :] = xn[tl(c - c0)]

    def mm2(tiles, sink):
        y = _mm(_upk(u[...]), cat(w2, slice(None), tiles))
        for i, t in enumerate(tiles):
            sink(0, 5, t, y[:, tl(i)])

    def mm2_fine(tiles, sink):
        w = cat(w2, slice(1536, F), tiles)
        rem = []
        for c in range(5):
            rem.append(_mm(_upk(u[64 * c:64 * (c + 1), 1536:F]), w))
            yield
        for i, t in enumerate(tiles):
            y = [r[:, tl(i)] for r in rem]
            for k0 in range(0, 1536, 512):
                w = w2[k0:k0 + 512, tl(t)]
                for c in range(5):
                    y[c] = y[c] + _mm(_upk(u[64 * c:64 * (c + 1), k0:k0 + 512]), w)
                    if k0 == 1024:
                        sink(c, c + 1, t, y[c])
                    yield

    def phase3_mm1(first):
        marking = []
        mm = mm1_first(marking)
        emit(p3pre(0))
        sync('w1a' if first else None)
        if first:
            b1f = b1v[...].astype(f32).reshape(1, F)
            b1[...] = jnp.broadcast_to(b1f, (8, F))
            b1c[...] = jnp.broadcast_to(b1f[:, F - 128:F], (128, 128)).T[64:128]
            b2[...] = jnp.broadcast_to(b2v[...].astype(f32).reshape(1, S), (8, S))
        emit(p3dot(0))
        sync()
        emit(p3post(0), woven(take(mm, 52), chain(p3pre(1), p3pre(2), p3pre(3)), 48 / 50))
        sync('w1b' if first else None)
        emit(p3dot(1), p3dot(2), p3dot(3))
        marking.append(True)
        emit(take(mm, 3), woven(mm, chain(p3post(1), p3post(2), p3post(3)), 6.0))
        tok.clear()
        for i, c0 in enumerate(range(0, FM, 256)):
            mm1_rest(c0, min(FM, c0 + 256))
            if i == 5:
                mm1_tail()
            if first and i == 3:
                sync('w2')

    def mm2_phase1():
        for i, pair in enumerate(([1, 5], [9, 13], [2, 6], [10, 14], [3, 7], [11, 15])):
            mm2(pair, to_state)
            if i in (2, 4):
                emit(p1dot(i // 2))
        mm = chain(mm2_fine([0, 4], to_state), mm2_fine([8, 12], to_state))
        emit(take(mm, 4), p1dot(3), take(mm, 2))
        sync()
        emit(woven(mm, chain(p1post(1), p1post(2), p1post(3)), 0.9), p1dot(0), p1post(0))
        sync()

    outs = []

    def flush(t0, t1):
        for t in range(t0, t1):
            xin[tl(t), :] = stage[t].astype(bf16).T
        cp = pltpu.make_async_copy(xin.at[128 * t0:128 * t1], o_hbm.at[128 * t0:128 * t1],
                                   sems.at[len(groups) + len(outs)])
        cp.start()
        outs.append(cp)

    def mm2_output():
        for c in range(7):
            mm2([2 * c, 2 * c + 1], to_output)
            if c == 5:
                flush(0, 10)
                sync()
        mm = mm2_fine([14, 15], to_output)
        emit(take(mm, 25))
        flush(10, 15)
        sync()
        emit(mm)
        flush(15, 16)

    build_tables()
    sync('wr0')
    emit(wstep1(wr, wn0, 0, 128), wstep2a(wn0, wpr))
    sync('wr1')
    wp = chain(wstep1(wr, wn0, 128, 321), wstep2b(wn0, wpr))
    emit(take(wp, 20))
    sync('x1')
    emit(woven(wp, xload(1), 0.5))
    sync('wi0')
    emit(woven(chain(p1cast(1), p1dot(1)), wstep1(wi, wn1, 0, 128), 1.0))
    sync('x2')
    emit(woven(xload(2), woven(p1post(1), wstep2a(wn1, wpi), 0.9), 4.5))
    sync('x3')
    emit(woven(xload(3), chain(p1cast(2), p1dot(2)), 2.3))
    sync()
    emit(woven(chain(p1cast(3), p1dot(3)), p1post(2), 2.0))
    sync('wi1')
    emit(woven(wstep1(wi, wn1, 128, 321), p1post(3), 2.3))
    sync('x0')
    emit(woven(chain(xload(0), p1cast(0), p1dot(0)), wstep2b(wn1, wpi), 1.3), p1post(0))
    sync('ms0')
    for layer in range(2):
        phase2(layer == 0)
        phase3_mm1(layer == 0)
        if layer == 0:
            mm2_phase1()
        else:
            mm2_output()
    for cp in outs:
        cp.wait()


@jax.jit
def pallas_interleave_layers__spectral_gfnet__mixer_token_mlp__prompt_kernel(A_x, A_w_r, A_w_i, B_x, B_w1, B_b1, B_w2, B_b2):
    gi, ms = _tables()
    args = (A_x.reshape(S, D), A_w_r.T, A_w_i.T, B_w1.T, B_b1, B_w2, B_b2, gi, ms)
    vmem = pltpu.VMEM
    out = pl.pallas_call(
        _kernel,
        out_shape=jax.ShapeDtypeStruct((S, D), bf16),
        in_specs=[pl.BlockSpec(memory_space=pltpu.HBM)] * len(args),
        out_specs=pl.BlockSpec(memory_space=pltpu.HBM),
        scratch_shapes=[
            vmem((S, D), bf16), vmem((321, S), bf16), vmem((321, S), bf16),
            vmem((F, S), bf16), vmem((F,), bf16), vmem((F, S), bf16), vmem((S,), bf16),
            vmem((5, 64, 128), u32), vmem((5, 64, 128), u32),
            vmem((16, 5, 64, 128), u32), vmem((200, 128), u32),
            vmem((64, 6144), u32), vmem((64, 6144), u32),
            vmem((R + 8, S), f32), vmem((R + 8, S), f32),
            vmem((D, S), f32), vmem((16, D, 128), f32),
            vmem((R, S), f32), vmem((R, S), f32),
            vmem((D // 2, S), u32), vmem((D // 2, F), u32), vmem((D, FM), f32),
            vmem((D // 2, S), u32), vmem((656, S), f32), vmem((80, S), f32),
            vmem((8, F), f32), vmem((8, S), f32), vmem((64, 128), f32),
            vmem((8, 128), i32), vmem((TMP_ROWS, 128 * TMP_TILES), u32),
            pltpu.SemaphoreType.DMA((16,)), pltpu.SemaphoreType.REGULAR,
        ],
        compiler_params=pltpu.CompilerParams(vmem_limit_bytes=100 * 1024 * 1024),
    )(*args)
    return out.reshape(1, S, D)
```
